```python
import os as _os
_os.environ.setdefault("JAX_PLATFORMS", "cpu")
import jax
import jax.numpy as jnp

def _softmax(x, axis=-1):
    return jax.nn.softmax(x, axis=axis)
def _gelu(x):
    return jax.nn.gelu(x, approximate=True)
def _silu(x):
    return jax.nn.silu(x)
def _sigmoid(x):
    return jax.nn.sigmoid(x)
def _layernorm(x, axis=-1, eps=1e-5):
    m = jnp.mean(x, axis=axis, keepdims=True)
    v = jnp.var(x, axis=axis, keepdims=True)
    return (x - m) / jnp.sqrt(v + eps)
def _scatter_add(tgt, idx, src, axis=0):
    return tgt.at[idx].add(src)
def _segment_sum(src, seg, n):
    return jax.ops.segment_sum(src, seg, n)
class _Rng:
    def __init__(self, key):
        self._k = key
    def _next(self):
        self._k, sub = jax.random.split(self._k)
        return sub
    def normal(self, shape):
        return jax.random.normal(self._next(), shape, dtype=jnp.bfloat16)
    def randint(self, lo, hi, shape):
        return jax.random.randint(self._next(), shape, lo, hi, dtype=jnp.int32)
    def uniform(self, shape, lo=0.0, hi=1.0):
        return jax.random.uniform(self._next(), shape, jnp.bfloat16, lo, hi)
    def permutation(self, n):
        return jax.random.permutation(self._next(), n)


kernel_name = 'gated_mix__linear_kernel_hedgehog__mixer_s_mlp__prompt'

def setup_inputs():
    _rng = _Rng(jax.random.key(int.from_bytes(__import__("os").urandom(4), "little")))
    _w = (lambda a: (lambda t: t.astype(jnp.bfloat16) if jnp.issubdtype(t.dtype, jnp.floating) else t)(jnp.asarray(a)))
    def _A_setup():
        B, S, D, H = 1, 2048, 512, 32
        Dh = D // H
        return {
            "x": _w((lambda *s: _rng.normal(s) * 0.05)(B, S, D)),
            "wqkv": _w((lambda *s: _rng.normal(s) * 1.6)(D, 3 * D)),
            "w_phi": _w((lambda *s: _rng.normal(s) * 1.6)(H, Dh, Dh) * (Dh ** -0.5)),
            "wo": _w((lambda *s: _rng.normal(s) * 0.05)(D, D)),
        }
    _A_in = _A_setup()

    def _B_setup():
        B, S, D, F = 1, 2048, 512, 1376
        return {
            "x":  _w((lambda *s: _rng.normal(s) * 0.05)(B, S, D)),
            "w1": _w((lambda *s: _rng.normal(s) * 0.4)(D, D) * (D ** -0.5)),
            "w2": _w((lambda *s: _rng.normal(s) * 0.4)(D, D) * (D ** -0.5)),
            "w3": _w((lambda *s: _rng.normal(s) * 0.4)(D, F) * (D ** -0.5)),
            "w4": _w((lambda *s: _rng.normal(s) * 0.4)(F, D) * (F ** -0.5)),
        }
    _B_in = _B_setup()

    return {
        "A_x": _A_in["x"],
        "A_wqkv": _A_in["wqkv"],
        "A_w_phi": _A_in["w_phi"],
        "A_wo": _A_in["wo"],
        "B_x": _B_in["x"],
        "B_w1": _B_in["w1"],
        "B_w2": _B_in["w2"],
        "B_w3": _B_in["w3"],
        "B_w4": _B_in["w4"],
        "gate_w": _w((lambda *s: _rng.normal(s) * 0.05)(512) * 16.0),
    }

def reference(A_x, A_wqkv, A_w_phi, A_wo, B_x, B_w1, B_w2, B_w3, B_w4, gate_w):
    def _A_ref(x, wqkv, w_phi, wo):
        B, S, D = x.shape
        H = 32; Dh = D // H
        qkv = (lambda x, *d: x.transpose(*d))((x @ wqkv).reshape(B, S, 3, H, Dh), 2, 0, 3, 1, 4)
        q, k, v = qkv[0], qkv[1], qkv[2]
        pq = jnp.einsum("bhsd,hdf->bhsf", q, w_phi)
        pk = jnp.einsum("bhsd,hdf->bhsf", k, w_phi)
        phi_q = jnp.concatenate([_softmax(pq, axis=-1), _softmax(-pq, axis=-1)], axis=-1)
        phi_k = jnp.concatenate([_softmax(pk, axis=-1), _softmax(-pk, axis=-1)], axis=-1)
        kv = jnp.einsum("bhsf,bhsd->bhfd", phi_k, v)
        z  = jnp.einsum("bhsf->bhf", phi_k)
        num = jnp.einsum("bhqf,bhfd->bhqd", phi_q, kv)
        den = jnp.einsum("bhqf,bhf->bhq", phi_q, z)[..., None] + 1e-6
        o = num / den
        return (lambda x, *d: x.transpose(*d))(o, 0, 2, 1, 3).reshape(B, S, D) @ wo

    def _B_ref(x, w1, w2, w3, w4):
        B, S, D = x.shape
        h = _gelu(_layernorm(x, axis=-1) @ w1)
        c = D // 4
        g0 = jnp.pad(h[:, :, 0*c:1*c], ((0, 0), (1, 0), (0, 0)))[:, :S, :]
        g1 = jnp.pad(h[:, :, 1*c:2*c], ((0, 0), (0, 1), (0, 0)))[:, 1:, :]
        g2 = jnp.pad(h[:, :, 2*c:3*c], ((0, 0), (2, 0), (0, 0)))[:, :S, :]
        g3 = jnp.pad(h[:, :, 3*c:   ], ((0, 0), (0, 2), (0, 0)))[:, 2:, :]
        hs = jnp.concatenate([g0, g1, g2, g3], axis=-1) @ w2
        x1 = x + hs
        h2 = _gelu(_layernorm(x1, axis=-1) @ w3) @ w4
        return x1 + h2

    x = A_x
    g = _sigmoid((x * gate_w).sum(-1, keepdims=True))
    a = _A_ref(x, A_wqkv, A_w_phi, A_wo)
    b = _B_ref(x, B_w1, B_w2, B_w3, B_w4)
    return g * a + (1 - g) * b
```

```python
import jax
import jax.numpy as jnp
from jax import lax
import jax.experimental.pallas as pl
import jax.experimental.pallas.tpu as pltpu

S, D, H, DH, F = 2048, 512, 32, 16, 1376
NJ = 8
T = 256
NT = S // T
PAD = 8
LOG2E = 1.4426950408889634
NT_DIMS = (((1,), (1,)), ((), ()))
f32 = jnp.float32
bf16 = jnp.bfloat16


def _gelu(x):
    c = 0.7978845608028654
    return 0.5 * x * (1.0 + jnp.tanh(c * (x + 0.044715 * (x * x * x))))


def _ln(x):
    m = jnp.mean(x, axis=-1, keepdims=True)
    xc = x - m
    v = jnp.mean(xc * xc, axis=-1, keepdims=True)
    return xc * lax.rsqrt(v + 1e-5)


def _fold4(a, op):
    return op(a, pltpu.roll(a, 4, 0))


def _dual_exp(p):
    mx = _fold4(jnp.max(p, axis=0), jnp.maximum)
    mn = _fold4(jnp.min(p, axis=0), jnp.minimum)
    ep = jnp.exp2(p - mx[None])
    en = jnp.exp2(mn[None] - p)
    rp = 1.0 / _fold4(jnp.sum(ep, axis=0), jnp.add)
    rn = 1.0 / _fold4(jnp.sum(en, axis=0), jnp.add)
    return ep, en, rp, rn


def kernel(x_hbm, wqkv_hbm, wphi_hbm, wo_hbm, w1_hbm, w2_hbm, w3t_hbm, w4_hbm, gw_hbm,
           out_hbm,
           x_v, wq_v, wk_v, wv_v, wphi_v, wo_v, w1_v, w2_v, w3t_v, w4_v, gw_v, out_v,
           wt_ref, h_ref, kv_ref, z_ref, kvt_ref, phi_ref, p_ref, wsem, xsem, osem):
    def xcopy(t):
        return pltpu.make_async_copy(x_hbm.at[pl.ds(t * T, T)], x_v.at[pl.ds(t * T, T)], xsem.at[t])

    def ocopy(t):
        return pltpu.make_async_copy(out_v.at[pl.ds(t * T, T)], out_hbm.at[pl.ds(t * T, T)], osem.at[t])

    c_phi = pltpu.make_async_copy(wphi_hbm, wphi_v, wsem.at[0])
    c_wk = pltpu.make_async_copy(wqkv_hbm.at[:, D:2 * D], wk_v, wsem.at[1])
    c_wv = pltpu.make_async_copy(wqkv_hbm.at[:, 2 * D:3 * D], wv_v, wsem.at[2])
    c_w1 = pltpu.make_async_copy(w1_hbm, w1_v, wsem.at[3])
    c_wq = pltpu.make_async_copy(wqkv_hbm.at[:, 0:D], wq_v, wsem.at[4])
    c_w2 = pltpu.make_async_copy(w2_hbm, w2_v, wsem.at[5])
    c_w3 = pltpu.make_async_copy(w3t_hbm, w3t_v, wsem.at[6])
    c_w4 = pltpu.make_async_copy(w4_hbm, w4_v, wsem.at[7])
    c_wo = pltpu.make_async_copy(wo_hbm, wo_v, wsem.at[8])
    c_gw = pltpu.make_async_copy(gw_hbm, gw_v, wsem.at[9])
    c_phi.start()
    c_wk.start()
    c_wv.start()
    xcopy(0).start()
    c_w1.start()
    for t in range(1, NT):
        xcopy(t).start()
    for c in (c_wq, c_w2, c_w3, c_w4, c_wo, c_gw):
        c.start()

    kv_ref[...] = jnp.zeros_like(kv_ref)
    z_ref[...] = jnp.zeros_like(z_ref)
    h_ref[0:PAD, :] = jnp.zeros((PAD, D), f32)
    h_ref[PAD + S:PAD + S + PAD, :] = jnp.zeros((PAD, D), f32)

    c_phi.wait()
    sel = (lax.broadcasted_iota(jnp.int32, (H, D), 0)
           == lax.broadcasted_iota(jnp.int32, (H, D), 1) // DH)
    sel = jnp.where(sel, 1.0, 0.0).astype(bf16)
    bm = jnp.dot(wphi_v[...], sel, preferred_element_type=f32)
    dmask = (lax.broadcasted_iota(jnp.int32, (DH * DH, D), 0) // DH
             == lax.broadcasted_iota(jnp.int32, (DH * DH, D), 1) % DH)
    cm = jnp.sum(jnp.where(dmask, bm, 0.0).reshape(DH, DH, D), axis=0).astype(bf16)
    e3 = ((lax.broadcasted_iota(jnp.int32, (128, DH), 0) % 64) // 4
          == lax.broadcasted_iota(jnp.int32, (128, DH), 1))
    e3 = jnp.where(e3, 1.0, 0.0).astype(bf16)
    pall = jnp.dot(e3, cm, preferred_element_type=f32)
    rr = lax.broadcasted_iota(jnp.int32, (128, D), 0)
    cc = lax.broadcasted_iota(jnp.int32, (128, D), 1)
    pmask = ((cc // DH) % 8) == ((rr // 64) * 4 + rr % 4)
    p_ref[...] = jnp.where(pmask, pall, 0.0).astype(bf16)

    def fold(w_v, base):
        for g in range(4):
            wt = lax.dot_general(p_ref[:, g * 128:(g + 1) * 128], w_v[:, g * 128:(g + 1) * 128],
                                 NT_DIMS, preferred_element_type=f32)
            wt_ref[base + g * 128: base + (g + 1) * 128, :] = (wt * LOG2E).astype(bf16)

    c_wk.wait()
    fold(wk_v, D)
    c_wv.wait()
    wt_ref[2 * D:3 * D, :] = wv_v[...].T
    c_w1.wait()

    def p1(t, carry):
        r0 = pl.multiple_of(t * T, T)
        xcopy(t).wait()
        x = x_v[pl.ds(r0, T), :]
        pv = lax.dot_general(wt_ref[D:3 * D, :], x, NT_DIMS, preferred_element_type=f32)
        xn = _ln(x.astype(f32)).astype(bf16)
        hpre = jnp.dot(xn, w1_v[...], preferred_element_type=f32)
        vt = pv[D:2 * D, :].astype(bf16)
        for j in range(NJ):
            zp = zn = None
            for c in range(T // 128):
                p = pv[j * 64:(j + 1) * 64, c * 128:(c + 1) * 128].reshape(8, 8, 128)
                ep, en, rp, rn = _dual_exp(p)
                ep = (ep * rp[None]).reshape(64, 128)
                en = (en * rn[None]).reshape(64, 128)
                zp = ep if zp is None else zp + ep
                zn = en if zn is None else zn + en
                phi_ref[j * 128:j * 128 + 64, c * 128:(c + 1) * 128] = ep.astype(bf16)
                phi_ref[j * 128 + 64:(j + 1) * 128, c * 128:(c + 1) * 128] = en.astype(bf16)
            z_ref[j * 128:j * 128 + 64, :] += zp
            z_ref[j * 128 + 64:(j + 1) * 128, :] += zn
            kv_ref[j * 64:(j + 1) * 64, :] += lax.dot_general(
                vt[j * 64:(j + 1) * 64, :], phi_ref[j * 128:(j + 1) * 128, :], NT_DIMS,
                preferred_element_type=f32)
        h_ref[pl.ds(PAD + r0, T), :] = _gelu(hpre)
        return carry

    lax.fori_loop(0, NT, p1, 0)

    c_wq.wait()
    fold(wq_v, 0)
    r2 = lax.broadcasted_iota(jnp.int32, (D, 128), 0)
    c2 = lax.broadcasted_iota(jnp.int32, (D, 128), 1)
    kmask = ((r2 // DH) % 4) == (c2 % 4)
    kvt_ref[...] = jnp.where(kmask, kv_ref[...], 0.0).astype(bf16)
    z_ref[...] = jnp.broadcast_to(jnp.sum(z_ref[...], axis=1, keepdims=True), z_ref.shape)
    for c in (c_w2, c_w3, c_w4, c_wo, c_gw):
        c.wait()
    gw = gw_v[...].astype(f32)

    def p2(t, carry):
        r0 = pl.multiple_of(t * T, T)
        x = x_v[pl.ds(r0, T), :]
        xf = x.astype(f32)
        hw = h_ref[pl.ds(r0, T + 2 * PAD), :]
        hs = jnp.concatenate([
            hw[PAD - 1:PAD - 1 + T, 0:128],
            hw[PAD + 1:PAD + 1 + T, 128:256],
            hw[PAD - 2:PAD - 2 + T, 256:384],
            hw[PAD + 2:PAD + 2 + T, 384:512]], axis=1).astype(bf16)
        x1 = xf + jnp.dot(hs, w2_v[...], preferred_element_type=f32)
        pq = lax.dot_general(wt_ref[0:D, :], x, NT_DIMS, preferred_element_type=f32)
        x1n = _ln(x1).astype(bf16)
        upre = lax.dot_general(x1n, w3t_v[...], NT_DIMS, preferred_element_type=f32)
        ots = []
        for j in range(NJ):
            zp = z_ref[j * 128:j * 128 + 64, :].reshape(8, 8, 128)
            zn = z_ref[j * 128 + 64:(j + 1) * 128, :].reshape(8, 8, 128)
            for c in range(T // 128):
                p = pq[j * 64:(j + 1) * 64, c * 128:(c + 1) * 128].reshape(8, 8, 128)
                ep, en, rp, rn = _dual_exp(p)
                den = jnp.sum(ep * zp, axis=0) * rp + jnp.sum(en * zn, axis=0) * rn
                rd = 1.0 / (_fold4(den, jnp.add) + 1e-6)
                ep = (ep * (rp * rd)[None]).reshape(64, 128)
                en = (en * (rn * rd)[None]).reshape(64, 128)
                phi_ref[j * 128:j * 128 + 64, c * 128:(c + 1) * 128] = ep.astype(bf16)
                phi_ref[j * 128 + 64:(j + 1) * 128, c * 128:(c + 1) * 128] = en.astype(bf16)
            ots.append(jnp.dot(kvt_ref[j * 64:(j + 1) * 64, :], phi_ref[j * 128:(j + 1) * 128, :],
                               preferred_element_type=f32))
        u = _gelu(upre).astype(bf16)
        o = jnp.concatenate(ots, axis=0).T.astype(bf16)
        b = x1 + jnp.dot(u, w4_v[...], preferred_element_type=f32)
        a = jnp.dot(o, wo_v[...], preferred_element_type=f32)
        gl = jnp.sum(xf * gw, axis=-1, keepdims=True)
        gate = 1.0 / (1.0 + jnp.exp(-gl))
        out_v[pl.ds(r0, T), :] = (b + gate * (a - b)).astype(bf16)
        ocopy(t).start()
        return carry

    lax.fori_loop(0, NT, p2, 0)
    for t in range(NT):
        ocopy(t).wait()


@jax.jit
def pallas_gated_mix__linear_kernel_hedgehog__mixer_s_mlp__prompt_kernel(
        A_x, A_wqkv, A_w_phi, A_wo, B_x, B_w1, B_w2, B_w3, B_w4, gate_w):
    x = A_x.reshape(S, D)
    wphi = jnp.transpose(A_w_phi, (1, 2, 0)).reshape(DH * DH, H)
    gw = gate_w.reshape(1, D)
    w3t = B_w3.T
    hbm = pl.BlockSpec(memory_space=pl.ANY)
    out = pl.pallas_call(
        kernel,
        out_shape=jax.ShapeDtypeStruct((S, D), bf16),
        in_specs=[hbm] * 9,
        out_specs=hbm,
        scratch_shapes=[
            pltpu.VMEM((S, D), bf16),
            pltpu.VMEM((D, D), bf16),
            pltpu.VMEM((D, D), bf16),
            pltpu.VMEM((D, D), bf16),
            pltpu.VMEM((DH * DH, H), bf16),
            pltpu.VMEM((D, D), bf16),
            pltpu.VMEM((D, D), bf16),
            pltpu.VMEM((D, D), bf16),
            pltpu.VMEM((F, D), bf16),
            pltpu.VMEM((F, D), bf16),
            pltpu.VMEM((1, D), bf16),
            pltpu.VMEM((S, D), bf16),
            pltpu.VMEM((3 * D, D), bf16),
            pltpu.VMEM((S + 2 * PAD, D), f32),
            pltpu.VMEM((D, 128), f32),
            pltpu.VMEM((NJ * 128, 128), f32),
            pltpu.VMEM((D, 128), bf16),
            pltpu.VMEM((NJ * 128, T), bf16),
            pltpu.VMEM((128, D), bf16),
            pltpu.SemaphoreType.DMA((10,)),
            pltpu.SemaphoreType.DMA((NT,)),
            pltpu.SemaphoreType.DMA((NT,)),
        ],
        compiler_params=pltpu.CompilerParams(vmem_limit_bytes=100 * 1024 * 1024),
    )(x, A_wqkv, wphi, A_wo, B_w1, B_w2, w3t, B_w4, gw)
    return out.reshape(1, S, D)
```

```python
import jax
import jax.numpy as jnp
from jax import lax
import jax.experimental.pallas as pl
import jax.experimental.pallas.tpu as pltpu

S, D, H, DH, F = 2048, 512, 32, 16, 1376
NJ = 8
T0 = 256
T = 512
NT = S // T
SPL = [int(v) for v in '256,128,128'.split(',')]
P1ORD = 'w2,pk,ln1,v,w1,kv'.split(',')
LN2POS = [int(v) for v in '0,1'.split(',')]
AH = 16
PAD = 8
LNC = int(32)
LOG2E = 1.4426950408889634
NT_DIMS = (((1,), (1,)), ((), ()))
SHIFTS = (-1, 1, -2, 2)
f32 = jnp.float32
bf16 = jnp.bfloat16


def _gelu(x):
    c = 0.7978845608028654
    t = jnp.tanh(x * (c + (c * 0.044715) * (x * x)))
    hx = 0.5 * x
    return hx + hx * t


def _ln(x):
    m = jnp.mean(x, axis=-1, keepdims=True)
    xc = x - m
    v = jnp.mean(xc * xc, axis=-1, keepdims=True)
    return xc * lax.rsqrt(v + 1e-5)


def _recip(x):
    r = pl.reciprocal(x, approx=True)
    return r * (2.0 - x * r)


def _fold4(a, op):
    return op(a, pltpu.roll(a, 4, 0))


def _dual_exp(p):
    mx = _fold4(jnp.max(p, axis=0), jnp.maximum)
    mn = _fold4(jnp.min(p, axis=0), jnp.minimum)
    ep = jnp.exp2(p - mx[None])
    en = jnp.exp2(mn[None] - p)
    rp = _recip(_fold4(jnp.sum(ep, axis=0), jnp.add))
    rn = _recip(_fold4(jnp.sum(en, axis=0), jnp.add))
    return ep, en, rp, rn


def kernel(x_hbm, wqkv_hbm, wphi_hbm, wo_hbm, w1_hbm, w2_hbm, w3t_hbm, w4_hbm, gw_hbm,
           out_hbm,
           x_v, wq_v, wk_v, wv_v, wphi_v, wo_v, w1_v, w2_v, w3t_v, w4_v, gw_v, out_v,
           wt_ref, h_ref, kv_ref, z_ref, kvt_ref, phi_ref, p_ref, xn_ref, vt_ref,
           x1_ref, x1n_ref, sem):
    def xcopy(a, b, k):
        return pltpu.make_async_copy(x_hbm.at[a:b], x_v.at[a:b], sem.at[k])

    c_phi = pltpu.make_async_copy(wphi_hbm, wphi_v, sem.at[0])
    c_wk = pltpu.make_async_copy(wqkv_hbm.at[:, D:2 * D], wk_v, sem.at[1])
    c_x0 = xcopy(0, T0 + AH, 2)
    c_wv = pltpu.make_async_copy(wqkv_hbm.at[:, 2 * D:3 * D], wv_v, sem.at[3])
    g4 = [pltpu.make_async_copy(w1_hbm, w1_v, sem.at[4]), xcopy(T0 + AH, T + AH, 4)]
    g5 = [pltpu.make_async_copy(w2_hbm, w2_v, sem.at[5]), xcopy(T + AH, S, 5)]
    late = [pltpu.make_async_copy(wqkv_hbm.at[:, 0:D], wq_v, sem.at[6]),
            pltpu.make_async_copy(w3t_hbm, w3t_v, sem.at[6]),
            pltpu.make_async_copy(w4_hbm, w4_v, sem.at[6]),
            pltpu.make_async_copy(wo_hbm, wo_v, sem.at[6]),
            pltpu.make_async_copy(gw_hbm, gw_v, sem.at[6])]
    c_phi.start()
    c_wk.start()

    x_v[S:S + AH, :] = jnp.zeros((AH, D), bf16)
    for n in range(4):
        h_ref[n, 0:PAD, :] = jnp.zeros((PAD, 128), f32)

    c_phi.wait()
    c_x0.start()
    c_wv.start()
    sel = (lax.broadcasted_iota(jnp.int32, (H, D), 0)
           == lax.broadcasted_iota(jnp.int32, (H, D), 1) // DH)
    sel = jnp.where(sel, 1.0, 0.0).astype(bf16)
    bm = jnp.dot(wphi_v[...], sel, preferred_element_type=f32)
    dmask = (lax.broadcasted_iota(jnp.int32, (DH * DH, D), 0) // DH
             == lax.broadcasted_iota(jnp.int32, (DH * DH, D), 1) % DH)
    cm = jnp.sum(jnp.where(dmask, bm, 0.0).reshape(DH, DH, D), axis=0).astype(bf16)
    e3 = ((lax.broadcasted_iota(jnp.int32, (128, DH), 0) % 64) // 4
          == lax.broadcasted_iota(jnp.int32, (128, DH), 1))
    e3 = jnp.where(e3, 1.0, 0.0).astype(bf16)
    pall = jnp.dot(e3, cm, preferred_element_type=f32)
    rr = lax.broadcasted_iota(jnp.int32, (128, D), 0)
    cc = lax.broadcasted_iota(jnp.int32, (128, D), 1)
    pmask = ((cc // DH) % 8) == ((rr // 64) * 4 + rr % 4)
    p_ref[...] = jnp.where(pmask, pall, 0.0).astype(bf16)

    def fold(w_v, base):
        for g in range(4):
            wt = lax.dot_general(p_ref[:, g * 128:(g + 1) * 128], w_v[:, g * 128:(g + 1) * 128],
                                 NT_DIMS, preferred_element_type=f32)
            wt_ref[base + g * 128: base + (g + 1) * 128, :] = (wt * LOG2E).astype(bf16)

    def st_pk(r0, n, off=0, first=False):
        x = x_v[pl.ds(r0, n), :]
        pk = lax.dot_general(wt_ref[D:2 * D, :], x, NT_DIMS, preferred_element_type=f32)
        for c in range(n // 128):
            cs = slice(off + c * 128, off + (c + 1) * 128)
            for j in range(NJ):
                p = pk[j * 64:(j + 1) * 64, c * 128:(c + 1) * 128].reshape(8, 8, 128)
                ep, en, rp, rn = _dual_exp(p)
                ep = (ep * rp[None]).reshape(64, 128)
                en = (en * rn[None]).reshape(64, 128)
                if first and c == 0:
                    z_ref[j * 128:j * 128 + 64, :] = ep
                    z_ref[j * 128 + 64:(j + 1) * 128, :] = en
                else:
                    z_ref[j * 128:j * 128 + 64, :] += ep
                    z_ref[j * 128 + 64:(j + 1) * 128, :] += en
                phi_ref[j * 128:j * 128 + 64, cs] = ep.astype(bf16)
                phi_ref[j * 128 + 64:(j + 1) * 128, cs] = en.astype(bf16)

    def st_v(r0, n, off=0):
        x = x_v[pl.ds(r0, n), :]
        vt_ref[:, off:off + n] = lax.dot_general(wt_ref[2 * D:3 * D, :], x, NT_DIMS,
                                                 preferred_element_type=f32).astype(bf16)

    def st_kv(first=False):
        for j in range(NJ):
            r = lax.dot_general(vt_ref[j * 64:(j + 1) * 64, :], phi_ref[j * 128:(j + 1) * 128, :],
                                NT_DIMS, preferred_element_type=f32)
            if first:
                kv_ref[j * 64:(j + 1) * 64, :] = r
            else:
                kv_ref[j * 64:(j + 1) * 64, :] += r

    def st_ln1(r0, n, off=0):
        for r in range(0, n, LNC):
            m = min(LNC, n - r)
            xn_ref[off + r:off + r + m, :] = _ln(x_v[pl.ds(r0 + r, m), :].astype(f32)).astype(bf16)

    def st_w1(r0, n, off=0):
        h = _gelu(jnp.dot(xn_ref[off:off + n, :], w1_v[...], preferred_element_type=f32))
        for q in range(4):
            h_ref[q, pl.ds(PAD + r0, n), :] = h[:, q * 128:(q + 1) * 128]

    def st_w2(r0):
        hs = jnp.concatenate(
            [h_ref[q, pl.ds(PAD + r0 + SHIFTS[q], T), :].astype(bf16) for q in range(4)], axis=1)
        x1_ref[pl.ds(r0, T), :] = (x_v[pl.ds(r0, T), :].astype(f32)
                                   + jnp.dot(hs, w2_v[...], preferred_element_type=f32))

    def st_ln2(r0, a, b):
        for r in range(a, b, LNC):
            x1n_ref[r:r + LNC, :] = _ln(x1_ref[pl.ds(r0 + r, LNC), :]).astype(bf16)

    c_wk.wait()
    for c in g4:
        c.start()
    fold(wk_v, D)
    c_x0.wait()
    for c in g5:
        c.start()
    st_pk(0, T0, first=True)
    c_wv.wait()
    for c in late:
        c.start()
    wt_ref[2 * D:3 * D, :] = wv_v[...].T
    st_v(0, T0)
    st_ln1(0, T0 + AH)
    for c in g4:
        c.wait()
    st_w1(0, T0 + AH)
    st_pk(T0, T - T0, off=T0)
    st_ln1(T0 + AH, T - T0, off=T0 + AH)
    st_v(T0, T - T0, off=T0)
    st_w1(T0 + AH, T - T0, off=T0 + AH)
    st_kv(True)
    for c in g5:
        c.wait()

    def p1(t, carry):
        r0 = pl.multiple_of(t * T, T)
        for s in P1ORD:
            if s == 'pk': st_pk(r0, T)
            elif s == 'w2': st_w2(r0 - T)
            elif s == 'ln1': st_ln1(r0 + AH, T)
            elif s == 'v': st_v(r0, T)
            elif s == 'w1': st_w1(r0 + AH, T)
            elif s == 'kv': st_kv()
        return carry

    lax.fori_loop(1, NT, p1, 0)

    for c in late:
        c.wait()
    st_w2(S - T)
    fold(wq_v, 0)
    st_ln2(0, 0, T)
    r2 = lax.broadcasted_iota(jnp.int32, (D, 128), 0)
    c2 = lax.broadcasted_iota(jnp.int32, (D, 128), 1)
    kmask = ((r2 // DH) % 4) == (c2 % 4)
    kvt_ref[...] = jnp.where(kmask, kv_ref[...], 0.0).astype(bf16)
    z_ref[...] = jnp.broadcast_to(jnp.sum(z_ref[...], axis=1, keepdims=True), z_ref.shape)

    def st_pq(r0):
        x = x_v[pl.ds(r0, T), :]
        pq = lax.dot_general(wt_ref[0:D, :], x, NT_DIMS, preferred_element_type=f32)
        for c in range(T // 128):
            for j in range(NJ):
                zp = z_ref[j * 128:j * 128 + 64, :].reshape(8, 8, 128)
                zn = z_ref[j * 128 + 64:(j + 1) * 128, :].reshape(8, 8, 128)
                p = pq[j * 64:(j + 1) * 64, c * 128:(c + 1) * 128].reshape(8, 8, 128)
                ep, en, rp, rn = _dual_exp(p)
                den = jnp.sum(ep * zp, axis=0) * rp + jnp.sum(en * zn, axis=0) * rn
                rd = _recip(_fold4(den, jnp.add) + 1e-6)
                ep = (ep * (rp * rd)[None]).reshape(64, 128)
                en = (en * (rn * rd)[None]).reshape(64, 128)
                phi_ref[j * 128:j * 128 + 64, c * 128:(c + 1) * 128] = ep.astype(bf16)
                phi_ref[j * 128 + 64:(j + 1) * 128, c * 128:(c + 1) * 128] = en.astype(bf16)

    def p2(t, carry):
        r0 = pl.multiple_of(t * T, T)
        rn = pl.multiple_of(((t + 1) % NT) * T, T)
        st_pq(r0)
        u = _gelu(lax.dot_general(x1n_ref[...], w3t_v[...], NT_DIMS,
                                  preferred_element_type=f32)).astype(bf16)
        ots = [jnp.dot(kvt_ref[j * 64:(j + 1) * 64, :], phi_ref[j * 128:(j + 1) * 128, :],
                       preferred_element_type=f32) for j in range(NJ)]
        o = jnp.concatenate(ots, axis=0).T.astype(bf16)
        gw = gw_v[...].astype(f32).reshape(1, D)
        off = 0
        lnstep = T // len(LN2POS)
        for k, n in enumerate(SPL):
            if k in LN2POS:
                i = LN2POS.index(k)
                st_ln2(rn, i * lnstep, (i + 1) * lnstep)
            rk = r0 + off
            b = x1_ref[pl.ds(rk, n), :] + jnp.dot(u[off:off + n], w4_v[...],
                                                  preferred_element_type=f32)
            a = jnp.dot(o[off:off + n], wo_v[...], preferred_element_type=f32)
            gl = jnp.sum(x_v[pl.ds(rk, n), :].astype(f32) * gw, axis=-1, keepdims=True)
            gate = 0.5 * jnp.tanh(0.5 * gl) + 0.5
            out_v[pl.ds(rk, n), :] = (b + gate * (a - b)).astype(bf16)
            pltpu.make_async_copy(out_v.at[pl.ds(rk, n)], out_hbm.at[pl.ds(rk, n)], sem.at[7]).start()
            off += n
        return carry

    lax.fori_loop(0, NT, p2, 0)
    pltpu.make_async_copy(out_v, out_hbm, sem.at[7]).wait()


@jax.jit
def pallas_gated_mix__linear_kernel_hedgehog__mixer_s_mlp__prompt_kernel(
        A_x, A_wqkv, A_w_phi, A_wo, B_x, B_w1, B_w2, B_w3, B_w4, gate_w):
    x = A_x.reshape(S, D)
    wphi = jnp.transpose(A_w_phi, (1, 2, 0)).reshape(DH * DH, H)
    w3t = B_w3.T
    hbm = pl.BlockSpec(memory_space=pl.ANY)
    out = pl.pallas_call(
        kernel,
        out_shape=jax.ShapeDtypeStruct((S, D), bf16),
        in_specs=[hbm] * 9,
        out_specs=hbm,
        scratch_shapes=[
            pltpu.VMEM((S + AH, D), bf16),
            pltpu.VMEM((D, D), bf16),
            pltpu.VMEM((D, D), bf16),
            pltpu.VMEM((D, D), bf16),
            pltpu.VMEM((DH * DH, H), bf16),
            pltpu.VMEM((D, D), bf16),
            pltpu.VMEM((D, D), bf16),
            pltpu.VMEM((D, D), bf16),
            pltpu.VMEM((F, D), bf16),
            pltpu.VMEM((F, D), bf16),
            pltpu.VMEM((D,), bf16),
            pltpu.VMEM((S, D), bf16),
            pltpu.VMEM((3 * D, D), bf16),
            pltpu.VMEM((4, PAD + S + AH, 128), f32),
            pltpu.VMEM((D, 128), f32),
            pltpu.VMEM((NJ * 128, 128), f32),
            pltpu.VMEM((D, 128), bf16),
            pltpu.VMEM((NJ * 128, T), bf16),
            pltpu.VMEM((128, D), bf16),
            pltpu.VMEM((T + AH, D), bf16),
            pltpu.VMEM((D, T), bf16),
            pltpu.VMEM((S, D), f32),
            pltpu.VMEM((T, D), bf16),
            pltpu.SemaphoreType.DMA((8,)),
        ],
        compiler_params=pltpu.CompilerParams(vmem_limit_bytes=100 * 1024 * 1024),
    )(x, A_wqkv, wphi, A_wo, B_w1, B_w2, w3t, B_w4, gate_w)
    return out.reshape(1, S, D)
```

```python
import jax
import jax.numpy as jnp
from jax import lax
import jax.experimental.pallas as pl
import jax.experimental.pallas.tpu as pltpu

S, D, H, DH, F = 2048, 512, 32, 16, 1376
NJ = 8
T0 = 256
T = 512
NT = S // T
T2 = int(1024)
NT2 = S // T2
HC = 512
SPL = [int(v) for v in '256,256,256,192,64'.split(',')]
P1ORD = 'w2,pk,ln1,v,w1,kv'.split(',')
P1LAST = 'pk,finz,ln1,v,w1,kv,fin,w2,fq,ln2,w2l,wait'.split(',')
P1MID = 'w2l,fq,ln2,fin,finz,wait'.split(',')
NLOOP1 = int(3)
FIRST2 = int(0)
P2ORD = 'w3m0,ln2c1,w3r0,pq,w3r1,w3m1,num,ln2n,w40,wo0,w41,wo1,w42,wo2,w43,wo3,w44,wo4'.split(',')
GC = int(64)
LN2POS = [int(v) for v in '0'.split(',')]
GPOS = int(3)
FM = 1280
RSQ = int(1)
AH = 16
PAD = 8
LNC = int(16)
LNC1 = int(16)
LNC0 = int(32)
U2 = int(1)
PRO = int(1)
LOG2E = 1.4426950408889634
NT_DIMS = (((1,), (1,)), ((), ()))
SHIFTS = (-1, 1, -2, 2)
f32 = jnp.float32
bf16 = jnp.bfloat16
u32 = jnp.uint32


SC = int(0)


class _Null:
    def __enter__(self):
        return None

    def __exit__(self, *a):
        return False


def scope(name):
    return jax.named_scope(name) if SC else _Null()


def _pk(x):
    return pltpu.bitcast(x.astype(bf16), u32)


def _up(x):
    return pltpu.bitcast(x, bf16)


def _gelu(x):
    c = 0.7978845608028654
    t = jnp.tanh(x * (c + (c * 0.044715) * (x * x)))
    hx = 0.5 * x
    return hx + hx * t


def _ln(x):
    m = jnp.mean(x, axis=-1, keepdims=True)
    xc = x - m
    v = jnp.mean(xc * xc, axis=-1, keepdims=True)
    if RSQ:
        return xc * jnp.exp2(-0.5 * jnp.log2(v + 1e-5))
    return xc * lax.rsqrt(v + 1e-5)


def _recip(x):
    r = pl.reciprocal(x, approx=True)
    return r * (2.0 - x * r)


def _fold4(a, op):
    return op(a, pltpu.roll(a, 4, 0))


def _dual_exp(p):
    mx = _fold4(jnp.max(p, axis=0), jnp.maximum)
    mn = _fold4(jnp.min(p, axis=0), jnp.minimum)
    ep = jnp.exp2(p - mx[None])
    en = jnp.exp2(mn[None] - p)
    rp = _recip(_fold4(jnp.sum(ep, axis=0), jnp.add))
    rn = _recip(_fold4(jnp.sum(en, axis=0), jnp.add))
    return ep, en, rp, rn


def kernel_body(x_hbm, wqkv_hbm, wphi_hbm, wo_hbm, w1_hbm, w2_hbm, w3t_hbm, w4_hbm, gw_hbm,
           out_hbm,
           x_v, wq_v, wk_v, wv_v, wphi_v, wo_v, w1_v, w2_v, w3t_v, w4_v, gw_v, out_v,
           wt_ref, h_ref, kv_ref, z_ref, kvt_ref, phi_ref, p_ref, xn_ref, vt_ref,
           x1_ref, x1n_ref, u_ref, o_ref, g_ref, sem):
    def xcopy(a, b, k):
        return pltpu.make_async_copy(x_hbm.at[a:b], x_v.at[a:b], sem.at[k])

    c_phi = pltpu.make_async_copy(wphi_hbm, wphi_v, sem.at[0])
    c_wk = pltpu.make_async_copy(wqkv_hbm.at[:, D:2 * D], wk_v, sem.at[1])
    c_x0 = xcopy(0, T0, 2)
    c_wv = pltpu.make_async_copy(wqkv_hbm.at[:, 2 * D:3 * D], wv_v, sem.at[3])
    c_w1 = pltpu.make_async_copy(w1_hbm, w1_v, sem.at[4])
    c_x1 = xcopy(T0, T + AH, 3)
    g5 = [pltpu.make_async_copy(w2_hbm, w2_v, sem.at[5]), xcopy(T + AH, S, 5),
          pltpu.make_async_copy(wqkv_hbm.at[:, 0:D], wq_v, sem.at[5])]
    late = [pltpu.make_async_copy(w3t_hbm, w3t_v, sem.at[6]),
            pltpu.make_async_copy(w4_hbm, w4_v, sem.at[6]),
            pltpu.make_async_copy(wo_hbm, wo_v, sem.at[6]),
            pltpu.make_async_copy(gw_hbm, gw_v, sem.at[6])]
    c_phi.start()
    c_wk.start()

    x_v[S:S + AH, :] = jnp.zeros((AH, D), bf16)
    for n in range(4):
        h_ref[n, 0:PAD, :] = jnp.zeros((PAD, 128), f32)

    c_phi.wait()
    c_x0.start()
    c_x1.start()
    sel = (lax.broadcasted_iota(jnp.int32, (H, D), 0)
           == lax.broadcasted_iota(jnp.int32, (H, D), 1) // DH)
    sel = jnp.where(sel, 1.0, 0.0).astype(bf16)
    bm = jnp.dot(wphi_v[...], sel, preferred_element_type=f32)
    dmask = (lax.broadcasted_iota(jnp.int32, (DH * DH, D), 0) // DH
             == lax.broadcasted_iota(jnp.int32, (DH * DH, D), 1) % DH)
    cm = jnp.sum(jnp.where(dmask, bm, 0.0).reshape(DH, DH, D), axis=0).astype(bf16)
    e3 = ((lax.broadcasted_iota(jnp.int32, (128, DH), 0) % 64) // 4
          == lax.broadcasted_iota(jnp.int32, (128, DH), 1))
    e3 = jnp.where(e3, 1.0, 0.0).astype(bf16)
    pall = jnp.dot(e3, cm, preferred_element_type=f32)
    rr = lax.broadcasted_iota(jnp.int32, (128, D), 0)
    cc = lax.broadcasted_iota(jnp.int32, (128, D), 1)
    pmask = ((cc // DH) % 8) == ((rr // 64) * 4 + rr % 4)
    p_ref[...] = _pk(jnp.where(pmask, pall, 0.0))

    def fold(w_v, base):
        for g in range(4):
            wt = lax.dot_general(_up(p_ref[:, g * 128:(g + 1) * 128]), w_v[:, g * 128:(g + 1) * 128],
                                 NT_DIMS, preferred_element_type=f32)
            wt_ref[base // 2 + g * 64: base // 2 + (g + 1) * 64, :] = _pk(wt * LOG2E)

    def st_pk(r0, n, off=0, first=False):
        x = x_v[pl.ds(r0, n), :]
        pk = lax.dot_general(_up(wt_ref[D // 2:D, :]), x, NT_DIMS, preferred_element_type=f32)
        for c in range(n // 128):
            cs = slice(off + c * 128, off + (c + 1) * 128)
            for j in range(NJ):
                p = pk[j * 64:(j + 1) * 64, c * 128:(c + 1) * 128].reshape(8, 8, 128)
                ep, en, rp, rn = _dual_exp(p)
                ep = (ep * rp[None]).reshape(64, 128)
                en = (en * rn[None]).reshape(64, 128)
                if first and c == 0:
                    z_ref[j * 128:j * 128 + 64, :] = ep
                    z_ref[j * 128 + 64:(j + 1) * 128, :] = en
                else:
                    z_ref[j * 128:j * 128 + 64, :] += ep
                    z_ref[j * 128 + 64:(j + 1) * 128, :] += en
                phi_ref[j * 64:j * 64 + 32, cs] = _pk(ep)
                phi_ref[j * 64 + 32:(j + 1) * 64, cs] = _pk(en)

    def st_v(r0, n, off=0):
        x = x_v[pl.ds(r0, n), :]
        vt_ref[:, off:off + n] = _pk(lax.dot_general(_up(wt_ref[D:3 * D // 2, :]), x, NT_DIMS,
                                                     preferred_element_type=f32))

    def st_kv(first=False):
        for j in range(NJ):
            r = lax.dot_general(_up(vt_ref[j * 32:(j + 1) * 32, :]), _up(phi_ref[j * 64:(j + 1) * 64, 0:T]),
                                NT_DIMS, preferred_element_type=f32)
            if first:
                kv_ref[j * 64:(j + 1) * 64, :] = r
            else:
                kv_ref[j * 64:(j + 1) * 64, :] += r

    def st_ln1(r0, n, off=0, ch=LNC1):
        for r in range(0, n, ch):
            m = min(ch, n - r)
            xn_ref[(off + r) // 2:(off + r + m) // 2, :] = _pk(_ln(x_v[pl.ds(r0 + r, m), :].astype(f32)))

    def st_w1(r0, n, off=0):
        h = _gelu(jnp.dot(_up(xn_ref[off // 2:(off + n) // 2, :]), w1_v[...], preferred_element_type=f32))
        for q in range(4):
            h_ref[q, pl.ds(PAD + r0, n), :] = h[:, q * 128:(q + 1) * 128]

    def st_w2(r0):
        hs = jnp.concatenate(
            [h_ref[q, pl.ds(PAD + r0 + SHIFTS[q], T), :] for q in range(4)], axis=1).astype(bf16)
        x1_ref[pl.ds(r0, T), :] = (x_v[pl.ds(r0, T), :].astype(f32)
                                   + jnp.dot(hs, w2_v[...], preferred_element_type=f32))

    def st_ln2(r0, a, b):
        for r in range(a, b, LNC):
            x1n_ref[r // 2:(r + LNC) // 2, :] = _pk(_ln(x1_ref[pl.ds(r0 + r, LNC), :]))

    with scope("w_wk"):
        c_wk.wait()
    with scope("r_fold"):
        c_wv.start()
        c_w1.start()
        fold(wk_v, D)
    with scope("w_x0"):
        c_x0.wait()
    with scope("r_pk0"):
        for c in g5:
            c.start()
        st_pk(0, T0, first=True)
    with scope("w_wv"):
        c_x1.wait()
        c_wv.wait()
    with scope("r_v0"):
        for c in late:
            c.start()
        wt_ref[D:3 * D // 2, :] = _pk(wv_v[...].T)
        st_pk(T0, T - T0, off=T0)
        st_ln1(0, T + AH, ch=LNC0)
        st_v(0, T)
    with scope("w_w1"):
        c_w1.wait()
    with scope("r_5"):
        st_w1(0, T + AH)
        st_kv(True)
    with scope("w_g5"):
        for c in g5:
            c.wait()

    def finalize():
        r2 = lax.broadcasted_iota(jnp.int32, (D, 128), 0)
        c2 = lax.broadcasted_iota(jnp.int32, (D, 128), 1)
        kmask = ((r2 // DH) % 4) == (c2 % 4)
        kvt_ref[...] = _pk(jnp.where(kmask, kv_ref[...], 0.0))

    def finalize_z():
        z_ref[...] = jnp.broadcast_to(jnp.sum(z_ref[...], axis=1, keepdims=True), z_ref.shape)

    def run1(order, r0):
        for s in order:
            if s == 'pk': st_pk(r0, T)
            elif s == 'w2': st_w2(r0 - T)
            elif s == 'ln1': st_ln1(r0 + AH, T)
            elif s == 'v': st_v(r0, T)
            elif s == 'w1': st_w1(r0 + AH, T)
            elif s == 'kv': st_kv()
            elif s == 'w2l': st_w2(S - T)
            elif s == 'fq': fold(wq_v, 0)
            elif s == 'ln2': st_ln2(FIRST2 * T, 0, T)
            elif s == 'fin': finalize()
            elif s == 'finz': finalize_z()
            elif s == 'wait':
                for c in late:
                    c.wait()

    def p1(t, carry):
        with scope('p1body'):
            run1(P1ORD, pl.multiple_of(t * T, T))
        return carry

    if NLOOP1 > 1:
        lax.fori_loop(1, 1 + NLOOP1, p1, 0)
        t1 = 1 + NLOOP1
    else:
        t1 = 1
    for t in range(t1, NT - 1):
        run1(P1ORD, t * T)
    if t1 < NT:
        run1(P1LAST, (NT - 1) * T)
    else:
        with scope('mid'):
            run1(P1MID, 0)

    def st_pq(r0):
        x = x_v[pl.ds(r0, T2), :]
        pq = lax.dot_general(_up(wt_ref[0:D // 2, :]), x, NT_DIMS, preferred_element_type=f32)
        for c in range(T2 // 128):
            for j in range(NJ):
                zp = z_ref[j * 128:j * 128 + 64, :].reshape(8, 8, 128)
                zn = z_ref[j * 128 + 64:(j + 1) * 128, :].reshape(8, 8, 128)
                p = pq[j * 64:(j + 1) * 64, c * 128:(c + 1) * 128].reshape(8, 8, 128)
                ep, en, rp, rn = _dual_exp(p)
                den = jnp.sum(ep * zp, axis=0) * rp + jnp.sum(en * zn, axis=0) * rn
                rd = _recip(_fold4(den, jnp.add) + 1e-6)
                ep = (ep * (rp * rd)[None]).reshape(64, 128)
                en = (en * (rn * rd)[None]).reshape(64, 128)
                phi_ref[j * 64:j * 64 + 32, c * 128:(c + 1) * 128] = _pk(ep)
                phi_ref[j * 64 + 32:(j + 1) * 64, c * 128:(c + 1) * 128] = _pk(en)

    def p2(t, carry):
        r0 = pl.multiple_of(t * T2, T2)
        rn = pl.multiple_of(((t + 1) & (NT2 - 1)) * T2, T2)
        offs = [sum(SPL[:k]) for k in range(len(SPL))]
        bs = {}

        def gate_of(rk, n):
            gw = gw_v[...].astype(f32).reshape(1, D)
            gl = jnp.sum(x_v[pl.ds(rk, n), :].astype(f32) * gw, axis=-1, keepdims=True)
            return 0.5 * jnp.tanh(0.5 * gl) + 0.5

        for s in P2ORD:
            if s == 'pq':
                st_pq(r0)
            elif s[:3] == 'w3m':
                k = int(s[3:])
                rs = slice(k * HC // 2, (k + 1) * HC // 2)
                u_ref[rs, 0:FM] = _pk(_gelu(lax.dot_general(_up(x1n_ref[rs, :]), w3t_v[0:FM, :], NT_DIMS,
                                                            preferred_element_type=f32)))
            elif s[:3] == 'w3r':
                k = int(s[3:])
                rs = slice(k * HC // 2, (k + 1) * HC // 2)
                urt = _gelu(lax.dot_general(w3t_v[FM:F, :], _up(x1n_ref[rs, :]), NT_DIMS,
                                            preferred_element_type=f32))
                urt = jnp.concatenate([urt, jnp.zeros((128 - (F - FM), HC), f32)], axis=0)
                u_ref[rs, FM:F] = _pk(urt.T)[:, 0:F - FM]
            elif s == 'num':
                ots = [jnp.dot(_up(kvt_ref[j * 32:(j + 1) * 32, :]), _up(phi_ref[j * 64:(j + 1) * 64, :]),
                               preferred_element_type=f32) for j in range(NJ)]
                o_ref[...] = _pk(jnp.concatenate(ots, axis=0).T)
            elif s[:4] == 'ln2c':
                k = int(s[4:])
                st_ln2(r0, k * HC, (k + 1) * HC)
            elif s == 'ln2n':
                st_ln2(rn, 0, HC)
            elif s[:2] == 'w4':
                k = int(s[2:])
                off, n = offs[k], SPL[k]
                bs[k] = x1_ref[pl.ds(r0 + off, n), :] + jnp.dot(
                    _up(u_ref[off // 2:(off + n) // 2, :]), w4_v[...], preferred_element_type=f32)
            elif s[:2] == 'wo':
                k = int(s[2:])
                off, n = offs[k], SPL[k]
                rk = r0 + off
                a = jnp.dot(_up(o_ref[off // 2:(off + n) // 2, :]), wo_v[...], preferred_element_type=f32)
                gate = gate_of(rk, n)
                b = bs[k]
                out_v[pl.ds(rk, n), :] = (b + gate * (a - b)).astype(bf16)
                pltpu.make_async_copy(out_v.at[pl.ds(rk, n)], out_hbm.at[pl.ds(rk, n)], sem.at[7]).start()
        return carry

    def p2u(i, carry):
        with scope('p2body'):
            for k in range(U2):
                p2(i * U2 + k, carry)
        return carry

    lax.fori_loop(0, NT2, p2u, 0)
    with scope('w_out'):
        pltpu.make_async_copy(out_v, out_hbm, sem.at[7]).wait()


def kernel(*refs):
    cnt = refs[-1]
    cnt[0] = 1

    def step(i, c):
        kernel_body(*refs[:-1])
        return c

    lax.fori_loop(0, cnt[0], step, 0)


@jax.jit
def pallas_gated_mix__linear_kernel_hedgehog__mixer_s_mlp__prompt_kernel(
        A_x, A_wqkv, A_w_phi, A_wo, B_x, B_w1, B_w2, B_w3, B_w4, gate_w):
    x = A_x.reshape(S, D)
    wphi = jnp.transpose(A_w_phi, (1, 2, 0)).reshape(DH * DH, H)
    w3t = B_w3.T
    hbm = pl.BlockSpec(memory_space=pl.ANY)
    out = pl.pallas_call(
        kernel,
        out_shape=jax.ShapeDtypeStruct((S, D), bf16),
        in_specs=[hbm] * 9,
        out_specs=hbm,
        scratch_shapes=[
            pltpu.VMEM((S + AH, D), bf16),
            pltpu.VMEM((D, D), bf16),
            pltpu.VMEM((D, D), bf16),
            pltpu.VMEM((D, D), bf16),
            pltpu.VMEM((DH * DH, H), bf16),
            pltpu.VMEM((D, D), bf16),
            pltpu.VMEM((D, D), bf16),
            pltpu.VMEM((D, D), bf16),
            pltpu.VMEM((F, D), bf16),
            pltpu.VMEM((F, D), bf16),
            pltpu.VMEM((D,), bf16),
            pltpu.VMEM((S, D), bf16),
            pltpu.VMEM((3 * D // 2, D), u32),
            pltpu.VMEM((4, PAD + S + AH, 128), f32),
            pltpu.VMEM((D, 128), f32),
            pltpu.VMEM((NJ * 128, 128), f32),
            pltpu.VMEM((D // 2, 128), u32),
            pltpu.VMEM((NJ * 64, T2), u32),
            pltpu.VMEM((64, D), u32),
            pltpu.VMEM(((T + AH) // 2, D), u32),
            pltpu.VMEM((D // 2, T), u32),
            pltpu.VMEM((S, D), f32),
            pltpu.VMEM((T2 // 2, D), u32),
            pltpu.VMEM((T2 // 2, F), u32),
            pltpu.VMEM((T2 // 2, D), u32),
            pltpu.VMEM((T, 128), f32),
            pltpu.SemaphoreType.DMA((8,)),
            pltpu.SMEM((1,), jnp.int32),
        ],
        compiler_params=pltpu.CompilerParams(vmem_limit_bytes=100 * 1024 * 1024),
    )(x, A_wqkv, wphi, A_wo, B_w1, B_w2, w3t, B_w4, gate_w)
    return out.reshape(1, S, D)
```

```python
import jax
import jax.numpy as jnp
from jax import lax
import jax.experimental.pallas as pl
import jax.experimental.pallas.tpu as pltpu

S, D, H, DH, F = 2048, 512, 32, 16, 1376
NJ = 8
T0 = 256
P0 = 512
T1 = int(768)
N1 = (S - P0) // T1
R2 = 512
T2 = 1024
NT2 = S // T2
HC = 512
FM = 1280
AH = 16
PAD = 8
SPL = [int(v) for v in '384,384,128,96,32'.split(',')]
P1ORD = 'w2,pk,ln1,v,w1,kv'.split(',')
MID = 'fin,finz,w2l,ln2,fq'.split(',')
MIDLN = int(1024)
P2ORD = 'w3r0,w3r1,pq,w3m0,w3m1,num,ln2n0,w40,wo0,ln2n1,w41,wo1,w42,wo2,w43,wo3,w44,wo4'.split(',')
LNC = int(16)
LNC1 = int(16)
LNC0 = int(32)
SC = int(0)
LOG2E = 1.4426950408889634
NT_DIMS = (((1,), (1,)), ((), ()))
SHIFTS = (-1, 1, -2, 2)
f32 = jnp.float32
bf16 = jnp.bfloat16
u32 = jnp.uint32


class _Null:
    def __enter__(self):
        return None

    def __exit__(self, *a):
        return False


def scope(name):
    return jax.named_scope(name) if SC else _Null()


def _pk(x):
    return pltpu.bitcast(x.astype(bf16), u32)


def _up(x):
    return pltpu.bitcast(x, bf16)


def _gelu(x):
    c = 0.7978845608028654
    t = jnp.tanh(x * (c + (c * 0.044715) * (x * x)))
    hx = 0.5 * x
    return hx + hx * t


def _ln(x):
    m = jnp.mean(x, axis=-1, keepdims=True)
    xc = x - m
    v = jnp.mean(xc * xc, axis=-1, keepdims=True)
    return xc * jnp.exp2((-0.5 * LOG2E) * jnp.log(v + 1e-5))


def _recip(x):
    r = pl.reciprocal(x, approx=True)
    return r * (2.0 - x * r)


def _fold4(a, op):
    return op(a, pltpu.roll(a, 4, 0))


def _dual_exp(p):
    mx = _fold4(jnp.max(p, axis=0), jnp.maximum)
    mn = _fold4(jnp.min(p, axis=0), jnp.minimum)
    ep = jnp.exp2(p - mx[None])
    en = jnp.exp2(mn[None] - p)
    rp = _recip(_fold4(jnp.sum(ep, axis=0), jnp.add))
    rn = _recip(_fold4(jnp.sum(en, axis=0), jnp.add))
    return ep, en, rp, rn


def kernel_body(x_hbm, wqkv_hbm, wphi_hbm, wo_hbm, w1_hbm, w2_hbm, w3t_hbm, w4_hbm, gw_hbm,
                out_hbm,
                x_v, wq_v, wk_v, wv_v, wphi_v, wo_v, w1_v, w2_v, w3t_v, w4_v, gw_v, out_v,
                wt_ref, h_ref, kv_ref, z_ref, kvt_ref, phi_ref, p_ref, xn_ref, vt_ref,
                x1_ref, x1n_ref, u_ref, o_ref, sem):
    def xcopy(a, b, k):
        return pltpu.make_async_copy(x_hbm.at[a:b], x_v.at[a:b], sem.at[k])

    c_phi = pltpu.make_async_copy(wphi_hbm, wphi_v, sem.at[0])
    c_wk = pltpu.make_async_copy(wqkv_hbm.at[:, D:2 * D], wk_v, sem.at[1])
    c_x0 = xcopy(0, T0, 2)
    c_x1 = xcopy(T0, P0 + AH, 3)
    c_wv = pltpu.make_async_copy(wqkv_hbm.at[:, 2 * D:3 * D], wv_v, sem.at[3])
    c_w1 = pltpu.make_async_copy(w1_hbm, w1_v, sem.at[4])
    g5 = [pltpu.make_async_copy(w2_hbm, w2_v, sem.at[5]), xcopy(P0 + AH, S, 5)]
    late = [pltpu.make_async_copy(wqkv_hbm.at[:, 0:D], wq_v, sem.at[6]),
            pltpu.make_async_copy(w3t_hbm, w3t_v, sem.at[6]),
            pltpu.make_async_copy(w4_hbm, w4_v, sem.at[6]),
            pltpu.make_async_copy(wo_hbm, wo_v, sem.at[6]),
            pltpu.make_async_copy(gw_hbm, gw_v, sem.at[6])]
    c_phi.start()
    c_wk.start()

    x_v[S:S + AH, :] = jnp.zeros((AH, D), bf16)
    for n in range(4):
        h_ref[n, 0:PAD, :] = jnp.zeros((PAD, 128), f32)

    c_phi.wait()
    c_x0.start()
    c_x1.start()
    sel = (lax.broadcasted_iota(jnp.int32, (H, D), 0)
           == lax.broadcasted_iota(jnp.int32, (H, D), 1) // DH)
    sel = jnp.where(sel, 1.0, 0.0).astype(bf16)
    bm = jnp.dot(wphi_v[...], sel, preferred_element_type=f32)
    dmask = (lax.broadcasted_iota(jnp.int32, (DH * DH, D), 0) // DH
             == lax.broadcasted_iota(jnp.int32, (DH * DH, D), 1) % DH)
    cm = jnp.sum(jnp.where(dmask, bm, 0.0).reshape(DH, DH, D), axis=0).astype(bf16)
    e3 = ((lax.broadcasted_iota(jnp.int32, (128, DH), 0) % 64) // 4
          == lax.broadcasted_iota(jnp.int32, (128, DH), 1))
    e3 = jnp.where(e3, 1.0, 0.0).astype(bf16)
    pall = jnp.dot(e3, cm, preferred_element_type=f32)
    rr = lax.broadcasted_iota(jnp.int32, (128, D), 0)
    cc = lax.broadcasted_iota(jnp.int32, (128, D), 1)
    pmask = ((cc // DH) % 8) == ((rr // 64) * 4 + rr % 4)
    p_ref[...] = _pk(jnp.where(pmask, pall, 0.0))

    def fold(w_v, base):
        for g in range(4):
            wt = lax.dot_general(_up(p_ref[:, g * 128:(g + 1) * 128]), w_v[:, g * 128:(g + 1) * 128],
                                 NT_DIMS, preferred_element_type=f32)
            wt_ref[base // 2 + g * 64: base // 2 + (g + 1) * 64, :] = _pk(wt * LOG2E)

    def st_pk(r0, n, off=0, first=False):
        x = x_v[pl.ds(r0, n), :]
        pk = lax.dot_general(_up(wt_ref[D // 2:D, :]), x, NT_DIMS, preferred_element_type=f32)
        for c in range(n // 128):
            cs = slice(off + c * 128, off + (c + 1) * 128)
            for j in range(NJ):
                p = pk[j * 64:(j + 1) * 64, c * 128:(c + 1) * 128].reshape(8, 8, 128)
                ep, en, rp, rn = _dual_exp(p)
                ep = (ep * rp[None]).reshape(64, 128)
                en = (en * rn[None]).reshape(64, 128)
                if first and c == 0:
                    z_ref[j * 128:j * 128 + 64, :] = ep
                    z_ref[j * 128 + 64:(j + 1) * 128, :] = en
                else:
                    z_ref[j * 128:j * 128 + 64, :] += ep
                    z_ref[j * 128 + 64:(j + 1) * 128, :] += en
                phi_ref[j * 64:j * 64 + 32, cs] = _pk(ep)
                phi_ref[j * 64 + 32:(j + 1) * 64, cs] = _pk(en)

    def st_v(r0, n):
        x = x_v[pl.ds(r0, n), :]
        vt_ref[:, 0:n] = _pk(lax.dot_general(_up(wt_ref[D:3 * D // 2, :]), x, NT_DIMS,
                                             preferred_element_type=f32))

    def st_kv(n, first=False):
        for j in range(NJ):
            r = lax.dot_general(_up(vt_ref[j * 32:(j + 1) * 32, 0:n]), _up(phi_ref[j * 64:(j + 1) * 64, 0:n]),
                                NT_DIMS, preferred_element_type=f32)
            if first:
                kv_ref[j * 64:(j + 1) * 64, :] = r
            else:
                kv_ref[j * 64:(j + 1) * 64, :] += r

    def st_ln1(r0, n, ch):
        for r in range(0, n, ch):
            m = min(ch, n - r)
            xn_ref[r // 2:(r + m) // 2, :] = _pk(_ln(x_v[pl.ds(r0 + r, m), :].astype(f32)))

    def st_w1(r0, n):
        h = _gelu(jnp.dot(_up(xn_ref[0:n // 2, :]), w1_v[...], preferred_element_type=f32))
        for q in range(4):
            h_ref[q, pl.ds(PAD + r0, n), :] = h[:, q * 128:(q + 1) * 128]

    def st_w2(r0, n):
        hs = jnp.concatenate(
            [h_ref[q, pl.ds(PAD + r0 + SHIFTS[q], n), :] for q in range(4)], axis=1).astype(bf16)
        x1_ref[pl.ds(r0, n), :] = (x_v[pl.ds(r0, n), :].astype(f32)
                                   + jnp.dot(hs, w2_v[...], preferred_element_type=f32))

    def st_ln2(r0, a, b):
        for r in range(a, b, LNC):
            x1n_ref[r // 2:(r + LNC) // 2, :] = _pk(_ln(x1_ref[pl.ds(r0 + r, LNC), :]))

    with scope("w_wk"):
        c_wk.wait()
    with scope("r_fold"):
        c_wv.start()
        c_w1.start()
        fold(wk_v, D)
    with scope("w_x0"):
        c_x0.wait()
    with scope("r_pk0"):
        for c in g5:
            c.start()
        st_pk(0, T0, first=True)
    with scope("w_wv"):
        c_x1.wait()
        c_wv.wait()
    with scope("r_v0"):
        for c in late:
            c.start()
        wt_ref[D:3 * D // 2, :] = _pk(wv_v[...].T)
        st_pk(T0, P0 - T0, off=T0)
        st_ln1(0, P0 + AH, LNC0)
        st_v(0, P0)
    with scope("w_w1"):
        c_w1.wait()
    with scope("r_5"):
        st_w1(0, P0 + AH)
        st_kv(P0, True)
    with scope("w_g5"):
        for c in g5:
            c.wait()

    def p1(i, carry):
        r0 = pl.multiple_of(P0 + i * T1, 256)
        with scope('p1body'):
            for s in P1ORD:
                if s == 'pk': st_pk(r0, T1)
                elif s == 'w2': st_w2(pl.multiple_of(i * R2, R2), R2)
                elif s == 'ln1': st_ln1(r0 + AH, T1, LNC1)
                elif s == 'v': st_v(r0, T1)
                elif s == 'w1': st_w1(r0 + AH, T1)
                elif s == 'kv': st_kv(T1)
        return carry

    lax.fori_loop(0, N1, p1, 0)

    with scope('mid'):
        for c in late:
            c.wait()
        for s in MID:
            if s == 'w2l':
                for r in range(N1 * R2, S, 512):
                    st_w2(r, 512)
            elif s == 'fq': fold(wq_v, 0)
            elif s == 'ln2': st_ln2(0, 0, MIDLN)
            elif s == 'fin':
                r2 = lax.broadcasted_iota(jnp.int32, (D, 128), 0)
                c2 = lax.broadcasted_iota(jnp.int32, (D, 128), 1)
                kmask = ((r2 // DH) % 4) == (c2 % 4)
                kvt_ref[...] = _pk(jnp.where(kmask, kv_ref[...], 0.0))
            elif s == 'finz':
                z_ref[...] = jnp.broadcast_to(jnp.sum(z_ref[...], axis=1, keepdims=True), z_ref.shape)

    def st_pq(r0):
        x = x_v[pl.ds(r0, T2), :]
        pq = lax.dot_general(_up(wt_ref[0:D // 2, :]), x, NT_DIMS, preferred_element_type=f32)
        for c in range(T2 // 128):
            for j in range(NJ):
                zp = z_ref[j * 128:j * 128 + 64, :].reshape(8, 8, 128)
                zn = z_ref[j * 128 + 64:(j + 1) * 128, :].reshape(8, 8, 128)
                p = pq[j * 64:(j + 1) * 64, c * 128:(c + 1) * 128].reshape(8, 8, 128)
                ep, en, rp, rn = _dual_exp(p)
                den = jnp.sum(ep * zp, axis=0) * rp + jnp.sum(en * zn, axis=0) * rn
                rd = _recip(_fold4(den, jnp.add) + 1e-6)
                ep = (ep * (rp * rd)[None]).reshape(64, 128)
                en = (en * (rn * rd)[None]).reshape(64, 128)
                phi_ref[j * 64:j * 64 + 32, c * 128:(c + 1) * 128] = _pk(ep)
                phi_ref[j * 64 + 32:(j + 1) * 64, c * 128:(c + 1) * 128] = _pk(en)

    def p2(t, carry):
        r0 = pl.multiple_of(t * T2, T2)
        rn = pl.multiple_of(((t + 1) & (NT2 - 1)) * T2, T2)
        offs = [sum(SPL[:k]) for k in range(len(SPL))]
        bs = {}

        def gate_of(rk, n):
            gw = gw_v[...].astype(f32).reshape(1, D)
            gl = jnp.sum(x_v[pl.ds(rk, n), :].astype(f32) * gw, axis=-1, keepdims=True)
            return 0.5 * jnp.tanh(0.5 * gl) + 0.5

        with scope('p2body'):
            for s in P2ORD:
                if s == 'pq':
                    st_pq(r0)
                elif s[:3] == 'w3m':
                    k = int(s[3:])
                    rs = slice(k * HC // 2, (k + 1) * HC // 2)
                    u_ref[rs, 0:FM] = _pk(_gelu(lax.dot_general(
                        _up(x1n_ref[rs, :]), w3t_v[0:FM, :], NT_DIMS, preferred_element_type=f32)))
                elif s[:3] == 'w3r':
                    k = int(s[3:])
                    rs = slice(k * HC // 2, (k + 1) * HC // 2)
                    urt = _gelu(lax.dot_general(w3t_v[FM:F, :], _up(x1n_ref[rs, :]), NT_DIMS,
                                                preferred_element_type=f32))
                    urt = jnp.concatenate([urt, jnp.zeros((128 - (F - FM), HC), f32)], axis=0)
                    u_ref[rs, FM:F] = _pk(urt.T)[:, 0:F - FM]
                elif s == 'num':
                    ots = [jnp.dot(_up(kvt_ref[j * 32:(j + 1) * 32, :]), _up(phi_ref[j * 64:(j + 1) * 64, 0:T2]),
                                   preferred_element_type=f32) for j in range(NJ)]
                    o_ref[...] = _pk(jnp.concatenate(ots, axis=0).T)
                elif s[:4] == 'ln2c':
                    k = int(s[4:])
                    st_ln2(r0, k * HC, (k + 1) * HC)
                elif s[:4] == 'ln2n':
                    k = int(s[4:])
                    st_ln2(rn, k * HC, (k + 1) * HC)
                elif s[:4] == 'ln2q':
                    k = int(s[4:])
                    st_ln2(rn, k * 256, (k + 1) * 256)
                elif s[:2] == 'w4':
                    k = int(s[2:])
                    off, n = offs[k], SPL[k]
                    bs[k] = x1_ref[pl.ds(r0 + off, n), :] + jnp.dot(
                        _up(u_ref[off // 2:(off + n) // 2, :]), w4_v[...], preferred_element_type=f32)
                elif s[:2] == 'wo':
                    k = int(s[2:])
                    off, n = offs[k], SPL[k]
                    rk = r0 + off
                    a = jnp.dot(_up(o_ref[off // 2:(off + n) // 2, :]), wo_v[...], preferred_element_type=f32)
                    gate = gate_of(rk, n)
                    b = bs[k]
                    out_v[pl.ds(rk, n), :] = (b + gate * (a - b)).astype(bf16)
                    pltpu.make_async_copy(out_v.at[pl.ds(rk, n)], out_hbm.at[pl.ds(rk, n)], sem.at[7]).start()
        return carry

    lax.fori_loop(0, NT2, p2, 0)
    with scope('w_out'):
        pltpu.make_async_copy(out_v, out_hbm, sem.at[7]).wait()


def kernel(*refs):
    cnt = refs[-1]
    cnt[0] = 1

    def step(i, c):
        kernel_body(*refs[:-1])
        return c

    lax.fori_loop(0, cnt[0], step, 0)


@jax.jit
def pallas_gated_mix__linear_kernel_hedgehog__mixer_s_mlp__prompt_kernel(
        A_x, A_wqkv, A_w_phi, A_wo, B_x, B_w1, B_w2, B_w3, B_w4, gate_w):
    x = A_x.reshape(S, D)
    wphi = jnp.transpose(A_w_phi, (1, 2, 0)).reshape(DH * DH, H)
    w3t = B_w3.T
    hbm = pl.BlockSpec(memory_space=pl.ANY)
    TM = max(T1, P0 + AH)
    out = pl.pallas_call(
        kernel,
        out_shape=jax.ShapeDtypeStruct((S, D), bf16),
        in_specs=[hbm] * 9,
        out_specs=hbm,
        scratch_shapes=[
            pltpu.VMEM((S + AH, D), bf16),
            pltpu.VMEM((D, D), bf16),
            pltpu.VMEM((D, D), bf16),
            pltpu.VMEM((D, D), bf16),
            pltpu.VMEM((DH * DH, H), bf16),
            pltpu.VMEM((D, D), bf16),
            pltpu.VMEM((D, D), bf16),
            pltpu.VMEM((D, D), bf16),
            pltpu.VMEM((F, D), bf16),
            pltpu.VMEM((F, D), bf16),
            pltpu.VMEM((D,), bf16),
            pltpu.VMEM((S, D), bf16),
            pltpu.VMEM((3 * D // 2, D), u32),
            pltpu.VMEM((4, PAD + S + AH, 128), f32),
            pltpu.VMEM((D, 128), f32),
            pltpu.VMEM((NJ * 128, 128), f32),
            pltpu.VMEM((D // 2, 128), u32),
            pltpu.VMEM((NJ * 64, max(T1, T2)), u32),
            pltpu.VMEM((64, D), u32),
            pltpu.VMEM((TM // 2, D), u32),
            pltpu.VMEM((D // 2, max(T1, P0)), u32),
            pltpu.VMEM((S, D), f32),
            pltpu.VMEM((T2 // 2, D), u32),
            pltpu.VMEM((T2 // 2, F), u32),
            pltpu.VMEM((T2 // 2, D), u32),
            pltpu.SemaphoreType.DMA((8,)),
            pltpu.SMEM((1,), jnp.int32),
        ],
        compiler_params=pltpu.CompilerParams(vmem_limit_bytes=100 * 1024 * 1024),
    )(x, A_wqkv, wphi, A_wo, B_w1, B_w2, w3t, B_w4, gate_w)
    return out.reshape(1, S, D)
```

```python
import jax
import jax.numpy as jnp
from jax import lax
import jax.experimental.pallas as pl
import jax.experimental.pallas.tpu as pltpu

S, D, H, DH, F = 2048, 512, 32, 16, 1376
NJ = 8
T0 = 256
P0 = 512
T1 = int(768)
N1 = (S - P0) // T1
R2 = 512
T2 = 1024
NT2 = S // T2
HC = 512
FM = 1280
MQ = 480
AH = 16
PAD = 8
SPL = [int(v) for v in '384,384,128,96,32'.split(',')]
SPL4 = [int(v) for v in '384,384,128,96,32'.split(',')]
P1ORD = 'w2,pk,ln1,v,w1,kv'.split(',')
MID = 'w2a,fq,finz,ln2,fin,w2b'.split(',')
MIDLN = int(1024)
P2ORD = 'w3r0,w3r1,pq,w3m0,w3m1,num,ln2n0,w40,wo0,ln2n1,w41,wo1,w42,wo2,w43,wo3,w44,wo4'.split(',')
LNC = int(16)
LNC1 = int(16)
LNC0 = int(32)
SC = int(0)
LOG2E = 1.4426950408889634
NT_DIMS = (((1,), (1,)), ((), ()))
SHIFTS = (-1, 1, -2, 2)
f32 = jnp.float32
bf16 = jnp.bfloat16
u32 = jnp.uint32


class _Null:
    def __enter__(self):
        return None

    def __exit__(self, *a):
        return False


def scope(name):
    return jax.named_scope(name) if SC else _Null()


def _pk(x):
    return pltpu.bitcast(x.astype(bf16), u32)


def _up(x):
    return pltpu.bitcast(x, bf16)


def _gelu(x):
    c = 0.7978845608028654
    t = jnp.tanh(x * (c + (c * 0.044715) * (x * x)))
    hx = 0.5 * x
    return hx + hx * t


def _ln(x):
    m = jnp.mean(x, axis=-1, keepdims=True)
    xc = x - m
    v = jnp.mean(xc * xc, axis=-1, keepdims=True)
    return xc * jnp.exp2((-0.5 * LOG2E) * jnp.log(v + 1e-5))


def _recip(x):
    r = pl.reciprocal(x, approx=True)
    return r * (2.0 - x * r)


def _fold4(a, op):
    return op(a, pltpu.roll(a, 4, 0))


def _dual_exp(p):
    mx = _fold4(jnp.max(p, axis=0), jnp.maximum)
    mn = _fold4(jnp.min(p, axis=0), jnp.minimum)
    ep = jnp.exp2(p - mx[None])
    en = jnp.exp2(mn[None] - p)
    rp = _recip(_fold4(jnp.sum(ep, axis=0), jnp.add))
    rn = _recip(_fold4(jnp.sum(en, axis=0), jnp.add))
    return ep, en, rp, rn


def kernel_body(x_hbm, wqkv_hbm, wphi_hbm, wo_hbm, w1_hbm, w2_hbm, w3t_hbm, w4_hbm, gw_hbm,
                out_hbm,
                x_v, wq_v, wk_v, wv_v, wphi_v, wo_v, w1_v, w2_v, w3t_v, w4_v, gw_v, out_v,
                wt_ref, h_ref, kv_ref, z_ref, kvt_ref, phi_ref, p_ref, xn_ref, vt_ref,
                x1_ref, x1n_ref, u_ref, o_ref, sem):
    def xcopy(a, b, k):
        return pltpu.make_async_copy(x_hbm.at[a:b], x_v.at[a:b], sem.at[k])

    c_phi = pltpu.make_async_copy(wphi_hbm, wphi_v, sem.at[0])
    c_wk = pltpu.make_async_copy(wqkv_hbm.at[:, D:2 * D], wk_v, sem.at[1])
    c_x0 = xcopy(0, T0, 2)
    c_x1 = xcopy(T0, P0 + AH, 3)
    c_wv = pltpu.make_async_copy(wqkv_hbm.at[:, 2 * D:3 * D], wv_v, sem.at[3])
    c_w1 = pltpu.make_async_copy(w1_hbm, w1_v, sem.at[4])
    g5 = [pltpu.make_async_copy(w2_hbm, w2_v, sem.at[5]), xcopy(P0 + AH, S, 5)]
    late = [pltpu.make_async_copy(wqkv_hbm.at[:, 0:D], wq_v, sem.at[6]),
            pltpu.make_async_copy(w3t_hbm, w3t_v, sem.at[6]),
            pltpu.make_async_copy(w4_hbm, w4_v, sem.at[6]),
            pltpu.make_async_copy(wo_hbm, wo_v, sem.at[6]),
            pltpu.make_async_copy(gw_hbm, gw_v, sem.at[6])]
    c_phi.start()
    c_wk.start()

    x_v[S:S + AH, :] = jnp.zeros((AH, D), bf16)
    for n in range(4):
        h_ref[n, 0:PAD, :] = jnp.zeros((PAD, 128), f32)

    c_phi.wait()
    c_x0.start()
    c_x1.start()
    sel = (lax.broadcasted_iota(jnp.int32, (H, D), 0)
           == lax.broadcasted_iota(jnp.int32, (H, D), 1) // DH)
    sel = jnp.where(sel, 1.0, 0.0).astype(bf16)
    bm = jnp.dot(wphi_v[...], sel, preferred_element_type=f32)
    dmask = (lax.broadcasted_iota(jnp.int32, (DH * DH, D), 0) // DH
             == lax.broadcasted_iota(jnp.int32, (DH * DH, D), 1) % DH)
    cm = jnp.sum(jnp.where(dmask, bm, 0.0).reshape(DH, DH, D), axis=0).astype(bf16)
    e3 = ((lax.broadcasted_iota(jnp.int32, (128, DH), 0) % 64) // 4
          == lax.broadcasted_iota(jnp.int32, (128, DH), 1))
    e3 = jnp.where(e3, 1.0, 0.0).astype(bf16)
    pall = jnp.dot(e3, cm, preferred_element_type=f32)
    rr = lax.broadcasted_iota(jnp.int32, (128, D), 0)
    cc = lax.broadcasted_iota(jnp.int32, (128, D), 1)
    pmask = ((cc // DH) % 8) == ((rr // 64) * 4 + rr % 4)
    p_ref[...] = _pk(jnp.where(pmask, pall, 0.0))

    def fold(w_v, base):
        lo = lax.broadcasted_iota(jnp.int32, (8, D), 0) < 4
        for gp in range(2):
            rows = []
            for g in (2 * gp, 2 * gp + 1):
                wt = lax.dot_general(_up(p_ref[:, g * 128:(g + 1) * 128]), w_v[:, g * 128:(g + 1) * 128],
                                     NT_DIMS, preferred_element_type=f32)
                ds = []
                for jj in range(2):
                    a = wt[jj * 64:(jj + 1) * 64, :].reshape(8, 8, D)
                    ref = jnp.where(lo, pltpu.roll(a[7], 4, 0), a[7])
                    ds.append((a - ref[None]) * LOG2E)
                shared = jnp.where(lo, ds[0][7], pltpu.roll(ds[1][7], 4, 0))
                rows += [ds[0][0:7].reshape(56, D), shared, ds[1][0:7].reshape(56, D)]
            wt_ref[base + gp * 120: base + (gp + 1) * 120, :] = _pk(jnp.concatenate(rows, axis=0))

    def logits(pm, j, c):
        lo = lax.broadcasted_iota(jnp.int32, (8, 128), 0) < 4
        g, jj = j // 2, j % 2
        cs = slice(c * 128, (c + 1) * 128)
        own = pm[g * 120 + jj * 64:g * 120 + jj * 64 + 56, cs].reshape(7, 8, 128)
        sh = pm[g * 120 + 56:g * 120 + 64, cs]
        last = jnp.where(lo, sh, 0.0) if jj == 0 else jnp.where(lo, 0.0, sh)
        return jnp.concatenate([own, last[None]], axis=0)

    def st_pk(r0, n, off=0, first=False):
        x = x_v[pl.ds(r0, n), :]
        pk = lax.dot_general(_up(wt_ref[MQ // 2:MQ, :]), x, NT_DIMS, preferred_element_type=f32)
        for c in range(n // 128):
            cs = slice(off + c * 128, off + (c + 1) * 128)
            for j in range(NJ):
                p = logits(pk, j, c)
                ep, en, rp, rn = _dual_exp(p)
                ep = (ep * rp[None]).reshape(64, 128)
                en = (en * rn[None]).reshape(64, 128)
                if first and c == 0:
                    z_ref[j * 128:j * 128 + 64, :] = ep
                    z_ref[j * 128 + 64:(j + 1) * 128, :] = en
                else:
                    z_ref[j * 128:j * 128 + 64, :] += ep
                    z_ref[j * 128 + 64:(j + 1) * 128, :] += en
                phi_ref[j * 64:j * 64 + 32, cs] = _pk(ep)
                phi_ref[j * 64 + 32:(j + 1) * 64, cs] = _pk(en)

    def st_v(r0, n):
        x = x_v[pl.ds(r0, n), :]
        vt_ref[:, 0:n] = _pk(lax.dot_general(_up(wt_ref[MQ:MQ + D // 2, :]), x, NT_DIMS,
                                             preferred_element_type=f32))

    def st_kv(n, first=False):
        for j in range(NJ):
            r = lax.dot_general(_up(vt_ref[j * 32:(j + 1) * 32, 0:n]), _up(phi_ref[j * 64:(j + 1) * 64, 0:n]),
                                NT_DIMS, preferred_element_type=f32)
            if first:
                kv_ref[j * 64:(j + 1) * 64, :] = r
            else:
                kv_ref[j * 64:(j + 1) * 64, :] += r

    def st_ln1(r0, n, ch):
        for r in range(0, n, ch):
            m = min(ch, n - r)
            xn_ref[r // 2:(r + m) // 2, :] = _pk(_ln(x_v[pl.ds(r0 + r, m), :].astype(f32)))

    def st_w1(r0, n):
        h = _gelu(jnp.dot(_up(xn_ref[0:n // 2, :]), w1_v[...], preferred_element_type=f32))
        for q in range(4):
            h_ref[q, pl.ds(PAD + r0, n), :] = h[:, q * 128:(q + 1) * 128]

    def st_w2(r0, n):
        hs = jnp.concatenate(
            [h_ref[q, pl.ds(PAD + r0 + SHIFTS[q], n), :] for q in range(4)], axis=1).astype(bf16)
        x1_ref[pl.ds(r0, n), :] = (x_v[pl.ds(r0, n), :].astype(f32)
                                   + jnp.dot(hs, w2_v[...], preferred_element_type=f32))

    def st_ln2(r0, a, b):
        for r in range(a, b, LNC):
            x1n_ref[r // 2:(r + LNC) // 2, :] = _pk(_ln(x1_ref[pl.ds(r0 + r, LNC), :]))

    with scope("w_wk"):
        c_wk.wait()
    with scope("r_fold"):
        c_wv.start()
        c_w1.start()
        fold(wk_v, MQ // 2)
    with scope("w_x0"):
        c_x0.wait()
    with scope("r_pk0"):
        for c in g5:
            c.start()
        st_pk(0, T0, first=True)
    with scope("w_wv"):
        c_x1.wait()
        c_wv.wait()
    with scope("r_v0"):
        for c in late:
            c.start()
        wt_ref[MQ:MQ + D // 2, :] = _pk(wv_v[...].T)
        st_pk(T0, P0 - T0, off=T0)
        st_ln1(0, P0 + AH, LNC0)
        st_v(0, P0)
    with scope("w_w1"):
        c_w1.wait()
    with scope("r_5"):
        st_w1(0, P0 + AH)
        st_kv(P0, True)
    with scope("w_g5"):
        for c in g5:
            c.wait()

    def p1(i, carry):
        r0 = pl.multiple_of(P0 + i * T1, 256)
        with scope('p1body'):
            for s in P1ORD:
                if s == 'pk': st_pk(r0, T1)
                elif s == 'w2': st_w2(pl.multiple_of(i * R2, R2), R2)
                elif s == 'ln1': st_ln1(r0 + AH, T1, LNC1)
                elif s == 'v': st_v(r0, T1)
                elif s == 'w1': st_w1(r0 + AH, T1)
                elif s == 'kv': st_kv(T1)
                elif s == 'ln2':
                    rb = pl.multiple_of(i * R2, R2)
                    rh = pl.multiple_of(i * (R2 // 2), R2 // 2)
                    for r in range(0, R2, LNC):
                        x1n_ref[pl.ds(rh + r // 2, LNC // 2), :] = _pk(_ln(x1_ref[pl.ds(rb + r, LNC), :]))
        return carry

    lax.fori_loop(0, N1, p1, 0)

    with scope('mid'):
        for c in late:
            c.wait()
        for s in MID:
            if s == 'w2l':
                for r in range(N1 * R2, S, 512):
                    st_w2(r, 512)
            elif s == 'w2a': st_w2(N1 * R2, 512)
            elif s == 'w2b': st_w2(N1 * R2 + 512, 512)
            elif s == 'fq': fold(wq_v, 0)
            elif s == 'ln2': st_ln2(0, 0, MIDLN)
            elif s == 'fin':
                lane4 = lax.broadcasted_iota(jnp.int32, (DH, 128), 1) & 3
                for h in range(H):
                    kvt_ref[h * 8:(h + 1) * 8, :] = _pk(
                        jnp.where(lane4 == (h % 4), kv_ref[h * DH:(h + 1) * DH, :], 0.0))
            elif s == 'finz':
                z_ref[...] = jnp.broadcast_to(jnp.sum(z_ref[...], axis=1, keepdims=True), z_ref.shape)

    def st_pq(r0):
        x = x_v[pl.ds(r0, T2), :]
        pq = lax.dot_general(_up(wt_ref[0:MQ // 2, :]), x, NT_DIMS, preferred_element_type=f32)
        for c in range(T2 // 128):
            for j in range(NJ):
                zp = z_ref[j * 128:j * 128 + 64, :].reshape(8, 8, 128)
                zn = z_ref[j * 128 + 64:(j + 1) * 128, :].reshape(8, 8, 128)
                p = logits(pq, j, c)
                ep, en, rp, rn = _dual_exp(p)
                den = jnp.sum(ep * zp, axis=0) * rp + jnp.sum(en * zn, axis=0) * rn
                rd = _recip(_fold4(den, jnp.add) + 1e-6)
                ep = (ep * (rp * rd)[None]).reshape(64, 128)
                en = (en * (rn * rd)[None]).reshape(64, 128)
                phi_ref[j * 64:j * 64 + 32, c * 128:(c + 1) * 128] = _pk(ep)
                phi_ref[j * 64 + 32:(j + 1) * 64, c * 128:(c + 1) * 128] = _pk(en)

    def p2(t, carry):
        r0 = pl.multiple_of(t * T2, T2)
        rn = pl.multiple_of(((t + 1) & (NT2 - 1)) * T2, T2)
        offs = [sum(SPL[:k]) for k in range(len(SPL))]
        offs4 = [sum(SPL4[:k]) for k in range(len(SPL4))]
        bs = {}

        def gate_of(rk, n):
            gw = gw_v[...].astype(f32).reshape(1, D)
            gl = jnp.sum(x_v[pl.ds(rk, n), :].astype(f32) * gw, axis=-1, keepdims=True)
            return 0.5 * jnp.tanh(0.5 * gl) + 0.5

        with scope('p2body'):
            for s in P2ORD:
                if s == 'pq':
                    st_pq(r0)
                elif s[:3] == 'w3m':
                    k = int(s[3:])
                    rs = slice(k * HC // 2, (k + 1) * HC // 2)
                    u_ref[rs, 0:FM] = _pk(_gelu(lax.dot_general(
                        _up(x1n_ref[rs, :]), w3t_v[0:FM, :], NT_DIMS, preferred_element_type=f32)))
                elif s[:3] == 'w3r':
                    k = int(s[3:])
                    rs = slice(k * HC // 2, (k + 1) * HC // 2)
                    urt = _gelu(lax.dot_general(w3t_v[FM:F, :], _up(x1n_ref[rs, :]), NT_DIMS,
                                                preferred_element_type=f32))
                    urt = jnp.concatenate([urt, jnp.zeros((128 - (F - FM), HC), f32)], axis=0)
                    u_ref[rs, FM:F] = _pk(urt.T)[:, 0:F - FM]
                elif s == 'num':
                    ots = [jnp.dot(_up(kvt_ref[j * 32:(j + 1) * 32, :]), _up(phi_ref[j * 64:(j + 1) * 64, 0:T2]),
                                   preferred_element_type=f32) for j in range(NJ)]
                    o_ref[...] = _pk(jnp.concatenate(ots, axis=0).T)
                elif s[:4] == 'ln2c':
                    k = int(s[4:])
                    st_ln2(r0, k * HC, (k + 1) * HC)
                elif s[:4] == 'ln2n':
                    k = int(s[4:])
                    st_ln2(rn, k * HC, (k + 1) * HC)
                elif s[:4] == 'ln2q':
                    k = int(s[4:])
                    st_ln2(rn, k * 256, (k + 1) * 256)
                elif s[:2] == 'w4':
                    k = int(s[2:])
                    off, n = offs4[k], SPL4[k]
                    bs[k] = x1_ref[pl.ds(r0 + off, n), :] + jnp.dot(
                        _up(u_ref[off // 2:(off + n) // 2, :]), w4_v[...], preferred_element_type=f32)
                elif s[:2] == 'wo':
                    k = int(s[2:])
                    off, n = offs[k], SPL[k]
                    rk = r0 + off
                    a = jnp.dot(_up(o_ref[off // 2:(off + n) // 2, :]), wo_v[...], preferred_element_type=f32)
                    gate = gate_of(rk, n)
                    k4 = max(i for i in range(len(SPL4)) if offs4[i] <= off)
                    b = bs[k4][off - offs4[k4]:off - offs4[k4] + n]
                    out_v[pl.ds(rk, n), :] = (b + gate * (a - b)).astype(bf16)
                    pltpu.make_async_copy(out_v.at[pl.ds(rk, n)], out_hbm.at[pl.ds(rk, n)], sem.at[7]).start()
        return carry

    lax.fori_loop(0, NT2, p2, 0)
    with scope('w_out'):
        pltpu.make_async_copy(out_v, out_hbm, sem.at[7]).wait()


def kernel(*refs):
    cnt = refs[-1]
    cnt[0] = 1

    def step(i, c):
        kernel_body(*refs[:-1])
        return c

    lax.fori_loop(0, cnt[0], step, 0)


@jax.jit
def pallas_gated_mix__linear_kernel_hedgehog__mixer_s_mlp__prompt_kernel(
        A_x, A_wqkv, A_w_phi, A_wo, B_x, B_w1, B_w2, B_w3, B_w4, gate_w):
    x = A_x.reshape(S, D)
    wphi = jnp.transpose(A_w_phi, (1, 2, 0)).reshape(DH * DH, H)
    w3t = B_w3.T
    hbm = pl.BlockSpec(memory_space=pl.ANY)
    TM = max(T1, P0 + AH)
    out = pl.pallas_call(
        kernel,
        out_shape=jax.ShapeDtypeStruct((S, D), bf16),
        in_specs=[hbm] * 9,
        out_specs=hbm,
        scratch_shapes=[
            pltpu.VMEM((S + AH, D), bf16),
            pltpu.VMEM((D, D), bf16),
            pltpu.VMEM((D, D), bf16),
            pltpu.VMEM((D, D), bf16),
            pltpu.VMEM((DH * DH, H), bf16),
            pltpu.VMEM((D, D), bf16),
            pltpu.VMEM((D, D), bf16),
            pltpu.VMEM((D, D), bf16),
            pltpu.VMEM((F, D), bf16),
            pltpu.VMEM((F, D), bf16),
            pltpu.VMEM((D,), bf16),
            pltpu.VMEM((S, D), bf16),
            pltpu.VMEM((MQ + D // 2, D), u32),
            pltpu.VMEM((4, PAD + S + AH, 128), f32),
            pltpu.VMEM((D, 128), f32),
            pltpu.VMEM((NJ * 128, 128), f32),
            pltpu.VMEM((D // 2, 128), u32),
            pltpu.VMEM((NJ * 64, max(T1, T2)), u32),
            pltpu.VMEM((64, D), u32),
            pltpu.VMEM((TM // 2, D), u32),
            pltpu.VMEM((D // 2, max(T1, P0)), u32),
            pltpu.VMEM((S, D), f32),
            pltpu.VMEM((T2 // 2, D), u32),
            pltpu.VMEM((T2 // 2, F), u32),
            pltpu.VMEM((T2 // 2, D), u32),
            pltpu.SemaphoreType.DMA((8,)),
            pltpu.SMEM((1,), jnp.int32),
        ],
        compiler_params=pltpu.CompilerParams(vmem_limit_bytes=100 * 1024 * 1024),
    )(x, A_wqkv, wphi, A_wo, B_w1, B_w2, w3t, B_w4, gate_w)
    return out.reshape(1, S, D)
```

```python
import jax
import jax.numpy as jnp
from jax import lax
import jax.experimental.pallas as pl
import jax.experimental.pallas.tpu as pltpu

S, D, H, DH, F = 2048, 512, 32, 16, 1376
NJ = 8
MQ = 480
T0 = 256
P0 = 512
T1 = 768
N1 = (S - P0) // T1
R2 = 512
T2 = 1024
NT2 = S // T2
HC = 512
FM = 1280
AH = 16
PAD = 8
OUT_CHUNKS = (384, 384, 128, 96, 32)
LN_ROWS = 16
LOG2E = 1.4426950408889634
NT_DIMS = (((1,), (1,)), ((), ()))
SHIFTS = (-1, 1, -2, 2)
f32 = jnp.float32
bf16 = jnp.bfloat16
u32 = jnp.uint32


def _pk(x):
    return pltpu.bitcast(x.astype(bf16), u32)


def _up(x):
    return pltpu.bitcast(x, bf16)


def _dot(a, b):
    return jnp.dot(a, b, preferred_element_type=f32)


def _dot_nt(a, b):
    return lax.dot_general(a, b, NT_DIMS, preferred_element_type=f32)


def _gelu(x):
    c = 0.7978845608028654
    t = jnp.tanh(x * (c + (c * 0.044715) * (x * x)))
    hx = 0.5 * x
    return hx + hx * t


def _ln(x):
    m = jnp.mean(x, axis=-1, keepdims=True)
    xc = x - m
    v = jnp.mean(xc * xc, axis=-1, keepdims=True)
    return xc * jnp.exp2((-0.5 * LOG2E) * jnp.log(v + 1e-5))


def _recip(x):
    r = pl.reciprocal(x, approx=True)
    return r * (2.0 - x * r)


def _fold4(a, op):
    return op(a, pltpu.roll(a, 4, 0))


def _dual_exp(p):
    mx = _fold4(jnp.max(p, axis=0), jnp.maximum)
    mn = _fold4(jnp.min(p, axis=0), jnp.minimum)
    ep = jnp.exp2(p - mx[None])
    en = jnp.exp2(mn[None] - p)
    rp = _recip(_fold4(jnp.sum(ep, axis=0), jnp.add))
    rn = _recip(_fold4(jnp.sum(en, axis=0), jnp.add))
    return ep, en, rp, rn


def _logits(pm, j, c):
    lo = lax.broadcasted_iota(jnp.int32, (8, 128), 0) < 4
    g, jj = j // 2, j % 2
    cs = slice(c * 128, (c + 1) * 128)
    own = pm[g * 120 + jj * 64:g * 120 + jj * 64 + 56, cs].reshape(7, 8, 128)
    sh = pm[g * 120 + 56:g * 120 + 64, cs]
    last = jnp.where(lo, sh, 0.0) if jj == 0 else jnp.where(lo, 0.0, sh)
    return jnp.concatenate([own, last[None]], axis=0)


def _body(x_hbm, wqkv_hbm, wphi_hbm, wo_hbm, w1_hbm, w2_hbm, w3t_hbm, w4_hbm, gw_hbm,
          out_hbm,
          x_v, wq_v, wk_v, wv_v, wphi_v, wo_v, w1_v, w2_v, w3t_v, w4_v, gw_v, out_v,
          wt_ref, h_ref, kv_ref, z_ref, kvt_ref, phi_ref, p_ref, xn_ref, vt_ref,
          x1_ref, x1n_ref, u_ref, o_ref, sem):
    def copy(src, dst, k):
        return pltpu.make_async_copy(src, dst, sem.at[k])

    def xcopy(a, b, k):
        return copy(x_hbm.at[a:b], x_v.at[a:b], k)

    c_phi = copy(wphi_hbm, wphi_v, 0)
    c_wk = copy(wqkv_hbm.at[:, D:2 * D], wk_v, 1)
    c_x0 = xcopy(0, T0, 2)
    c_x1 = xcopy(T0, P0 + AH, 3)
    c_wv = copy(wqkv_hbm.at[:, 2 * D:3 * D], wv_v, 3)
    c_w1 = copy(w1_hbm, w1_v, 1)
    c_loop1 = [copy(w2_hbm, w2_v, 2), xcopy(P0 + AH, S, 2)]
    c_late = [copy(wqkv_hbm.at[:, 0:D], wq_v, 3), copy(w3t_hbm, w3t_v, 3), copy(w4_hbm, w4_v, 3),
              copy(wo_hbm, wo_v, 3), copy(gw_hbm, gw_v, 3)]
    c_phi.start()
    c_wk.start()

    x_v[S:S + AH, :] = jnp.zeros((AH, D), bf16)
    for q in range(4):
        h_ref[q, 0:PAD, :] = jnp.zeros((PAD, 128), f32)

    c_phi.wait()
    c_x0.start()
    c_x1.start()
    sel = (lax.broadcasted_iota(jnp.int32, (H, D), 0)
           == lax.broadcasted_iota(jnp.int32, (H, D), 1) // DH)
    bm = _dot(wphi_v[...], jnp.where(sel, 1.0, 0.0).astype(bf16))
    dmask = (lax.broadcasted_iota(jnp.int32, (DH * DH, D), 0) // DH
             == lax.broadcasted_iota(jnp.int32, (DH * DH, D), 1) % DH)
    cm = jnp.sum(jnp.where(dmask, bm, 0.0).reshape(DH, DH, D), axis=0).astype(bf16)
    e3 = ((lax.broadcasted_iota(jnp.int32, (128, DH), 0) % 64) // 4
          == lax.broadcasted_iota(jnp.int32, (128, DH), 1))
    pall = _dot(jnp.where(e3, 1.0, 0.0).astype(bf16), cm)
    rr = lax.broadcasted_iota(jnp.int32, (128, D), 0)
    cc = lax.broadcasted_iota(jnp.int32, (128, D), 1)
    pmask = ((cc // DH) % 8) == ((rr // 64) * 4 + rr % 4)
    p_ref[...] = _pk(jnp.where(pmask, pall, 0.0))

    def fold(w_v, base):
        lo = lax.broadcasted_iota(jnp.int32, (8, D), 0) < 4
        for gp in range(2):
            rows = []
            for g in (2 * gp, 2 * gp + 1):
                gs = slice(g * 128, (g + 1) * 128)
                wt = _dot_nt(_up(p_ref[:, gs]), w_v[:, gs])
                ds = []
                for jj in range(2):
                    a = wt[jj * 64:(jj + 1) * 64, :].reshape(8, 8, D)
                    f15 = jnp.where(lo, pltpu.roll(a[7], 4, 0), a[7])
                    ds.append((a - f15[None]) * LOG2E)
                f14 = jnp.where(lo, ds[0][7], pltpu.roll(ds[1][7], 4, 0))
                rows += [ds[0][0:7].reshape(56, D), f14, ds[1][0:7].reshape(56, D)]
            wt_ref[base + gp * 120:base + (gp + 1) * 120, :] = _pk(jnp.concatenate(rows, axis=0))

    def phi_k(r0, n, off=0, first=False):
        pk = _dot_nt(_up(wt_ref[MQ // 2:MQ, :]), x_v[pl.ds(r0, n), :])
        for c in range(n // 128):
            cs = slice(off + c * 128, off + (c + 1) * 128)
            for j in range(NJ):
                ep, en, rp, rn = _dual_exp(_logits(pk, j, c))
                ep = (ep * rp[None]).reshape(64, 128)
                en = (en * rn[None]).reshape(64, 128)
                if first and c == 0:
                    z_ref[j * 128:j * 128 + 64, :] = ep
                    z_ref[j * 128 + 64:(j + 1) * 128, :] = en
                else:
                    z_ref[j * 128:j * 128 + 64, :] += ep
                    z_ref[j * 128 + 64:(j + 1) * 128, :] += en
                phi_ref[j * 64:j * 64 + 32, cs] = _pk(ep)
                phi_ref[j * 64 + 32:(j + 1) * 64, cs] = _pk(en)

    def v_proj(r0, n):
        vt_ref[:, 0:n] = _pk(_dot_nt(_up(wt_ref[MQ:MQ + D // 2, :]), x_v[pl.ds(r0, n), :]))

    def kv_acc(n, first=False):
        for j in range(NJ):
            r = _dot_nt(_up(vt_ref[j * 32:(j + 1) * 32, 0:n]), _up(phi_ref[j * 64:(j + 1) * 64, 0:n]))
            if first:
                kv_ref[j * 64:(j + 1) * 64, :] = r
            else:
                kv_ref[j * 64:(j + 1) * 64, :] += r

    def ln1(r0, n, ch):
        for r in range(0, n, ch):
            m = min(ch, n - r)
            xn_ref[r // 2:(r + m) // 2, :] = _pk(_ln(x_v[pl.ds(r0 + r, m), :].astype(f32)))

    def mix_in(r0, n):
        h = _gelu(_dot(_up(xn_ref[0:n // 2, :]), w1_v[...]))
        for q in range(4):
            h_ref[q, pl.ds(PAD + r0, n), :] = h[:, q * 128:(q + 1) * 128]

    def mix_out(r0, n):
        hs = jnp.concatenate(
            [h_ref[q, pl.ds(PAD + r0 + SHIFTS[q], n), :] for q in range(4)], axis=1).astype(bf16)
        x1_ref[pl.ds(r0, n), :] = x_v[pl.ds(r0, n), :].astype(f32) + _dot(hs, w2_v[...])

    def ln2(r0, a, b):
        for r in range(a, b, LN_ROWS):
            x1n_ref[r // 2:(r + LN_ROWS) // 2, :] = _pk(_ln(x1_ref[pl.ds(r0 + r, LN_ROWS), :]))

    c_wk.wait()
    c_wv.start()
    c_w1.start()
    fold(wk_v, MQ // 2)
    c_x0.wait()
    for c in c_loop1:
        c.start()
    phi_k(0, T0, first=True)
    c_x1.wait()
    c_wv.wait()
    for c in c_late:
        c.start()
    wt_ref[MQ:MQ + D // 2, :] = _pk(wv_v[...].T)
    phi_k(T0, P0 - T0, off=T0)
    ln1(0, P0 + AH, 2 * LN_ROWS)
    v_proj(0, P0)
    c_w1.wait()
    mix_in(0, P0 + AH)
    kv_acc(P0, first=True)
    for c in c_loop1:
        c.wait()

    def phase1(i, carry):
        r0 = pl.multiple_of(P0 + i * T1, 256)
        mix_out(pl.multiple_of(i * R2, R2), R2)
        phi_k(r0, T1)
        ln1(r0 + AH, T1, LN_ROWS)
        v_proj(r0, T1)
        mix_in(r0 + AH, T1)
        kv_acc(T1)
        return carry

    lax.fori_loop(0, N1, phase1, 0)

    for c in c_late:
        c.wait()
    mix_out(N1 * R2, R2)
    fold(wq_v, 0)
    z_ref[...] = jnp.broadcast_to(jnp.sum(z_ref[...], axis=1, keepdims=True), z_ref.shape)
    ln2(0, 0, T2)
    lane4 = lax.broadcasted_iota(jnp.int32, (DH, 128), 1) & 3
    for h in range(H):
        kvt_ref[h * 8:(h + 1) * 8, :] = _pk(
            jnp.where(lane4 == (h % 4), kv_ref[h * DH:(h + 1) * DH, :], 0.0))
    mix_out((N1 + 1) * R2, R2)

    def phi_q(r0):
        pq = _dot_nt(_up(wt_ref[0:MQ // 2, :]), x_v[pl.ds(r0, T2), :])
        for c in range(T2 // 128):
            cs = slice(c * 128, (c + 1) * 128)
            for j in range(NJ):
                zp = z_ref[j * 128:j * 128 + 64, :].reshape(8, 8, 128)
                zn = z_ref[j * 128 + 64:(j + 1) * 128, :].reshape(8, 8, 128)
                ep, en, rp, rn = _dual_exp(_logits(pq, j, c))
                den = jnp.sum(ep * zp, axis=0) * rp + jnp.sum(en * zn, axis=0) * rn
                rd = _recip(_fold4(den, jnp.add) + 1e-6)
                phi_ref[j * 64:j * 64 + 32, cs] = _pk((ep * (rp * rd)[None]).reshape(64, 128))
                phi_ref[j * 64 + 32:(j + 1) * 64, cs] = _pk((en * (rn * rd)[None]).reshape(64, 128))

    def mlp_in_tail(k):
        rs = slice(k * HC // 2, (k + 1) * HC // 2)
        ut = _gelu(_dot_nt(w3t_v[FM:F, :], _up(x1n_ref[rs, :])))
        ut = jnp.concatenate([ut, jnp.zeros((128 - (F - FM), HC), f32)], axis=0)
        u_ref[rs, FM:F] = _pk(ut.T)[:, 0:F - FM]

    def mlp_in(k):
        rs = slice(k * HC // 2, (k + 1) * HC // 2)
        u_ref[rs, 0:FM] = _pk(_gelu(_dot_nt(_up(x1n_ref[rs, :]), w3t_v[0:FM, :])))

    def phase2(t, carry):
        r0 = pl.multiple_of(t * T2, T2)
        r_next = pl.multiple_of(((t + 1) & (NT2 - 1)) * T2, T2)
        mlp_in_tail(0)
        mlp_in_tail(1)
        phi_q(r0)
        mlp_in(0)
        mlp_in(1)
        ot = [_dot(_up(kvt_ref[j * 32:(j + 1) * 32, :]), _up(phi_ref[j * 64:(j + 1) * 64, :]))
              for j in range(NJ)]
        o_ref[...] = _pk(jnp.concatenate(ot, axis=0).T)
        off = 0
        for k, n in enumerate(OUT_CHUNKS):
            if k < T2 // HC:
                ln2(r_next, k * HC, (k + 1) * HC)
            rows = pl.ds(r0 + off, n)
            hs = slice(off // 2, (off + n) // 2)
            b = x1_ref[rows, :] + _dot(_up(u_ref[hs, :]), w4_v[...])
            a = _dot(_up(o_ref[hs, :]), wo_v[...])
            gw = gw_v[...].astype(f32).reshape(1, D)
            gl = jnp.sum(x_v[rows, :].astype(f32) * gw, axis=-1, keepdims=True)
            gate = 0.5 * jnp.tanh(0.5 * gl) + 0.5
            out_v[rows, :] = (b + gate * (a - b)).astype(bf16)
            copy(out_v.at[rows], out_hbm.at[rows], 0).start()
            off += n
        return carry

    lax.fori_loop(0, NT2, phase2, 0)
    copy(out_v, out_hbm, 0).wait()


def _kernel(*refs):
    trips = refs[-1]
    trips[0] = 1

    def once(i, carry):
        _body(*refs[:-1])
        return carry

    lax.fori_loop(0, trips[0], once, 0)


@jax.jit
def pallas_gated_mix__linear_kernel_hedgehog__mixer_s_mlp__prompt_kernel(
        A_x, A_wqkv, A_w_phi, A_wo, B_x, B_w1, B_w2, B_w3, B_w4, gate_w):
    del B_x
    x = A_x.reshape(S, D)
    wphi = jnp.transpose(A_w_phi, (1, 2, 0)).reshape(DH * DH, H)
    w3t = B_w3.T
    hbm = pl.BlockSpec(memory_space=pl.ANY)
    out = pl.pallas_call(
        _kernel,
        out_shape=jax.ShapeDtypeStruct((S, D), bf16),
        in_specs=[hbm] * 9,
        out_specs=hbm,
        scratch_shapes=[
            pltpu.VMEM((S + AH, D), bf16),
            pltpu.VMEM((D, D), bf16),
            pltpu.VMEM((D, D), bf16),
            pltpu.VMEM((D, D), bf16),
            pltpu.VMEM((DH * DH, H), bf16),
            pltpu.VMEM((D, D), bf16),
            pltpu.VMEM((D, D), bf16),
            pltpu.VMEM((D, D), bf16),
            pltpu.VMEM((F, D), bf16),
            pltpu.VMEM((F, D), bf16),
            pltpu.VMEM((D,), bf16),
            pltpu.VMEM((S, D), bf16),
            pltpu.VMEM((MQ + D // 2, D), u32),
            pltpu.VMEM((4, PAD + S + AH, 128), f32),
            pltpu.VMEM((D, 128), f32),
            pltpu.VMEM((NJ * 128, 128), f32),
            pltpu.VMEM((D // 2, 128), u32),
            pltpu.VMEM((NJ * 64, T2), u32),
            pltpu.VMEM((64, D), u32),
            pltpu.VMEM((T1 // 2, D), u32),
            pltpu.VMEM((D // 2, T1), u32),
            pltpu.VMEM((S, D), f32),
            pltpu.VMEM((T2 // 2, D), u32),
            pltpu.VMEM((T2 // 2, F), u32),
            pltpu.VMEM((T2 // 2, D), u32),
            pltpu.SemaphoreType.DMA((4,)),
            pltpu.SMEM((1,), jnp.int32),
        ],
        compiler_params=pltpu.CompilerParams(vmem_limit_bytes=100 * 1024 * 1024),
    )(x, A_wqkv, wphi, A_wo, B_w1, B_w2, w3t, B_w4, gate_w)
    return out.reshape(1, S, D)
```

```python
import jax
import jax.numpy as jnp
from jax import lax
import jax.experimental.pallas as pl
import jax.experimental.pallas.tpu as pltpu

S, D, H, DH, F = 2048, 512, 32, 16, 1376
NJ = 8
MQ = 480
T0 = 256
P0 = 512
T1 = 768
N1 = (S - P0) // T1
R2 = 512
T2 = 1024
NT2 = S // T2
HC = 512
FM = 1280
AH = 32
PAD = 8
OUT_CHUNKS = tuple(int(v) for v in '192,192,96,32'.split(','))
KH = D // 2
LHS_TERMS = ((0, 3, 1), (2, 3, 1), (0, None, 1), (3, None, 1), (0, 1, 1), (2, 0, -1), (1, 3, -1))
W2ORD = [int(v) for v in '1,3,0,2,4,5,6'.split(',')]
AC = int(512)
WOC = int(256)
LNPOS = int(0)
RHS_TERMS = ((0, 3, 1), (1, 3, -1), (2, 0, -1), (0, 1, 1), (2, 3, 1))
WC = int(16)
AR = int(16)
FH = FM // 2
FQ = FH // 2
HH = HC // 2
NB = int(128)
WPRE = int(0)
LN_ROWS = 16
LOG2E = 1.4426950408889634
NT_DIMS = (((1,), (1,)), ((), ()))
SHIFTS = (-1, 1, -2, 2)
f32 = jnp.float32
bf16 = jnp.bfloat16
u32 = jnp.uint32


def _pk(x):
    return pltpu.bitcast(x.astype(bf16), u32)


def _up(x):
    return pltpu.bitcast(x, bf16)


def _dot(a, b):
    return jnp.dot(a, b, preferred_element_type=f32)


def _dot_nt(a, b):
    return lax.dot_general(a, b, NT_DIMS, preferred_element_type=f32)


def _gelu(x):
    c = 0.7978845608028654
    t = jnp.tanh(x * (c + (c * 0.044715) * (x * x)))
    hx = 0.5 * x
    return hx + hx * t


def _ln(x):
    m = jnp.mean(x, axis=-1, keepdims=True)
    xc = x - m
    v = jnp.mean(xc * xc, axis=-1, keepdims=True)
    return xc * jnp.exp2((-0.5 * LOG2E) * jnp.log(v + 1e-5))


def _recip(x):
    r = pl.reciprocal(x, approx=True)
    return r * (2.0 - x * r)


def _fold4(a, op):
    return op(a, pltpu.roll(a, 4, 0))


def _dual_exp(p):
    mx = _fold4(jnp.max(p, axis=0), jnp.maximum)
    mn = _fold4(jnp.min(p, axis=0), jnp.minimum)
    ep = jnp.exp2(p - mx[None])
    en = jnp.exp2(mn[None] - p)
    rp = _recip(_fold4(jnp.sum(ep, axis=0), jnp.add))
    rn = _recip(_fold4(jnp.sum(en, axis=0), jnp.add))
    return ep, en, rp, rn


def _lhs_sums(a11, a12, a21, a22):
    return (a11 + a22, a21 + a22, a11 + a12, a21 - a11, a12 - a22)


def _rhs_sums(b11, b12, b21, b22):
    b11, b12, b21, b22 = (b.astype(f32) for b in (b11, b12, b21, b22))
    return (b11 + b22, b12 - b22, b21 - b11, b11 + b12, b21 + b22)


def _quadrants(m1, m2, m3, m4, m5, m6, m7):
    return m1 + m4 - m5 + m7, m3 + m5, m2 + m4, m1 - m2 + m3 + m6


def _logits(pm, j, c):
    lo = lax.broadcasted_iota(jnp.int32, (8, 128), 0) < 4
    g, jj = j // 2, j % 2
    cs = slice(c * 128, (c + 1) * 128)
    own = pm[g * 120 + jj * 64:g * 120 + jj * 64 + 56, cs].reshape(7, 8, 128)
    sh = pm[g * 120 + 56:g * 120 + 64, cs]
    last = jnp.where(lo, sh, 0.0) if jj == 0 else jnp.where(lo, 0.0, sh)
    return jnp.concatenate([own, last[None]], axis=0)


def _body(zero, x_hbm, wqkv_hbm, wphi_hbm, wo_hbm, w1_hbm, w2_hbm, w3t_hbm, w4_hbm, gw_hbm,
          out_hbm,
          x_v, wq_v, wk_v, wv_v, wphi_v, wo_v, w1_v, w2_v, w3t_v, w4_v, gw_v, out_v,
          wt_ref, h_ref, kv_ref, z_ref, kvt_ref, phi_ref, p_ref, xn_ref, vt_ref,
          x1_ref, sa_ref, big_ref, ur_ref, t4_ref, o_ref, acc_ref, g_ref, sem):
    def copy(src, dst, k):
        return pltpu.make_async_copy(src, dst, sem.at[k])

    def xcopy(a, b, k):
        return copy(x_hbm.at[a:b], x_v.at[a:b], k)

    c_phi = copy(wphi_hbm, wphi_v, 0)
    c_wk = copy(wqkv_hbm.at[:, D:2 * D], wk_v, 1)
    c_x0 = xcopy(0, T0, 2)
    c_x1 = xcopy(T0, P0 + AH, 3)
    c_wv = copy(wqkv_hbm.at[:, 2 * D:3 * D], wv_v, 3)
    c_w1 = copy(w1_hbm, w1_v, 1)
    c_loop1 = [copy(w2_hbm, w2_v, 2), xcopy(P0 + AH, S, 2)]
    c_late = [copy(wqkv_hbm.at[:, 0:D], wq_v, 3), copy(w3t_hbm, w3t_v, 3), copy(w4_hbm, w4_v, 3),
              copy(wo_hbm, wo_v, 3), copy(gw_hbm, gw_v, 3)]
    c_phi.start()
    c_wk.start()

    x_v[S:S + AH, :] = jnp.zeros((AH, D), bf16)
    for q in range(4):
        h_ref[q, 0:PAD, :] = jnp.zeros((PAD, 128), f32)

    c_phi.wait()
    c_x0.start()
    c_x1.start()
    sel = (lax.broadcasted_iota(jnp.int32, (H, D), 0)
           == lax.broadcasted_iota(jnp.int32, (H, D), 1) // DH)
    bm = _dot(wphi_v[...], jnp.where(sel, 1.0, 0.0).astype(bf16))
    dmask = (lax.broadcasted_iota(jnp.int32, (DH * DH, D), 0) // DH
             == lax.broadcasted_iota(jnp.int32, (DH * DH, D), 1) % DH)
    cm = jnp.sum(jnp.where(dmask, bm, 0.0).reshape(DH, DH, D), axis=0).astype(bf16)
    e3 = ((lax.broadcasted_iota(jnp.int32, (128, DH), 0) % 64) // 4
          == lax.broadcasted_iota(jnp.int32, (128, DH), 1))
    pall = _dot(jnp.where(e3, 1.0, 0.0).astype(bf16), cm)
    rr = lax.broadcasted_iota(jnp.int32, (128, D), 0)
    cc = lax.broadcasted_iota(jnp.int32, (128, D), 1)
    pmask = ((cc // DH) % 8) == ((rr // 64) * 4 + rr % 4)
    p_ref[...] = _pk(jnp.where(pmask, pall, 0.0))

    def fold(w_v, base):
        lo = lax.broadcasted_iota(jnp.int32, (8, D), 0) < 4
        for gp in range(2):
            rows = []
            for g in (2 * gp, 2 * gp + 1):
                gs = slice(g * 128, (g + 1) * 128)
                wt = _dot_nt(_up(p_ref[:, gs]), w_v[:, gs])
                ds = []
                for jj in range(2):
                    a = wt[jj * 64:(jj + 1) * 64, :].reshape(8, 8, D)
                    f15 = jnp.where(lo, pltpu.roll(a[7], 4, 0), a[7])
                    ds.append((a - f15[None]) * LOG2E)
                f14 = jnp.where(lo, ds[0][7], pltpu.roll(ds[1][7], 4, 0))
                rows += [ds[0][0:7].reshape(56, D), f14, ds[1][0:7].reshape(56, D)]
            wt_ref[base + gp * 120:base + (gp + 1) * 120, :] = _pk(jnp.concatenate(rows, axis=0))

    def phi_k(r0, n, off=0, first=False):
        pk = _dot_nt(_up(wt_ref[MQ // 2:MQ, :]), x_v[pl.ds(r0, n), :])
        for c in range(n // 128):
            cs = slice(off + c * 128, off + (c + 1) * 128)
            for j in range(NJ):
                ep, en, rp, rn = _dual_exp(_logits(pk, j, c))
                ep = (ep * rp[None]).reshape(64, 128)
                en = (en * rn[None]).reshape(64, 128)
                if first and c == 0:
                    z_ref[j * 128:j * 128 + 64, :] = ep
                    z_ref[j * 128 + 64:(j + 1) * 128, :] = en
                else:
                    z_ref[j * 128:j * 128 + 64, :] += ep
                    z_ref[j * 128 + 64:(j + 1) * 128, :] += en
                phi_ref[j * 64:j * 64 + 32, cs] = _pk(ep)
                phi_ref[j * 64 + 32:(j + 1) * 64, cs] = _pk(en)

    def v_proj(r0, n):
        vt_ref[:, 0:n] = _pk(_dot_nt(_up(wt_ref[MQ:MQ + D // 2, :]), x_v[pl.ds(r0, n), :]))

    def kv_acc(n, first=False):
        for j in range(NJ):
            r = _dot_nt(_up(vt_ref[j * 32:(j + 1) * 32, 0:n]), _up(phi_ref[j * 64:(j + 1) * 64, 0:n]))
            if first:
                kv_ref[j * 64:(j + 1) * 64, :] = r
            else:
                kv_ref[j * 64:(j + 1) * 64, :] += r

    def ln1(r0, n, ch):
        for r in range(0, n, ch):
            m = min(ch, n - r)
            xn_ref[r:r + m, :] = _ln(x_v[pl.ds(r0 + r, m), :].astype(f32))

    def sq_rhs(w_v, i):
        blk = lambda t: w_v[(t // 2) * KH:(t // 2 + 1) * KH, (t % 2) * KH:(t % 2 + 1) * KH]
        ti = (0, None, 1, 2, None, 3, 4)[i]
        if ti is None:
            return blk(0) if i == 1 else blk(3)
        p, q, sign = RHS_TERMS[ti]
        bp, bq = blk(p).astype(f32), blk(q).astype(f32)
        return (bp + bq if sign > 0 else bp - bq).astype(bf16)

    def sq_strassen(blk, w_v):
        ms = [None] * 7
        for i in W2ORD:
            p, q, sign = LHS_TERMS[i]
            lhs = blk(p) if q is None else (blk(p) + blk(q) if sign > 0 else blk(p) - blk(q))
            ms[i] = _dot(lhs.astype(bf16), sq_rhs(w_v, i))
        return _quadrants(*ms)

    def mix_in(r0, n):
        m = n // 2
        blk = lambda t: xn_ref[(t // 2) * m:(t // 2 + 1) * m, (t % 2) * KH:(t % 2 + 1) * KH]
        for t, c in enumerate(sq_strassen(blk, w1_v)):
            h = _gelu(c)
            for q in range(2):
                h_ref[2 * (t % 2) + q, pl.ds(PAD + r0 + (t // 2) * m, m), :] = h[:, q * 128:(q + 1) * 128]

    def mix_out(r0, n):
        m = n // 2

        def blk(t):
            return jnp.concatenate(
                [h_ref[q, pl.ds(PAD + r0 + (t // 2) * m + SHIFTS[q], m), :]
                 for q in (2 * (t % 2), 2 * (t % 2) + 1)], axis=1)

        c11, c12, c21, c22 = sq_strassen(blk, w2_v)
        for half, cc in enumerate(((c11, c12), (c21, c22))):
            rows = pl.ds(r0 + half * m, m)
            x1_ref[rows, :] = x_v[rows, :].astype(f32) + jnp.concatenate(cc, axis=1)

    def ln2(r0, a, b):
        for r in range(a, b, LN_ROWS):
            ya = _ln(x1_ref[pl.ds(r0 + r, LN_ROWS), :])
            yb = _ln(x1_ref[pl.ds(r0 + HC + r, LN_ROWS), :])
            quads = (ya[:, :KH], ya[:, KH:], yb[:, :KH], yb[:, KH:])
            for i, s in enumerate(quads + _lhs_sums(*quads)):
                sa_ref[i * HH + r // 2:i * HH + (r + LN_ROWS) // 2, :] = _pk(s)

    def w4_sum(i):
        p, q, sign = RHS_TERMS[i]
        for k0 in range(0, FH, WC):
            blk = lambda t: w4_v[(t // 2) * FH + k0:(t // 2) * FH + k0 + WC,
                                 (t % 2) * KH:(t % 2 + 1) * KH].astype(f32)
            s = blk(p) + blk(q) if sign > 0 else blk(p) - blk(q)
            t4_ref[i * FQ + k0 // 2:i * FQ + (k0 + WC) // 2, :] = _pk(s)

    c_wk.wait()
    c_wv.start()
    c_w1.start()
    fold(wk_v, MQ // 2)
    c_x0.wait()
    for c in c_loop1:
        c.start()
    phi_k(0, T0, first=True)
    c_x1.wait()
    c_wv.wait()
    for c in c_late:
        c.start()
    wt_ref[MQ:MQ + D // 2, :] = _pk(wv_v[...].T)
    phi_k(T0, P0 - T0, off=T0)
    ln1(0, P0 + AH, 2 * LN_ROWS)
    v_proj(0, P0)
    c_w1.wait()
    mix_in(0, P0 + AH)
    kv_acc(P0, first=True)
    for c in c_loop1:
        c.wait()

    def phase1(i, carry):
        r0 = pl.multiple_of(P0 + i * T1, 256)
        mix_out(pl.multiple_of(i * R2, R2), R2)
        phi_k(r0, T1)
        ln1(r0 + AH, T1, LN_ROWS)
        v_proj(r0, T1)
        mix_in(r0 + AH, T1)
        kv_acc(T1)
        return carry

    lax.fori_loop(0, N1, phase1, 0)

    for c in c_late:
        c.wait()
    mix_out(N1 * R2, R2)
    fold(wq_v, 0)
    z_ref[...] = jnp.broadcast_to(jnp.sum(z_ref[...], axis=1, keepdims=True), z_ref.shape)
    for n0 in range(0, FH, 64):
        big_ref[7 * HH + n0 // 2:7 * HH + n0 // 2 + 32, 0:KH] = _pk(w3t_v[n0:n0 + 64, 0:KH])
    lane4 = lax.broadcasted_iota(jnp.int32, (DH, 128), 1) & 3
    for h in range(H):
        kvt_ref[h * 8:(h + 1) * 8, :] = _pk(
            jnp.where(lane4 == (h % 4), kv_ref[h * DH:(h + 1) * DH, :], 0.0))
    mix_out((N1 + 1) * R2, R2)

    def phi_q(r0):
        pq = _dot_nt(_up(wt_ref[0:MQ // 2, :]), x_v[pl.ds(r0, T2), :])
        for c in range(T2 // 128):
            cs = slice(c * 128, (c + 1) * 128)
            for j in range(NJ):
                zp = z_ref[j * 128:j * 128 + 64, :].reshape(8, 8, 128)
                zn = z_ref[j * 128 + 64:(j + 1) * 128, :].reshape(8, 8, 128)
                ep, en, rp, rn = _dual_exp(_logits(pq, j, c))
                den = jnp.sum(ep * zp, axis=0) * rp + jnp.sum(en * zn, axis=0) * rn
                rd = _recip(_fold4(den, jnp.add) + 1e-6)
                phi_ref[j * 64:j * 64 + 32, cs] = _pk((ep * (rp * rd)[None]).reshape(64, 128))
                phi_ref[j * 64 + 32:(j + 1) * 64, cs] = _pk((en * (rn * rd)[None]).reshape(64, 128))

    def mlp_in_tail(k):
        rs = slice(k * HC // 2, (k + 1) * HC // 2)
        xh = jnp.concatenate([sa_ref[2 * k * HH:(2 * k + 1) * HH, :], sa_ref[(2 * k + 1) * HH:(2 * k + 2) * HH, :]], axis=1)
        ut = _gelu(_dot_nt(w3t_v[FM:F, :], _up(xh)))
        ut = jnp.concatenate([ut, jnp.zeros((128 - (F - FM), HC), f32)], axis=0)
        ur_ref[rs, :] = _pk(ut.T)[:, 0:F - FM]

    def mlp_dots(n0, nb):
        lhs = lambda i: _up(sa_ref[i * HH:(i + 1) * HH, :])
        blk = lambda t: w3t_v[(t % 2) * FH + n0:(t % 2) * FH + n0 + nb, (t // 2) * KH:(t // 2 + 1) * KH]

        def rsum(i):
            p, q, sign = RHS_TERMS[i]
            bp, bq = blk(p).astype(f32), blk(q).astype(f32)
            return (bp + bq if sign > 0 else bp - bq).astype(bf16)

        m2 = _dot_nt(lhs(5), _up(big_ref[7 * HH + n0 // 2:7 * HH + (n0 + nb) // 2, 0:KH]))
        m4 = _dot_nt(lhs(3), rsum(2))
        m1 = _dot_nt(lhs(4), rsum(0))
        m3 = _dot_nt(lhs(0), rsum(1))
        m5 = _dot_nt(lhs(6), blk(3))
        m6 = _dot_nt(lhs(7), rsum(3))
        m7 = _dot_nt(lhs(8), rsum(4))
        return [m1, m2, m3, m4, m5, m6, m7]

    act_ref = big_ref.at[pl.ds(pl.multiple_of(zero * 8, 8), 7 * HH)]

    def mlp_act(ms, n0, nb):
        for r in range(0, HC, AR):
            u11, u12, u21, u22 = (_gelu(c) for c in _quadrants(*[m[r:r + AR] for m in ms]))
            s1, s2, s5, s6, s7 = _lhs_sums(u11, u12, u21, u22)
            for i, s in enumerate((s1, s2, u11, u22, s5, s6, s7)):
                act_ref[i * HH + r // 2:i * HH + (r + AR) // 2, n0:n0 + nb] = _pk(s)

    def attn_out(r0, h):
        cs = slice(h * AC, (h + 1) * AC)
        ot = [_dot(_up(kvt_ref[j * 32:(j + 1) * 32, :]), _up(phi_ref[j * 64:(j + 1) * 64, cs]))
              for j in range(NJ)]
        o_ref[h * AC // 2:(h + 1) * AC // 2, :] = _pk(jnp.concatenate(ot, axis=0).T)

    def attn_mix(r0, off, n):
        rows = pl.ds(r0 + off, n)
        a = _dot(_up(o_ref[off // 2:(off + n) // 2, :]), wo_v[...])
        gw = gw_v[...].astype(f32).reshape(1, D)
        gl = jnp.sum(x_v[rows, :].astype(f32) * gw, axis=-1, keepdims=True)
        th = 0.5 * jnp.tanh(0.5 * gl)
        x1 = x1_ref[rows, :]
        acc_ref[off:off + n, :] = x1 + (0.5 + th) * (a - x1)
        g_ref[off:off + n, :] = jnp.broadcast_to(0.5 - th, (n, 128))

    def phase2(t, carry):
        r0 = pl.multiple_of(t * T2, T2)
        phi_q(r0)
        for h in range(T2 // AC):
            attn_out(r0, h)
        nw = T2 // WOC
        for k in range(nw):
            if LNPOS == 0:
                ln2(r0, k * HC // nw, (k + 1) * HC // nw)
            attn_mix(r0, k * WOC, WOC)
        if LNPOS == 1:
            ln2(r0, 0, HC)
        prev = None
        for n0 in range(0, FH, NB):
            cur = (mlp_dots(n0, min(NB, FH - n0)), n0, min(NB, FH - n0))
            if prev is not None:
                mlp_act(*prev)
            prev = cur
        mlp_in_tail(0)
        mlp_in_tail(1)
        mlp_act(*prev)
        off = 0
        for k, n in enumerate(OUT_CHUNKS):
            ms = []
            for i, ti in enumerate((0, None, 1, 2, None, 3, 4)):
                if ti is None:
                    rhs = w4_v[0:FH, 0:KH] if i == 1 else w4_v[FH:FM, KH:D]
                else:
                    if k == 0:
                        w4_sum(ti)
                    rhs = _up(t4_ref[ti * FQ:(ti + 1) * FQ, :])
                ms.append(_dot(_up(big_ref[i * HH + off // 2:i * HH + (off + n) // 2, :]), rhs))
            c11, c12, c21, c22 = _quadrants(*ms)
            for half, cc in enumerate(((c11, c12), (c21, c22))):
                o2 = off + half * HC
                rows = pl.ds(r0 + o2, n)
                h2 = jnp.concatenate(cc, axis=1) + _dot(_up(ur_ref[o2 // 2:(o2 + n) // 2, :]), w4_v[FM:F, :])
                gb = jnp.concatenate([g_ref[o2:o2 + n, :]] * 4, axis=1)
                out_v[rows, :] = (acc_ref[o2:o2 + n, :] + gb * h2).astype(bf16)
                copy(out_v.at[rows], out_hbm.at[rows], 0).start()
            off += n
        return carry

    lax.fori_loop(0, NT2, phase2, 0)
    copy(out_v, out_hbm, 0).wait()


def _kernel(*refs):
    trips = refs[-1]
    trips[0] = 1

    def once(i, carry):
        _body(i, *refs[:-1])
        return carry

    lax.fori_loop(0, trips[0], once, 0)


@jax.jit
def pallas_gated_mix__linear_kernel_hedgehog__mixer_s_mlp__prompt_kernel(
        A_x, A_wqkv, A_w_phi, A_wo, B_x, B_w1, B_w2, B_w3, B_w4, gate_w):
    del B_x
    x = A_x.reshape(S, D)
    wphi = jnp.transpose(A_w_phi, (1, 2, 0)).reshape(DH * DH, H)
    w3t = B_w3.T
    hbm = pl.BlockSpec(memory_space=pl.ANY)
    out = pl.pallas_call(
        _kernel,
        out_shape=jax.ShapeDtypeStruct((S, D), bf16),
        in_specs=[hbm] * 9,
        out_specs=hbm,
        scratch_shapes=[
            pltpu.VMEM((S + AH, D), bf16),
            pltpu.VMEM((D, D), bf16),
            pltpu.VMEM((D, D), bf16),
            pltpu.VMEM((D, D), bf16),
            pltpu.VMEM((DH * DH, H), bf16),
            pltpu.VMEM((D, D), bf16),
            pltpu.VMEM((D, D), bf16),
            pltpu.VMEM((D, D), bf16),
            pltpu.VMEM((F, D), bf16),
            pltpu.VMEM((F, D), bf16),
            pltpu.VMEM((D,), bf16),
            pltpu.VMEM((S, D), bf16),
            pltpu.VMEM((MQ + D // 2, D), u32),
            pltpu.VMEM((4, PAD + S + AH, 128), f32),
            pltpu.VMEM((D, 128), f32),
            pltpu.VMEM((NJ * 128, 128), f32),
            pltpu.VMEM((D // 2, 128), u32),
            pltpu.VMEM((NJ * 64, T2), u32),
            pltpu.VMEM((64, D), u32),
            pltpu.VMEM((T1, D), f32),
            pltpu.VMEM((D // 2, T1), u32),
            pltpu.VMEM((S, D), f32),
            pltpu.VMEM((9 * HH, KH), u32),
            pltpu.VMEM((7 * HH + FQ, FH), u32),
            pltpu.VMEM((T2 // 2, F - FM), u32),
            pltpu.VMEM((5 * FQ, KH), u32),
            pltpu.VMEM((T2 // 2, D), u32),
            pltpu.VMEM((T2, D), f32),
            pltpu.VMEM((T2, 128), f32),
            pltpu.SemaphoreType.DMA((4,)),
            pltpu.SMEM((1,), jnp.int32),
        ],
        compiler_params=pltpu.CompilerParams(vmem_limit_bytes=100 * 1024 * 1024),
    )(x, A_wqkv, wphi, A_wo, B_w1, B_w2, w3t, B_w4, gate_w)
    return out.reshape(1, S, D)
```

```python
import jax
import jax.numpy as jnp
from jax import lax
import jax.experimental.pallas as pl
import jax.experimental.pallas.tpu as pltpu

S, D, H, DH, F = 2048, 512, 32, 16, 1376
NJ = 8
MQ = 480
T0 = 256
P0 = 512
T1 = 768
N1 = (S - P0) // T1
R2 = 512
T2 = 1024
NT2 = S // T2
HC = 512
FM = 1280
AH = 32
PAD = 8
OUT_CHUNKS = tuple(int(v) for v in '192,192,96,32'.split(','))
KH = D // 2
LHS_TERMS = ((0, 3, 1), (2, 3, 1), (0, None, 1), (3, None, 1), (0, 1, 1), (2, 0, -1), (1, 3, -1))
W2ORD = [int(v) for v in '1,3,0,2,4,5,6'.split(',')]
AC = int(512)
WOC = int(512)
PIPE = int(0)
MID2 = int(1)
W4ORD = [int(v) for v in '1,3,0,2,4,5,6'.split(',')]
LDYN = int(0)
L2R = int(16)
VSTR = int(1)
SBR = int(64)
SUM_TERMS = ((0, 3, 1), (2, 3, 1), (0, 1, 1), (2, 0, -1), (1, 3, -1))
LNPOS = int(0)
RHS_TERMS = ((0, 3, 1), (1, 3, -1), (2, 0, -1), (0, 1, 1), (2, 3, 1))
WC = int(16)
AR = int(16)
FH = FM // 2
FQ = FH // 2
HH = HC // 2
NB = int(128)
WPRE = int(0)
LN_ROWS = 16
LOG2E = 1.4426950408889634
NT_DIMS = (((1,), (1,)), ((), ()))
SHIFTS = (-1, 1, -2, 2)
f32 = jnp.float32
bf16 = jnp.bfloat16
u32 = jnp.uint32


def _pk(x):
    return pltpu.bitcast(x.astype(bf16), u32)


def _up(x):
    return pltpu.bitcast(x, bf16)


def _dot(a, b):
    return jnp.dot(a, b, preferred_element_type=f32)


def _dot_nt(a, b):
    return lax.dot_general(a, b, NT_DIMS, preferred_element_type=f32)


def _gelu(x):
    c = 0.7978845608028654
    t = jnp.tanh(x * (c + (c * 0.044715) * (x * x)))
    hx = 0.5 * x
    return hx + hx * t


def _ln(x):
    m = jnp.mean(x, axis=-1, keepdims=True)
    xc = x - m
    v = jnp.mean(xc * xc, axis=-1, keepdims=True)
    return xc * jnp.exp2((-0.5 * LOG2E) * jnp.log(v + 1e-5))


def _recip(x):
    r = pl.reciprocal(x, approx=True)
    return r * (2.0 - x * r)


def _fold4(a, op):
    return op(a, pltpu.roll(a, 4, 0))


def _dual_exp(p):
    mx = _fold4(jnp.max(p, axis=0), jnp.maximum)
    mn = _fold4(jnp.min(p, axis=0), jnp.minimum)
    ep = jnp.exp2(p - mx[None])
    en = jnp.exp2(mn[None] - p)
    rp = _recip(_fold4(jnp.sum(ep, axis=0), jnp.add))
    rn = _recip(_fold4(jnp.sum(en, axis=0), jnp.add))
    return ep, en, rp, rn


def _lhs_sums(a11, a12, a21, a22):
    return (a11 + a22, a21 + a22, a11 + a12, a21 - a11, a12 - a22)


def _rhs_sums(b11, b12, b21, b22):
    b11, b12, b21, b22 = (b.astype(f32) for b in (b11, b12, b21, b22))
    return (b11 + b22, b12 - b22, b21 - b11, b11 + b12, b21 + b22)


def _quadrants(m1, m2, m3, m4, m5, m6, m7):
    return m1 + m4 - m5 + m7, m3 + m5, m2 + m4, m1 - m2 + m3 + m6


def _logits(pm, j, c):
    lo = lax.broadcasted_iota(jnp.int32, (8, 128), 0) < 4
    g, jj = j // 2, j % 2
    cs = slice(c * 128, (c + 1) * 128)
    own = pm[g * 120 + jj * 64:g * 120 + jj * 64 + 56, cs].reshape(7, 8, 128)
    sh = pm[g * 120 + 56:g * 120 + 64, cs]
    last = jnp.where(lo, sh, 0.0) if jj == 0 else jnp.where(lo, 0.0, sh)
    return jnp.concatenate([own, last[None]], axis=0)


def _body(zero, x_hbm, wqkv_hbm, wphi_hbm, wo_hbm, w1_hbm, w2_hbm, w3t_hbm, w4_hbm, gw_hbm,
          out_hbm,
          x_v, wq_v, wk_v, wv_v, wphi_v, wo_v, w1_v, w2_v, w3t_v, w4_v, gw_v, out_v,
          wt_ref, h_ref, kv_ref, z_ref, kvt_ref, phi_ref, p_ref, xn_ref, vt_ref,
          x1_ref, sa_ref, big_ref, ur_ref, t4_ref, o_ref, acc_ref, x1n_ref, va_ref, sem):
    def copy(src, dst, k):
        return pltpu.make_async_copy(src, dst, sem.at[k])

    def xcopy(a, b, k):
        return copy(x_hbm.at[a:b], x_v.at[a:b], k)

    c_phi = copy(wphi_hbm, wphi_v, 0)
    c_wk = copy(wqkv_hbm.at[:, D:2 * D], wk_v, 1)
    c_x0 = xcopy(0, T0, 2)
    c_x1 = xcopy(T0, P0 + AH, 3)
    c_wv = copy(wqkv_hbm.at[:, 2 * D:3 * D], wv_v, 3)
    c_w1 = copy(w1_hbm, w1_v, 1)
    c_loop1 = [copy(w2_hbm, w2_v, 2), xcopy(P0 + AH, S, 2)]
    c_late = [copy(wqkv_hbm.at[:, 0:D], wq_v, 3), copy(w3t_hbm, w3t_v, 3), copy(w4_hbm, w4_v, 3),
              copy(wo_hbm, wo_v, 3), copy(gw_hbm, gw_v, 3)]
    c_phi.start()
    c_wk.start()

    x_v[S:S + AH, :] = jnp.zeros((AH, D), bf16)
    for q in range(4):
        h_ref[q, 0:PAD, :] = jnp.zeros((PAD, 128), f32)

    c_phi.wait()
    c_x0.start()
    c_x1.start()
    sel = (lax.broadcasted_iota(jnp.int32, (H, D), 0)
           == lax.broadcasted_iota(jnp.int32, (H, D), 1) // DH)
    bm = _dot(wphi_v[...], jnp.where(sel, 1.0, 0.0).astype(bf16))
    dmask = (lax.broadcasted_iota(jnp.int32, (DH * DH, D), 0) // DH
             == lax.broadcasted_iota(jnp.int32, (DH * DH, D), 1) % DH)
    cm = jnp.sum(jnp.where(dmask, bm, 0.0).reshape(DH, DH, D), axis=0).astype(bf16)
    e3 = ((lax.broadcasted_iota(jnp.int32, (128, DH), 0) % 64) // 4
          == lax.broadcasted_iota(jnp.int32, (128, DH), 1))
    pall = _dot(jnp.where(e3, 1.0, 0.0).astype(bf16), cm)
    rr = lax.broadcasted_iota(jnp.int32, (128, D), 0)
    cc = lax.broadcasted_iota(jnp.int32, (128, D), 1)
    pmask = ((cc // DH) % 8) == ((rr // 64) * 4 + rr % 4)
    p_ref[...] = _pk(jnp.where(pmask, pall, 0.0))

    def fold(w_v, base):
        lo = lax.broadcasted_iota(jnp.int32, (8, D), 0) < 4
        for gp in range(2):
            rows = []
            for g in (2 * gp, 2 * gp + 1):
                gs = slice(g * 128, (g + 1) * 128)
                wt = _dot_nt(_up(p_ref[:, gs]), w_v[:, gs])
                ds = []
                for jj in range(2):
                    a = wt[jj * 64:(jj + 1) * 64, :].reshape(8, 8, D)
                    f15 = jnp.where(lo, pltpu.roll(a[7], 4, 0), a[7])
                    ds.append((a - f15[None]) * LOG2E)
                f14 = jnp.where(lo, ds[0][7], pltpu.roll(ds[1][7], 4, 0))
                rows += [ds[0][0:7].reshape(56, D), f14, ds[1][0:7].reshape(56, D)]
            wt_ref[base + gp * 120:base + (gp + 1) * 120, :] = _pk(jnp.concatenate(rows, axis=0))

    def phi_k(r0, n, off=0, first=False):
        pk = _dot_nt(_up(wt_ref[MQ // 2:MQ, :]), x_v[pl.ds(r0, n), :])
        for c in range(n // 128):
            cs = slice(off + c * 128, off + (c + 1) * 128)
            for j in range(NJ):
                ep, en, rp, rn = _dual_exp(_logits(pk, j, c))
                ep = (ep * rp[None]).reshape(64, 128)
                en = (en * rn[None]).reshape(64, 128)
                if first and c == 0:
                    z_ref[j * 128:j * 128 + 64, :] = ep
                    z_ref[j * 128 + 64:(j + 1) * 128, :] = en
                else:
                    z_ref[j * 128:j * 128 + 64, :] += ep
                    z_ref[j * 128 + 64:(j + 1) * 128, :] += en
                phi_ref[j * 64:j * 64 + 32, cs] = _pk(ep)
                phi_ref[j * 64 + 32:(j + 1) * 64, cs] = _pk(en)

    def v_proj(r0, n, first=False):
        if not VSTR:
            vt_ref[:, 0:n] = _pk(_dot_nt(_up(wt_ref[MQ:MQ + D // 2, :]), x_v[pl.ds(r0, n), :]))
            return
        m, kq = n // 2, KH // 2
        ablk = lambda t: _up(wt_ref[MQ + (t // 2) * kq:MQ + (t // 2 + 1) * kq, (t % 2) * KH:(t % 2 + 1) * KH])
        bblk = lambda t: x_v[pl.ds(r0 + (t % 2) * m, m), (t // 2) * KH:(t // 2 + 1) * KH]
        ms = [None] * 7
        for i in W2ORD:
            p, q, sign = LHS_TERMS[i]
            if q is None:
                lhs = ablk(p)
            else:
                if first:
                    ap, aq = ablk(p).astype(f32), ablk(q).astype(f32)
                    va_ref[i * kq:(i + 1) * kq, :] = _pk(ap + aq if sign > 0 else ap - aq)
                lhs = _up(va_ref[i * kq:(i + 1) * kq, :])
            ti = (0, None, 1, 2, None, 3, 4)[i]
            if ti is None:
                rhs = bblk(0) if i == 1 else bblk(3)
            else:
                p, q, sign = RHS_TERMS[ti]
                bp, bq = bblk(p).astype(f32), bblk(q).astype(f32)
                rhs = (bp + bq if sign > 0 else bp - bq).astype(bf16)
            ms[i] = _dot_nt(lhs, rhs)
        for t, c in enumerate(_quadrants(*ms)):
            vt_ref[(t // 2) * kq:(t // 2 + 1) * kq, (t % 2) * m:(t % 2 + 1) * m] = _pk(c)

    def kv_acc(n, first=False):
        for j in range(NJ):
            r = _dot_nt(_up(vt_ref[j * 32:(j + 1) * 32, 0:n]), _up(phi_ref[j * 64:(j + 1) * 64, 0:n]))
            if first:
                kv_ref[j * 64:(j + 1) * 64, :] = r
            else:
                kv_ref[j * 64:(j + 1) * 64, :] += r

    def ln1(r0, n, ch):
        for r in range(0, n, ch):
            m = min(ch, n - r)
            xn_ref[r:r + m, :] = _ln(x_v[pl.ds(r0 + r, m), :].astype(f32))

    def sq_rhs(w_v, i):
        blk = lambda t: w_v[(t // 2) * KH:(t // 2 + 1) * KH, (t % 2) * KH:(t % 2 + 1) * KH]
        ti = (0, None, 1, 2, None, 3, 4)[i]
        if ti is None:
            return blk(0) if i == 1 else blk(3)
        p, q, sign = RHS_TERMS[ti]
        bp, bq = blk(p).astype(f32), blk(q).astype(f32)
        return (bp + bq if sign > 0 else bp - bq).astype(bf16)

    def sq_strassen(blk, w_v):
        ms = [None] * 7
        for i in W2ORD:
            p, q, sign = LHS_TERMS[i]
            lhs = blk(p) if q is None else (blk(p) + blk(q) if sign > 0 else blk(p) - blk(q))
            ms[i] = _dot(lhs.astype(bf16), sq_rhs(w_v, i))
        return _quadrants(*ms)

    def mix_in(r0, n):
        m = n // 2
        blk = lambda t: xn_ref[(t // 2) * m:(t // 2 + 1) * m, (t % 2) * KH:(t % 2 + 1) * KH]
        for t, c in enumerate(sq_strassen(blk, w1_v)):
            h = _gelu(c)
            for q in range(2):
                h_ref[2 * (t % 2) + q, pl.ds(PAD + r0 + (t // 2) * m, m), :] = h[:, q * 128:(q + 1) * 128]

    def mix_out(r0, n):
        m = n // 2

        def blk(t):
            return jnp.concatenate(
                [h_ref[q, pl.ds(PAD + r0 + (t // 2) * m + SHIFTS[q], m), :]
                 for q in (2 * (t % 2), 2 * (t % 2) + 1)], axis=1)

        cs = sq_strassen(blk, w2_v)
        for t in (2, 1, 3, 0):
            rows, cols = pl.ds(r0 + (t // 2) * m, m), slice((t % 2) * KH, (t % 2 + 1) * KH)
            x1_ref[rows, cols] = x_v[rows, cols].astype(f32) + cs[t]

    x1n_dyn = x1n_ref.at[pl.ds(pl.multiple_of(zero * 8, 8), T2)] if LDYN else x1n_ref

    def ln2(r0, a, b):
        views = [x1_ref.at[pl.ds(pl.multiple_of(r0 + zero * (8 * p), 8), T2)] for p in range(3)]
        for r in range(a, b, L2R):
            m = jnp.mean(views[0][r:r + L2R, :], axis=-1, keepdims=True)
            xc = views[1][r:r + L2R, :] - m
            v = jnp.mean(xc * xc, axis=-1, keepdims=True)
            rs = jnp.exp2((-0.5 * LOG2E) * jnp.log(v + 1e-5))
            x1n_dyn[r:r + L2R, :] = (views[2][r:r + L2R, :] - m) * rs

    def sa_build(i):
        p, q, sign = (i, None, 1) if i < 4 else SUM_TERMS[i - 4]
        for r in range(0, HC, SBR):
            blk = lambda t: x1n_ref[(t // 2) * HC + r:(t // 2) * HC + r + SBR, (t % 2) * KH:(t % 2 + 1) * KH]
            s = blk(p) if q is None else (blk(p) + blk(q) if sign > 0 else blk(p) - blk(q))
            sa_ref[i * HH + r // 2:i * HH + (r + SBR) // 2, :] = _pk(s)

    def w4_sum(i):
        p, q, sign = RHS_TERMS[i]
        for k0 in range(0, FH, WC):
            blk = lambda t: w4_v[(t // 2) * FH + k0:(t // 2) * FH + k0 + WC,
                                 (t % 2) * KH:(t % 2 + 1) * KH].astype(f32)
            s = blk(p) + blk(q) if sign > 0 else blk(p) - blk(q)
            t4_ref[i * FQ + k0 // 2:i * FQ + (k0 + WC) // 2, :] = _pk(s)

    c_wk.wait()
    c_wv.start()
    c_w1.start()
    fold(wk_v, MQ // 2)
    c_x0.wait()
    for c in c_loop1:
        c.start()
    phi_k(0, T0, first=True)
    c_x1.wait()
    c_wv.wait()
    for c in c_late:
        c.start()
    wt_ref[MQ:MQ + D // 2, :] = _pk(wv_v[...].T)
    phi_k(T0, P0 - T0, off=T0)
    ln1(0, P0 + AH, 2 * LN_ROWS)
    v_proj(0, P0, first=True)
    c_w1.wait()
    mix_in(0, P0 + AH)
    kv_acc(P0, first=True)
    for c in c_loop1:
        c.wait()

    def phase1(i, carry):
        r0 = pl.multiple_of(P0 + i * T1, 256)
        mix_out(pl.multiple_of(i * R2, R2), R2)
        phi_k(r0, T1)
        ln1(r0 + AH, T1, LN_ROWS)
        v_proj(r0, T1)
        mix_in(r0 + AH, T1)
        kv_acc(T1)
        return carry

    lax.fori_loop(0, N1, phase1, 0)

    for c in c_late:
        c.wait()
    mix_out(N1 * R2, R2 * (2 - MID2))
    fold(wq_v, 0)
    if PIPE:
        ln2(0, 0, T2)
    z_ref[...] = jnp.broadcast_to(jnp.sum(z_ref[...], axis=1, keepdims=True), z_ref.shape)
    for n0 in range(0, FH, 64):
        big_ref[7 * HH + n0 // 2:7 * HH + n0 // 2 + 32, 0:KH] = _pk(w3t_v[n0:n0 + 64, 0:KH])
    lane4 = lax.broadcasted_iota(jnp.int32, (DH, 128), 1) & 3
    for h in range(H):
        kvt_ref[h * 8:(h + 1) * 8, :] = _pk(
            jnp.where(lane4 == (h % 4), kv_ref[h * DH:(h + 1) * DH, :], 0.0))
    if MID2:
        mix_out((N1 + 1) * R2, R2)

    def phi_q(r0):
        pq = _dot_nt(_up(wt_ref[0:MQ // 2, :]), x_v[pl.ds(r0, T2), :])
        for c in range(T2 // 128):
            cs = slice(c * 128, (c + 1) * 128)
            for j in range(NJ):
                zp = z_ref[j * 128:j * 128 + 64, :].reshape(8, 8, 128)
                zn = z_ref[j * 128 + 64:(j + 1) * 128, :].reshape(8, 8, 128)
                ep, en, rp, rn = _dual_exp(_logits(pq, j, c))
                den = jnp.sum(ep * zp, axis=0) * rp + jnp.sum(en * zn, axis=0) * rn
                rd = _recip(_fold4(den, jnp.add) + 1e-6)
                phi_ref[j * 64:j * 64 + 32, cs] = _pk((ep * (rp * rd)[None]).reshape(64, 128))
                phi_ref[j * 64 + 32:(j + 1) * 64, cs] = _pk((en * (rn * rd)[None]).reshape(64, 128))

    def mlp_in_tail(k):
        rs = slice(k * HC // 2, (k + 1) * HC // 2)
        xh = jnp.concatenate([sa_ref[2 * k * HH:(2 * k + 1) * HH, :], sa_ref[(2 * k + 1) * HH:(2 * k + 2) * HH, :]], axis=1)
        ut = _gelu(_dot_nt(w3t_v[FM:F, :], _up(xh)))
        ut = jnp.concatenate([ut, jnp.zeros((128 - (F - FM), HC), f32)], axis=0)
        ur_ref[rs, :] = _pk(ut.T)[:, 0:F - FM]

    def mlp_dots(n0, nb):
        def lhs(i):
            if n0 == 0:
                sa_build(i)
            return _up(sa_ref[i * HH:(i + 1) * HH, :])

        blk = lambda t: w3t_v[(t % 2) * FH + n0:(t % 2) * FH + n0 + nb, (t // 2) * KH:(t // 2 + 1) * KH]

        def rsum(i):
            p, q, sign = RHS_TERMS[i]
            bp, bq = blk(p).astype(f32), blk(q).astype(f32)
            return (bp + bq if sign > 0 else bp - bq).astype(bf16)

        m2 = _dot_nt(lhs(5), _up(big_ref[7 * HH + n0 // 2:7 * HH + (n0 + nb) // 2, 0:KH]))
        m4 = _dot_nt(lhs(3), rsum(2))
        m1 = _dot_nt(lhs(4), rsum(0))
        m3 = _dot_nt(lhs(0), rsum(1))
        m5 = _dot_nt(lhs(6), blk(3))
        m6 = _dot_nt(lhs(7), rsum(3))
        m7 = _dot_nt(lhs(8), rsum(4))
        return [m1, m2, m3, m4, m5, m6, m7]

    act_ref = big_ref.at[pl.ds(pl.multiple_of(zero * 8, 8), 7 * HH)]

    def mlp_act(ms, n0, nb):
        for r in range(0, HC, AR):
            u11, u12, u21, u22 = (_gelu(c) for c in _quadrants(*[m[r:r + AR] for m in ms]))
            s1, s2, s5, s6, s7 = _lhs_sums(u11, u12, u21, u22)
            for i, s in enumerate((s1, s2, u11, u22, s5, s6, s7)):
                act_ref[i * HH + r // 2:i * HH + (r + AR) // 2, n0:n0 + nb] = _pk(s)

    def attn_out(r0, h):
        cs = slice(h * AC, (h + 1) * AC)
        ot = [_dot(_up(kvt_ref[j * 32:(j + 1) * 32, :]), _up(phi_ref[j * 64:(j + 1) * 64, cs]))
              for j in range(NJ)]
        o_ref[h * AC:(h + 1) * AC, :] = jnp.concatenate(ot, axis=0).T

    def attn_mix(off, n):
        m = n // 2
        blk = lambda t: o_ref[off + (t // 2) * m:off + (t // 2 + 1) * m, (t % 2) * KH:(t % 2 + 1) * KH]
        for t, c in enumerate(sq_strassen(blk, wo_v)):
            acc_ref[off + (t // 2) * m:off + (t // 2 + 1) * m, (t % 2) * KH:(t % 2 + 1) * KH] = c

    def phase2(t, carry):
        r0 = pl.multiple_of(t * T2, T2)
        r_next = pl.multiple_of(((t + 1) & (NT2 - 1)) * T2, T2)
        phi_q(r0)
        for h in range(T2 // AC):
            attn_out(r0, h)
        if not PIPE:
            ln2(r0, 0, T2)
        for k in range(T2 // WOC):
            attn_mix(k * WOC, WOC)
        prev = None
        for n0 in range(0, FH, NB):
            cur = (mlp_dots(n0, min(NB, FH - n0)), n0, min(NB, FH - n0))
            if prev is not None:
                mlp_act(*prev)
            prev = cur
        sa_build(1)
        sa_build(2)
        mlp_in_tail(0)
        mlp_in_tail(1)
        mlp_act(*prev)
        off = 0
        for k, n in enumerate(OUT_CHUNKS):
            if PIPE and k < 2:
                ln2(r_next, k * HC, (k + 1) * HC)
            rems, gates = [], []
            gw = gw_v[...].astype(f32).reshape(1, D)
            for half in range(2):
                o2 = off + half * HC
                rems.append(_dot(_up(ur_ref[o2 // 2:(o2 + n) // 2, :]), w4_v[FM:F, :]))
                gl = jnp.sum(x_v[pl.ds(r0 + o2, n), :].astype(f32) * gw, axis=-1, keepdims=True)
                gates.append(0.5 * jnp.tanh(0.5 * gl) + 0.5)
            ms = [None] * 7
            for i in W4ORD:
                ti = (0, None, 1, 2, None, 3, 4)[i]
                if ti is None:
                    rhs = w4_v[0:FH, 0:KH] if i == 1 else w4_v[FH:FM, KH:D]
                else:
                    if k == 0:
                        w4_sum(ti)
                    rhs = _up(t4_ref[ti * FQ:(ti + 1) * FQ, :])
                ms[i] = _dot(_up(big_ref[i * HH + off // 2:i * HH + (off + n) // 2, :]), rhs)
            for q, c in enumerate(_quadrants(*ms)):
                half, cs = q // 2, slice((q % 2) * KH, (q % 2 + 1) * KH)
                o2 = off + half * HC
                rows = pl.ds(r0 + o2, n)
                b = x1_ref[rows, cs] + rems[half][:, cs] + c
                out_v[rows, cs] = (b + gates[half] * (acc_ref[o2:o2 + n, cs] - b)).astype(bf16)
            for half in range(2):
                rows = pl.ds(r0 + off + half * HC, n)
                copy(out_v.at[rows], out_hbm.at[rows], 0).start()
            off += n
        return carry

    lax.fori_loop(0, NT2, phase2, 0)
    copy(out_v, out_hbm, 0).wait()


def _kernel(*refs):
    trips = refs[-1]
    trips[0] = 1

    def once(i, carry):
        _body(i, *refs[:-1])
        return carry

    lax.fori_loop(0, trips[0], once, 0)


@jax.jit
def pallas_gated_mix__linear_kernel_hedgehog__mixer_s_mlp__prompt_kernel(
        A_x, A_wqkv, A_w_phi, A_wo, B_x, B_w1, B_w2, B_w3, B_w4, gate_w):
    del B_x
    x = A_x.reshape(S, D)
    wphi = jnp.transpose(A_w_phi, (1, 2, 0)).reshape(DH * DH, H)
    w3t = B_w3.T
    hbm = pl.BlockSpec(memory_space=pl.ANY)
    out = pl.pallas_call(
        _kernel,
        out_shape=jax.ShapeDtypeStruct((S, D), bf16),
        in_specs=[hbm] * 9,
        out_specs=hbm,
        scratch_shapes=[
            pltpu.VMEM((S + AH, D), bf16),
            pltpu.VMEM((D, D), bf16),
            pltpu.VMEM((D, D), bf16),
            pltpu.VMEM((D, D), bf16),
            pltpu.VMEM((DH * DH, H), bf16),
            pltpu.VMEM((D, D), bf16),
            pltpu.VMEM((D, D), bf16),
            pltpu.VMEM((D, D), bf16),
            pltpu.VMEM((F, D), bf16),
            pltpu.VMEM((F, D), bf16),
            pltpu.VMEM((D,), bf16),
            pltpu.VMEM((S, D), bf16),
            pltpu.VMEM((MQ + D // 2, D), u32),
            pltpu.VMEM((4, PAD + S + AH, 128), f32),
            pltpu.VMEM((D, 128), f32),
            pltpu.VMEM((NJ * 128, 128), f32),
            pltpu.VMEM((D // 2, 128), u32),
            pltpu.VMEM((NJ * 64, T2), u32),
            pltpu.VMEM((64, D), u32),
            pltpu.VMEM((T1, D), f32),
            pltpu.VMEM((D // 2, T1), u32),
            pltpu.VMEM((S, D), f32),
            pltpu.VMEM((9 * HH, KH), u32),
            pltpu.VMEM((7 * HH + FQ, FH), u32),
            pltpu.VMEM((T2 // 2, F - FM), u32),
            pltpu.VMEM((5 * FQ, KH), u32),
            pltpu.VMEM((T2, D), f32),
            pltpu.VMEM((T2, D), f32),
            pltpu.VMEM((T2 + 8, D), f32),
            pltpu.VMEM((7 * KH // 2, KH), u32),
            pltpu.SemaphoreType.DMA((4,)),
            pltpu.SMEM((1,), jnp.int32),
        ],
        compiler_params=pltpu.CompilerParams(vmem_limit_bytes=100 * 1024 * 1024),
    )(x, A_wqkv, wphi, A_wo, B_w1, B_w2, w3t, B_w4, gate_w)
    return out.reshape(1, S, D)
```

```python
import jax
import jax.numpy as jnp
from jax import lax
import jax.experimental.pallas as pl
import jax.experimental.pallas.tpu as pltpu

S, D, H, DH, F = 2048, 512, 32, 16, 1376
NJ = 8
MQ = 480
T0 = 256
P0 = 512
T1 = 768
N1 = (S - P0) // T1
R2 = 512
T2 = 1024
NT2 = S // T2
HC = 512
FM = 1280
AH = 32
PAD = 8
OUT_CHUNKS = tuple(int(v) for v in '224,160,96,32'.split(','))
KH = D // 2
LHS_TERMS = ((0, 3, 1), (2, 3, 1), (0, None, 1), (3, None, 1), (0, 1, 1), (2, 0, -1), (1, 3, -1))
W2ORD = [int(v) for v in '1,3,0,2,4,5,6'.split(',')]
AC = int(512)
WOC = int(512)
PIPE = int(0)
MID2 = int(1)
W4ORD = [int(v) for v in '1,3,0,2,4,5,6'.split(',')]
LDYN = int(0)
L2R = int(16)
VSTR = int(1)
FRESH = int(1)
FUSE = int(0)
SBR = int(64)
SUM_TERMS = ((0, 3, 1), (2, 3, 1), (0, 1, 1), (2, 0, -1), (1, 3, -1))
LNPOS = int(0)
RHS_TERMS = ((0, 3, 1), (1, 3, -1), (2, 0, -1), (0, 1, 1), (2, 3, 1))
WC = int(16)
AR = int(16)
FH = FM // 2
FQ = FH // 2
HH = HC // 2
NB = int(128)
WPRE = int(0)
LN_ROWS = 16
LOG2E = 1.4426950408889634
NT_DIMS = (((1,), (1,)), ((), ()))
SHIFTS = (-1, 1, -2, 2)
f32 = jnp.float32
bf16 = jnp.bfloat16
u32 = jnp.uint32


def _pk(x):
    return pltpu.bitcast(x.astype(bf16), u32)


def _up(x):
    return pltpu.bitcast(x, bf16)


def _dot(a, b):
    return jnp.dot(a, b, preferred_element_type=f32)


def _dot_nt(a, b):
    return lax.dot_general(a, b, NT_DIMS, preferred_element_type=f32)


def _gelu(hx):
    c = 0.7978845608028654
    t = jnp.tanh(hx * (2.0 * c + (8.0 * c * 0.044715) * (hx * hx)))
    return hx + hx * t


def _half_rstd(v):
    return jnp.exp2((-0.5 * LOG2E) * jnp.log(4.0 * v + 4e-5))


def _ln(x):
    m = jnp.mean(x, axis=-1, keepdims=True)
    xc = x - m
    v4 = jnp.sum(xc * xc, axis=-1, keepdims=True) * (4.0 / D)
    return xc * jnp.exp2((-0.5 * LOG2E) * jnp.log(v4 + 4e-5))


def _recip(x):
    r = pl.reciprocal(x, approx=True)
    return r * (2.0 - x * r)


def _fold4(a, op):
    return op(a, pltpu.roll(a, 4, 0))


def _dual_exp(p):
    mx = _fold4(jnp.max(p, axis=0), jnp.maximum)
    mn = _fold4(jnp.min(p, axis=0), jnp.minimum)
    ep = jnp.exp2(p - mx[None])
    en = jnp.exp2(mn[None] - p)
    rp = _recip(_fold4(jnp.sum(ep, axis=0), jnp.add))
    rn = _recip(_fold4(jnp.sum(en, axis=0), jnp.add))
    return ep, en, rp, rn


def _lhs_sums(a11, a12, a21, a22):
    return (a11 + a22, a21 + a22, a11 + a12, a21 - a11, a12 - a22)


def _rhs_sums(b11, b12, b21, b22):
    b11, b12, b21, b22 = (b.astype(f32) for b in (b11, b12, b21, b22))
    return (b11 + b22, b12 - b22, b21 - b11, b11 + b12, b21 + b22)


def _quadrants(m1, m2, m3, m4, m5, m6, m7):
    return m1 + m4 - m5 + m7, m3 + m5, m2 + m4, m1 - m2 + m3 + m6


def _logits(pm, j, c):
    lo = lax.broadcasted_iota(jnp.int32, (8, 128), 0) < 4
    g, jj = j // 2, j % 2
    cs = slice(c * 128, (c + 1) * 128)
    own = pm[g * 120 + jj * 64:g * 120 + jj * 64 + 56, cs].reshape(7, 8, 128)
    sh = pm[g * 120 + 56:g * 120 + 64, cs]
    last = jnp.where(lo, sh, 0.0) if jj == 0 else jnp.where(lo, 0.0, sh)
    return jnp.concatenate([own, last[None]], axis=0)


def _body(zero, x_hbm, wqkv_hbm, wphi_hbm, wo_hbm, w1_hbm, w2_hbm, w3t_hbm, w4_hbm, gw_hbm,
          out_hbm,
          x_v, wq_v, wk_v, wv_v, wphi_v, wo_v, w1_v, w2_v, w3t_v, w4_v, gw_v, out_v,
          wt_ref, h_ref, kv_ref, z_ref, kvt_ref, phi_ref, p_ref, xn_ref, vt_ref,
          x1_ref, sa_ref, big_ref, ur_ref, t4_ref, o_ref, acc_ref, x1n_ref, va_ref, sem):
    def copy(src, dst, k):
        return pltpu.make_async_copy(src, dst, sem.at[k])

    def xcopy(a, b, k):
        return copy(x_hbm.at[a:b], x_v.at[a:b], k)

    c_phi = copy(wphi_hbm, wphi_v, 0)
    c_wk = copy(wqkv_hbm.at[:, D:2 * D], wk_v, 1)
    c_x0 = xcopy(0, T0, 2)
    c_x1 = xcopy(T0, P0 + AH, 3)
    c_wv = copy(wqkv_hbm.at[:, 2 * D:3 * D], wv_v, 3)
    c_w1 = copy(w1_hbm, w1_v, 1)
    c_loop1 = [copy(w2_hbm, w2_v, 2), xcopy(P0 + AH, S, 2)]
    c_late = [copy(wqkv_hbm.at[:, 0:D], wq_v, 3), copy(w3t_hbm, w3t_v, 3), copy(w4_hbm, w4_v, 3),
              copy(wo_hbm, wo_v, 3), copy(gw_hbm, gw_v, 3)]
    c_phi.start()
    c_wk.start()

    x_v[S:S + AH, :] = jnp.zeros((AH, D), bf16)
    for q in range(4):
        h_ref[q, 0:PAD, :] = jnp.zeros((PAD, 128), f32)

    c_phi.wait()
    c_x0.start()
    c_x1.start()
    sel = (lax.broadcasted_iota(jnp.int32, (H, D), 0)
           == lax.broadcasted_iota(jnp.int32, (H, D), 1) // DH)
    bm = _dot(wphi_v[...], jnp.where(sel, 1.0, 0.0).astype(bf16))
    dmask = (lax.broadcasted_iota(jnp.int32, (DH * DH, D), 0) // DH
             == lax.broadcasted_iota(jnp.int32, (DH * DH, D), 1) % DH)
    cm = jnp.sum(jnp.where(dmask, bm, 0.0).reshape(DH, DH, D), axis=0).astype(bf16)
    e3 = ((lax.broadcasted_iota(jnp.int32, (128, DH), 0) % 64) // 4
          == lax.broadcasted_iota(jnp.int32, (128, DH), 1))
    pall = _dot(jnp.where(e3, 1.0, 0.0).astype(bf16), cm)
    rr = lax.broadcasted_iota(jnp.int32, (128, D), 0)
    cc = lax.broadcasted_iota(jnp.int32, (128, D), 1)
    pmask = ((cc // DH) % 8) == ((rr // 64) * 4 + rr % 4)
    p_ref[...] = _pk(jnp.where(pmask, pall, 0.0))

    def fresh(ref, k):
        if not FRESH:
            return ref
        return ref.at[pl.ds(pl.multiple_of(zero * (16 * (k + 1)), 16), ref.shape[0])]

    def fold(w_v, base):
        lo = lax.broadcasted_iota(jnp.int32, (8, D), 0) < 4
        for gp in range(2):
            rows = []
            for g in (2 * gp, 2 * gp + 1):
                gs = slice(g * 128, (g + 1) * 128)
                wt = _dot_nt(_up(p_ref[:, gs]), w_v[:, gs])
                ds = []
                for jj in range(2):
                    a = wt[jj * 64:(jj + 1) * 64, :].reshape(8, 8, D)
                    f15 = jnp.where(lo, pltpu.roll(a[7], 4, 0), a[7])
                    ds.append((a - f15[None]) * LOG2E)
                f14 = jnp.where(lo, ds[0][7], pltpu.roll(ds[1][7], 4, 0))
                rows += [ds[0][0:7].reshape(56, D), f14, ds[1][0:7].reshape(56, D)]
            wt_ref[base + gp * 120:base + (gp + 1) * 120, :] = _pk(jnp.concatenate(rows, axis=0))

    def phi_k(r0, n, off=0, first=False):
        pk = _dot_nt(_up(wt_ref[MQ // 2:MQ, :]), x_v[pl.ds(r0, n), :])
        for c in range(n // 128):
            cs = slice(off + c * 128, off + (c + 1) * 128)
            for j in range(NJ):
                ep, en, rp, rn = _dual_exp(_logits(pk, j, c))
                ep = (ep * rp[None]).reshape(64, 128)
                en = (en * rn[None]).reshape(64, 128)
                if first and c == 0:
                    z_ref[j * 128:j * 128 + 64, :] = ep
                    z_ref[j * 128 + 64:(j + 1) * 128, :] = en
                else:
                    z_ref[j * 128:j * 128 + 64, :] += ep
                    z_ref[j * 128 + 64:(j + 1) * 128, :] += en
                phi_ref[j * 64:j * 64 + 32, cs] = _pk(ep)
                phi_ref[j * 64 + 32:(j + 1) * 64, cs] = _pk(en)

    def v_proj(r0, n, first=False):
        if not VSTR:
            vt_ref[:, 0:n] = _pk(_dot_nt(_up(wt_ref[MQ:MQ + D // 2, :]), x_v[pl.ds(r0, n), :]))
            return
        m, kq = n // 2, KH // 2
        ablk = lambda t: _up(wt_ref[MQ + (t // 2) * kq:MQ + (t // 2 + 1) * kq, (t % 2) * KH:(t % 2 + 1) * KH])
        ms = [None] * 7
        for i in W2ORD:
            ri = r0 + zero * (16 * (i + 1)) if FRESH else r0
            bblk = lambda t: x_v[pl.ds(pl.multiple_of(ri + (t % 2) * m, 16), m), (t // 2) * KH:(t // 2 + 1) * KH]
            p, q, sign = LHS_TERMS[i]
            if q is None:
                lhs = ablk(p)
            else:
                if first:
                    ap, aq = ablk(p).astype(f32), ablk(q).astype(f32)
                    va_ref[i * kq:(i + 1) * kq, :] = _pk(ap + aq if sign > 0 else ap - aq)
                lhs = _up(va_ref[i * kq:(i + 1) * kq, :])
            ti = (0, None, 1, 2, None, 3, 4)[i]
            if ti is None:
                rhs = bblk(0) if i == 1 else bblk(3)
            else:
                p, q, sign = RHS_TERMS[ti]
                bp, bq = bblk(p).astype(f32), bblk(q).astype(f32)
                rhs = (bp + bq if sign > 0 else bp - bq).astype(bf16)
            ms[i] = _dot_nt(lhs, rhs)
        for t, c in enumerate(_quadrants(*ms)):
            vt_ref[(t // 2) * kq:(t // 2 + 1) * kq, (t % 2) * m:(t % 2 + 1) * m] = _pk(c)

    def kv_acc(n, first=False):
        for j in range(NJ):
            r = _dot_nt(_up(vt_ref[j * 32:(j + 1) * 32, 0:n]), _up(phi_ref[j * 64:(j + 1) * 64, 0:n]))
            if first:
                kv_ref[j * 64:(j + 1) * 64, :] = r
            else:
                kv_ref[j * 64:(j + 1) * 64, :] += r

    def ln1(r0, n, ch):
        for r in range(0, n, ch):
            m = min(ch, n - r)
            xn_ref[r:r + m, :] = _ln(x_v[pl.ds(r0 + r, m), :].astype(f32))

    def sq_rhs(w_v, i):
        w_v = fresh(w_v, i)
        blk = lambda t: w_v[(t // 2) * KH:(t // 2 + 1) * KH, (t % 2) * KH:(t % 2 + 1) * KH]
        ti = (0, None, 1, 2, None, 3, 4)[i]
        if ti is None:
            return blk(0) if i == 1 else blk(3)
        p, q, sign = RHS_TERMS[ti]
        bp, bq = blk(p).astype(f32), blk(q).astype(f32)
        return (bp + bq if sign > 0 else bp - bq).astype(bf16)

    def sq_strassen(blk, w_v):
        ms = [None] * 7
        for i in W2ORD:
            p, q, sign = LHS_TERMS[i]
            lhs = blk(p) if q is None else (blk(p) + blk(q) if sign > 0 else blk(p) - blk(q))
            ms[i] = _dot(lhs.astype(bf16), sq_rhs(w_v, i))
        return _quadrants(*ms)

    def mix_in(r0, n):
        m = n // 2
        blk = lambda t: xn_ref[(t // 2) * m:(t // 2 + 1) * m, (t % 2) * KH:(t % 2 + 1) * KH]
        cq = sq_strassen(blk, w1_v)
        for t in (2, 1, 3, 0):
            h = _gelu(cq[t])
            for q in range(2):
                h_ref[2 * (t % 2) + q, pl.ds(PAD + r0 + (t // 2) * m, m), :] = h[:, q * 128:(q + 1) * 128]

    def mix_out(r0, n):
        m = n // 2

        def blk(t):
            return jnp.concatenate(
                [h_ref[q, pl.ds(PAD + r0 + (t // 2) * m + SHIFTS[q], m), :]
                 for q in (2 * (t % 2), 2 * (t % 2) + 1)], axis=1)

        cs = sq_strassen(blk, w2_v)
        for t in (2, 1, 3, 0):
            rows, cols = pl.ds(r0 + (t // 2) * m, m), slice((t % 2) * KH, (t % 2 + 1) * KH)
            x1_ref[rows, cols] = x_v[rows, cols].astype(f32) + cs[t]

    sa_dyn = sa_ref.at[pl.ds(pl.multiple_of(zero * 8, 8), 9 * HH)] if LDYN else sa_ref

    def ln2(r0, a, b):
        views = [x1_ref.at[pl.ds(pl.multiple_of(r0 + zero * (8 * p), 8), T2)] for p in range(3)]

        def norm(r):
            m = jnp.mean(views[0][r:r + L2R, :], axis=-1, keepdims=True)
            xc = views[1][r:r + L2R, :] - m
            v4 = jnp.sum(xc * xc, axis=-1, keepdims=True) * (4.0 / D)
            rs = jnp.exp2((-0.5 * LOG2E) * jnp.log(v4 + 4e-5))
            return (views[2][r:r + L2R, :] - m) * rs

        if FUSE:
            for r in range(0, HC, L2R):
                ya, yb = norm(r), norm(HC + r)
                quads = (ya[:, :KH], ya[:, KH:], yb[:, :KH], yb[:, KH:])
                for i, s in enumerate(quads + _lhs_sums(*quads)):
                    sa_dyn[i * HH + r // 2:i * HH + (r + L2R) // 2, :] = _pk(s)
        else:
            for r in range(a, b, L2R):
                x1n_ref[r:r + L2R, :] = norm(r)

    def sa_build(i):
        if FUSE:
            return
        p, q, sign = (i, None, 1) if i < 4 else SUM_TERMS[i - 4]
        for r in range(0, HC, SBR):
            blk = lambda t: x1n_ref[(t // 2) * HC + r:(t // 2) * HC + r + SBR, (t % 2) * KH:(t % 2 + 1) * KH]
            s = blk(p) if q is None else (blk(p) + blk(q) if sign > 0 else blk(p) - blk(q))
            sa_ref[i * HH + r // 2:i * HH + (r + SBR) // 2, :] = _pk(s)

    def w4_sum(i):
        p, q, sign = RHS_TERMS[i]
        for k0 in range(0, FH, WC):
            blk = lambda t: w4_v[(t // 2) * FH + k0:(t // 2) * FH + k0 + WC,
                                 (t % 2) * KH:(t % 2 + 1) * KH].astype(f32)
            s = blk(p) + blk(q) if sign > 0 else blk(p) - blk(q)
            t4_ref[i * FQ + k0 // 2:i * FQ + (k0 + WC) // 2, :] = _pk(s)

    c_wk.wait()
    c_wv.start()
    c_w1.start()
    fold(wk_v, MQ // 2)
    c_x0.wait()
    for c in c_loop1:
        c.start()
    phi_k(0, T0, first=True)
    c_x1.wait()
    c_wv.wait()
    for c in c_late:
        c.start()
    wt_ref[MQ:MQ + D // 2, :] = _pk(wv_v[...].T)
    phi_k(T0, P0 - T0, off=T0)
    ln1(0, P0 + AH, 2 * LN_ROWS)
    v_proj(0, P0, first=True)
    c_w1.wait()
    mix_in(0, P0 + AH)
    kv_acc(P0, first=True)
    for c in c_loop1:
        c.wait()

    def phase1(i, carry):
        r0 = pl.multiple_of(P0 + i * T1, 256)
        mix_out(pl.multiple_of(i * R2, R2), R2)
        phi_k(r0, T1)
        ln1(r0 + AH, T1, LN_ROWS)
        v_proj(r0, T1)
        mix_in(r0 + AH, T1)
        kv_acc(T1)
        return carry

    lax.fori_loop(0, N1, phase1, 0)

    for c in c_late:
        c.wait()
    mix_out(N1 * R2, R2 * (2 - MID2))
    fold(wq_v, 0)
    if PIPE:
        ln2(0, 0, T2)
    z_ref[...] = jnp.broadcast_to(jnp.sum(z_ref[...], axis=1, keepdims=True), z_ref.shape)
    for n0 in range(0, FH, 64):
        big_ref[7 * HH + n0 // 2:7 * HH + n0 // 2 + 32, 0:KH] = _pk(w3t_v[n0:n0 + 64, 0:KH])
    lane4 = lax.broadcasted_iota(jnp.int32, (DH, 128), 1) & 3
    for h in range(H):
        kvt_ref[h * 8:(h + 1) * 8, :] = _pk(
            jnp.where(lane4 == (h % 4), kv_ref[h * DH:(h + 1) * DH, :], 0.0))
    if MID2:
        mix_out((N1 + 1) * R2, R2)

    def phi_q(r0):
        pq = _dot_nt(_up(wt_ref[0:MQ // 2, :]), x_v[pl.ds(r0, T2), :])
        for c in range(T2 // 128):
            cs = slice(c * 128, (c + 1) * 128)
            for j in range(NJ):
                zp = z_ref[j * 128:j * 128 + 64, :].reshape(8, 8, 128)
                zn = z_ref[j * 128 + 64:(j + 1) * 128, :].reshape(8, 8, 128)
                ep, en, rp, rn = _dual_exp(_logits(pq, j, c))
                den = jnp.sum(ep * zp, axis=0) * rp + jnp.sum(en * zn, axis=0) * rn
                rd = _recip(_fold4(den, jnp.add) + 1e-6)
                phi_ref[j * 64:j * 64 + 32, cs] = _pk((ep * (rp * rd)[None]).reshape(64, 128))
                phi_ref[j * 64 + 32:(j + 1) * 64, cs] = _pk((en * (rn * rd)[None]).reshape(64, 128))

    def mlp_in_tail(k):
        rs = slice(k * HC // 2, (k + 1) * HC // 2)
        xh = jnp.concatenate([sa_ref[2 * k * HH:(2 * k + 1) * HH, :], sa_ref[(2 * k + 1) * HH:(2 * k + 2) * HH, :]], axis=1)
        ut = _gelu(_dot_nt(w3t_v[FM:F, :], _up(xh)))
        ut = jnp.concatenate([ut, jnp.zeros((128 - (F - FM), HC), f32)], axis=0)
        ur_ref[rs, :] = _pk(ut.T)[:, 0:F - FM]

    def mlp_dots(n0, nb):
        def lhs(i):
            if n0 == 0:
                sa_build(i)
            return _up(sa_ref[i * HH:(i + 1) * HH, :])

        blk = lambda t: w3t_v[(t % 2) * FH + n0:(t % 2) * FH + n0 + nb, (t // 2) * KH:(t // 2 + 1) * KH]

        def rsum(i):
            p, q, sign = RHS_TERMS[i]
            w = fresh(w3t_v, i)
            blk = lambda t: w[(t % 2) * FH + n0:(t % 2) * FH + n0 + nb, (t // 2) * KH:(t // 2 + 1) * KH]
            bp, bq = blk(p).astype(f32), blk(q).astype(f32)
            return (bp + bq if sign > 0 else bp - bq).astype(bf16)

        m2 = _dot_nt(lhs(5), _up(big_ref[7 * HH + n0 // 2:7 * HH + (n0 + nb) // 2, 0:KH]))
        m4 = _dot_nt(lhs(3), rsum(2))
        m1 = _dot_nt(lhs(4), rsum(0))
        m3 = _dot_nt(lhs(0), rsum(1))
        m5 = _dot_nt(lhs(6), blk(3))
        m6 = _dot_nt(lhs(7), rsum(3))
        m7 = _dot_nt(lhs(8), rsum(4))
        return [m1, m2, m3, m4, m5, m6, m7]

    act_ref = big_ref.at[pl.ds(pl.multiple_of(zero * 8, 8), 7 * HH)]

    def mlp_act(ms, n0, nb):
        for r in range(0, HC, AR):
            u11, u12, u21, u22 = (_gelu(c) for c in _quadrants(*[m[r:r + AR] for m in ms]))
            s1, s2, s5, s6, s7 = _lhs_sums(u11, u12, u21, u22)
            for i, s in enumerate((s1, s2, u11, u22, s5, s6, s7)):
                act_ref[i * HH + r // 2:i * HH + (r + AR) // 2, n0:n0 + nb] = _pk(s)

    def attn_out(r0, h):
        cs = slice(h * AC, (h + 1) * AC)
        ot = [_dot(_up(kvt_ref[j * 32:(j + 1) * 32, :]), _up(phi_ref[j * 64:(j + 1) * 64, cs]))
              for j in range(NJ)]
        o_ref[h * AC:(h + 1) * AC, :] = jnp.concatenate(ot, axis=0).T

    def attn_mix(off, n):
        m = n // 2
        blk = lambda t: o_ref[off + (t // 2) * m:off + (t // 2 + 1) * m, (t % 2) * KH:(t % 2 + 1) * KH]
        for t, c in enumerate(sq_strassen(blk, wo_v)):
            acc_ref[off + (t // 2) * m:off + (t // 2 + 1) * m, (t % 2) * KH:(t % 2 + 1) * KH] = c

    def phase2(t, carry):
        r0 = pl.multiple_of(t * T2, T2)
        r_next = pl.multiple_of(((t + 1) & (NT2 - 1)) * T2, T2)
        phi_q(r0)
        for h in range(T2 // AC):
            attn_out(r0, h)
        if not PIPE:
            ln2(r0, 0, T2)
        for k in range(T2 // WOC):
            attn_mix(k * WOC, WOC)
        prev = None
        for n0 in range(0, FH, NB):
            cur = (mlp_dots(n0, min(NB, FH - n0)), n0, min(NB, FH - n0))
            if prev is not None:
                mlp_act(*prev)
            prev = cur
        sa_build(1)
        sa_build(2)
        mlp_in_tail(0)
        mlp_in_tail(1)
        mlp_act(*prev)
        off = 0
        for k, n in enumerate(OUT_CHUNKS):
            if PIPE and k < 2:
                ln2(r_next, k * HC, (k + 1) * HC)
            rems, gates = [], []
            gw = gw_v[...].astype(f32).reshape(1, D)
            for half in range(2):
                o2 = off + half * HC
                rems.append(_dot(_up(ur_ref[o2 // 2:(o2 + n) // 2, :]), w4_v[FM:F, :]))
                gl = jnp.sum(x_v[pl.ds(r0 + o2, n), :].astype(f32) * gw, axis=-1, keepdims=True)
                gates.append(0.5 * jnp.tanh(0.5 * gl) + 0.5)
            ms = [None] * 7
            for i in W4ORD:
                ti = (0, None, 1, 2, None, 3, 4)[i]
                if ti is None:
                    rhs = w4_v[0:FH, 0:KH] if i == 1 else w4_v[FH:FM, KH:D]
                else:
                    if k == 0:
                        w4_sum(ti)
                    rhs = _up(t4_ref[ti * FQ:(ti + 1) * FQ, :])
                ms[i] = _dot(_up(big_ref[i * HH + off // 2:i * HH + (off + n) // 2, :]), rhs)
            cq = _quadrants(*ms)
            for q in (2, 1, 3, 0):
                c = cq[q]
                half, cs = q // 2, slice((q % 2) * KH, (q % 2 + 1) * KH)
                o2 = off + half * HC
                rows = pl.ds(r0 + o2, n)
                b = x1_ref[rows, cs] + rems[half][:, cs] + c
                out_v[rows, cs] = (b + gates[half] * (acc_ref[o2:o2 + n, cs] - b)).astype(bf16)
            for half in (1, 0):
                rows = pl.ds(r0 + off + half * HC, n)
                copy(out_v.at[rows], out_hbm.at[rows], 0).start()
            off += n
        return carry

    lax.fori_loop(0, NT2, phase2, 0)
    copy(out_v, out_hbm, 0).wait()


def _kernel(*refs):
    trips = refs[-1]
    trips[0] = 1

    def once(i, carry):
        _body(i, *refs[:-1])
        return carry

    lax.fori_loop(0, trips[0], once, 0)


@jax.jit
def pallas_gated_mix__linear_kernel_hedgehog__mixer_s_mlp__prompt_kernel(
        A_x, A_wqkv, A_w_phi, A_wo, B_x, B_w1, B_w2, B_w3, B_w4, gate_w):
    del B_x
    x = A_x.reshape(S, D)
    wphi = jnp.transpose(A_w_phi, (1, 2, 0)).reshape(DH * DH, H)
    w3t = B_w3.T
    hbm = pl.BlockSpec(memory_space=pl.ANY)
    out = pl.pallas_call(
        _kernel,
        out_shape=jax.ShapeDtypeStruct((S, D), bf16),
        in_specs=[hbm] * 9,
        out_specs=hbm,
        scratch_shapes=[
            pltpu.VMEM((S + AH, D), bf16),
            pltpu.VMEM((D, D), bf16),
            pltpu.VMEM((D, D), bf16),
            pltpu.VMEM((D, D), bf16),
            pltpu.VMEM((DH * DH, H), bf16),
            pltpu.VMEM((D, D), bf16),
            pltpu.VMEM((D, D), bf16),
            pltpu.VMEM((D, D), bf16),
            pltpu.VMEM((F, D), bf16),
            pltpu.VMEM((F, D), bf16),
            pltpu.VMEM((D,), bf16),
            pltpu.VMEM((S, D), bf16),
            pltpu.VMEM((MQ + D // 2, D), u32),
            pltpu.VMEM((4, PAD + S + AH, 128), f32),
            pltpu.VMEM((D, 128), f32),
            pltpu.VMEM((NJ * 128, 128), f32),
            pltpu.VMEM((D // 2, 128), u32),
            pltpu.VMEM((NJ * 64, T2), u32),
            pltpu.VMEM((64, D), u32),
            pltpu.VMEM((T1, D), f32),
            pltpu.VMEM((D // 2, T1), u32),
            pltpu.VMEM((S, D), f32),
            pltpu.VMEM((9 * HH + 8, KH), u32),
            pltpu.VMEM((7 * HH + FQ, FH), u32),
            pltpu.VMEM((T2 // 2, F - FM), u32),
            pltpu.VMEM((5 * FQ, KH), u32),
            pltpu.VMEM((T2, D), f32),
            pltpu.VMEM((T2, D), f32),
            pltpu.VMEM((T2 + 8, D), f32),
            pltpu.VMEM((7 * KH // 2, KH), u32),
            pltpu.SemaphoreType.DMA((4,)),
            pltpu.SMEM((1,), jnp.int32),
        ],
        compiler_params=pltpu.CompilerParams(vmem_limit_bytes=100 * 1024 * 1024, disable_bounds_checks=True),
    )(x, A_wqkv, wphi, A_wo, B_w1, B_w2, w3t, B_w4, gate_w)
    return out.reshape(1, S, D)
```

```python
import jax
import jax.numpy as jnp
from jax import lax
import jax.experimental.pallas as pl
import jax.experimental.pallas.tpu as pltpu

S, D, H, DH, F = 2048, 512, 32, 16, 1376
NJ = 8
MQ = 480
T0 = 384
P0 = 512
T1 = 768
N1 = (S - P0) // T1
R2 = 512
T2 = 1024
NT2 = S // T2
HC = 512
FM = 1280
AH = 32
PAD = 8
OUT_CHUNKS = tuple(int(v) for v in '224,160,96,32'.split(','))
KH = D // 2
LHS_TERMS = ((0, 3, 1), (2, 3, 1), (0, None, 1), (3, None, 1), (0, 1, 1), (2, 0, -1), (1, 3, -1))
W2ORD = [int(v) for v in '1,3,2,4,0,5,6'.split(',')]
AC = int(512)
WOC = int(512)
PIPE = int(0)
MID2 = int(1)
W4ORD = [int(v) for v in '1,3,2,4,0,5,6'.split(',')]
LDYN = int(0)
L2R = int(16)
VSTR = int(1)
FRESH = int(1)
FUSE = int(0)
ASSOC = int(1)
W3O = int(1)
VORD = [int(v) for v in '1,3,2,4,0,5,6'.split(',')]
VORD0 = [int(v) for v in '1,3,0,2,4,5,6'.split(',')]
ANR = int(0)
PRE1 = int(1)
SBR = int(64)
SUM_TERMS = ((0, 3, 1), (2, 3, 1), (0, 1, 1), (2, 0, -1), (1, 3, -1))
LNPOS = int(0)
RHS_TERMS = ((0, 3, 1), (1, 3, -1), (2, 0, -1), (0, 1, 1), (2, 3, 1))
WC = int(16)
AR = int(16)
FH = FM // 2
FQ = FH // 2
HH = HC // 2
NB = int(128)
WPRE = int(0)
LN_ROWS = 16
LOG2E = 1.4426950408889634
NT_DIMS = (((1,), (1,)), ((), ()))
SHIFTS = (-1, 1, -2, 2)
f32 = jnp.float32
bf16 = jnp.bfloat16
u32 = jnp.uint32


def _pk(x):
    return pltpu.bitcast(x.astype(bf16), u32)


def _up(x):
    return pltpu.bitcast(x, bf16)


def _dot(a, b):
    return jnp.dot(a, b, preferred_element_type=f32)


def _dot_nt(a, b):
    return lax.dot_general(a, b, NT_DIMS, preferred_element_type=f32)


def _gelu(hx):
    c = 0.7978845608028654
    t = jnp.tanh(hx * (2.0 * c + (8.0 * c * 0.044715) * (hx * hx)))
    return hx + hx * t


def _half_rstd(v):
    return jnp.exp2((-0.5 * LOG2E) * jnp.log(4.0 * v + 4e-5))


def _ln(x):
    m = jnp.mean(x, axis=-1, keepdims=True)
    xc = x - m
    v4 = jnp.sum(xc * xc, axis=-1, keepdims=True) * (4.0 / D)
    return xc * jnp.exp2((-0.5 * LOG2E) * jnp.log(v4 + 4e-5))


def _recip(x):
    r = pl.reciprocal(x, approx=True)
    return r * (2.0 - x * r)


def _fold4(a, op):
    return op(a, pltpu.roll(a, 4, 0))


def _dual_exp(p):
    mx = _fold4(jnp.max(p, axis=0), jnp.maximum)
    mn = _fold4(jnp.min(p, axis=0), jnp.minimum)
    ep = jnp.exp2(p - mx[None])
    en = jnp.exp2(mn[None] - p)
    rp = _recip(_fold4(jnp.sum(ep, axis=0), jnp.add))
    rn = _recip(_fold4(jnp.sum(en, axis=0), jnp.add))
    return ep, en, rp, rn


def _lhs_sums(a11, a12, a21, a22):
    return (a11 + a22, a21 + a22, a11 + a12, a21 - a11, a12 - a22)


def _rhs_sums(b11, b12, b21, b22):
    b11, b12, b21, b22 = (b.astype(f32) for b in (b11, b12, b21, b22))
    return (b11 + b22, b12 - b22, b21 - b11, b11 + b12, b21 + b22)


def _quadrants(m1, m2, m3, m4, m5, m6, m7):
    if ASSOC:
        return m4 - m5 + m1 + m7, m3 + m5, m2 + m4, m3 - m2 + m1 + m6
    return m1 + m4 - m5 + m7, m3 + m5, m2 + m4, m1 - m2 + m3 + m6


def _logits(pm, j, c):
    lo = lax.broadcasted_iota(jnp.int32, (8, 128), 0) < 4
    g, jj = j // 2, j % 2
    cs = slice(c * 128, (c + 1) * 128)
    own = pm[g * 120 + jj * 64:g * 120 + jj * 64 + 56, cs].reshape(7, 8, 128)
    sh = pm[g * 120 + 56:g * 120 + 64, cs]
    last = jnp.where(lo, sh, 0.0) if jj == 0 else jnp.where(lo, 0.0, sh)
    return jnp.concatenate([own, last[None]], axis=0)


def _body(zero, x_hbm, wqkv_hbm, wphi_hbm, wo_hbm, w1_hbm, w2_hbm, w3t_hbm, w4_hbm, gw_hbm,
          out_hbm,
          x_v, wq_v, wk_v, wv_v, wphi_v, wo_v, w1_v, w2_v, w3t_v, w4_v, gw_v, out_v,
          wt_ref, h_ref, kv_ref, z_ref, phi_ref, p_ref, xn_ref, vt_ref,
          x1_ref, sa_ref, big_ref, ur_ref, t4_ref, o_ref, acc_ref, x1n_ref, va_ref, t1_ref, sem):
    def copy(src, dst, k):
        return pltpu.make_async_copy(src, dst, sem.at[k])

    def xcopy(a, b, k):
        return copy(x_hbm.at[a:b], x_v.at[a:b], k)

    c_phi = copy(wphi_hbm, wphi_v, 0)
    c_wk = copy(wqkv_hbm.at[:, D:2 * D], wk_v, 1)
    c_x0 = xcopy(0, T0, 2)
    c_x1 = xcopy(T0, P0 + AH, 3)
    c_wv = copy(wqkv_hbm.at[:, 2 * D:3 * D], wv_v, 3)
    c_w1 = copy(w1_hbm, w1_v, 1)
    c_loop1 = [copy(w2_hbm, w2_v, 2), xcopy(P0 + AH, S, 2)]
    c_late = [copy(wqkv_hbm.at[:, 0:D], wq_v, 3), copy(w3t_hbm, w3t_v, 3), copy(w4_hbm, w4_v, 3),
              copy(wo_hbm, wo_v, 3), copy(gw_hbm, gw_v, 3)]
    c_phi.start()
    c_wk.start()

    x_v[S:S + AH, :] = jnp.zeros((AH, D), bf16)
    for q in range(4):
        h_ref[q, 0:PAD, :] = jnp.zeros((PAD, 128), f32)

    c_phi.wait()
    c_x0.start()
    c_x1.start()
    sel = (lax.broadcasted_iota(jnp.int32, (H, D), 0)
           == lax.broadcasted_iota(jnp.int32, (H, D), 1) // DH)
    bm = _dot(wphi_v[...], jnp.where(sel, 1.0, 0.0).astype(bf16))
    dmask = (lax.broadcasted_iota(jnp.int32, (DH * DH, D), 0) // DH
             == lax.broadcasted_iota(jnp.int32, (DH * DH, D), 1) % DH)
    cm = jnp.sum(jnp.where(dmask, bm, 0.0).reshape(DH, DH, D), axis=0).astype(bf16)
    e3 = ((lax.broadcasted_iota(jnp.int32, (128, DH), 0) % 64) // 4
          == lax.broadcasted_iota(jnp.int32, (128, DH), 1))
    pall = _dot(jnp.where(e3, 1.0, 0.0).astype(bf16), cm)
    rr = lax.broadcasted_iota(jnp.int32, (128, D), 0)
    cc = lax.broadcasted_iota(jnp.int32, (128, D), 1)
    pmask = ((cc // DH) % 8) == ((rr // 64) * 4 + rr % 4)
    p_ref[...] = _pk(jnp.where(pmask, pall, 0.0))

    def fresh(ref, k):
        if not FRESH:
            return ref
        return ref.at[pl.ds(pl.multiple_of(zero * (16 * (k + 1)), 16), ref.shape[0])]

    def fold(w_v, base):
        lo = lax.broadcasted_iota(jnp.int32, (8, D), 0) < 4
        for gp in range(2):
            rows = []
            for g in (2 * gp, 2 * gp + 1):
                gs = slice(g * 128, (g + 1) * 128)
                wt = _dot_nt(_up(p_ref[:, gs]), w_v[:, gs])
                ds = []
                for jj in range(2):
                    a = wt[jj * 64:(jj + 1) * 64, :].reshape(8, 8, D)
                    f15 = jnp.where(lo, pltpu.roll(a[7], 4, 0), a[7])
                    ds.append((a - f15[None]) * LOG2E)
                f14 = jnp.where(lo, ds[0][7], pltpu.roll(ds[1][7], 4, 0))
                rows += [ds[0][0:7].reshape(56, D), f14, ds[1][0:7].reshape(56, D)]
            wt_ref[base + gp * 120:base + (gp + 1) * 120, :] = _pk(jnp.concatenate(rows, axis=0))

    def phi_k(r0, n, off=0, first=False):
        pk = _dot_nt(_up(wt_ref[MQ // 2:MQ, :]), x_v[pl.ds(r0, n), :])
        for c in range(n // 128):
            cs = slice(off + c * 128, off + (c + 1) * 128)
            for j in range(NJ):
                ep, en, rp, rn = _dual_exp(_logits(pk, j, c))
                ep = (ep * rp[None]).reshape(64, 128)
                en = (en * rn[None]).reshape(64, 128)
                if first and c == 0:
                    z_ref[j * 128:j * 128 + 64, :] = ep
                    z_ref[j * 128 + 64:(j + 1) * 128, :] = en
                else:
                    z_ref[j * 128:j * 128 + 64, :] += ep
                    z_ref[j * 128 + 64:(j + 1) * 128, :] += en
                phi_ref[j * 64:j * 64 + 32, cs] = _pk(ep)
                phi_ref[j * 64 + 32:(j + 1) * 64, cs] = _pk(en)

    def v_proj(r0, n, first=False):
        if not VSTR:
            vt_ref[:, 0:n] = _pk(_dot_nt(_up(wt_ref[MQ:MQ + D // 2, :]), x_v[pl.ds(r0, n), :]))
            return
        m, kq = n // 2, KH // 2
        ablk = lambda t: _up(wt_ref[MQ + (t // 2) * kq:MQ + (t // 2 + 1) * kq, (t % 2) * KH:(t % 2 + 1) * KH])
        ms = [None] * 7
        for i in (VORD0 if first else VORD):
            ri = r0 + zero * (16 * (i + 1)) if FRESH else r0
            bblk = lambda t: x_v[pl.ds(pl.multiple_of(ri + (t % 2) * m, 16), m), (t // 2) * KH:(t // 2 + 1) * KH]
            p, q, sign = LHS_TERMS[i]
            if q is None:
                lhs = ablk(p)
            else:
                if first:
                    ap, aq = ablk(p).astype(f32), ablk(q).astype(f32)
                    va_ref[i * kq:(i + 1) * kq, :] = _pk(ap + aq if sign > 0 else ap - aq)
                lhs = _up(va_ref[i * kq:(i + 1) * kq, :])
            ti = (0, None, 1, 2, None, 3, 4)[i]
            if ti is None:
                rhs = bblk(0) if i == 1 else bblk(3)
            else:
                p, q, sign = RHS_TERMS[ti]
                bp, bq = bblk(p).astype(f32), bblk(q).astype(f32)
                rhs = (bp + bq if sign > 0 else bp - bq).astype(bf16)
            ms[i] = _dot_nt(lhs, rhs)
        for t, c in enumerate(_quadrants(*ms)):
            vt_ref[(t // 2) * kq:(t // 2 + 1) * kq, (t % 2) * m:(t % 2 + 1) * m] = _pk(c)

    def kv_acc(n, first=False):
        for j in range(NJ):
            r = _dot_nt(_up(vt_ref[j * 32:(j + 1) * 32, 0:n]), _up(phi_ref[j * 64:(j + 1) * 64, 0:n]))
            if first:
                kv_ref[j * 64:(j + 1) * 64, :] = r
            else:
                kv_ref[j * 64:(j + 1) * 64, :] += r

    def ln1(r0, n, ch):
        for r in range(0, n, ch):
            m = min(ch, n - r)
            xn_ref[r:r + m, :] = _ln(x_v[pl.ds(r0 + r, m), :].astype(f32))

    def sq_rhs(w_v, i):
        w_v = fresh(w_v, i)
        blk = lambda t: w_v[(t // 2) * KH:(t // 2 + 1) * KH, (t % 2) * KH:(t % 2 + 1) * KH]
        ti = (0, None, 1, 2, None, 3, 4)[i]
        if ti is None:
            return blk(0) if i == 1 else blk(3)
        p, q, sign = RHS_TERMS[ti]
        bp, bq = blk(p).astype(f32), blk(q).astype(f32)
        return (bp + bq if sign > 0 else bp - bq).astype(bf16)

    def sq_strassen(blk, w_v, keep=None, build=True):
        ms = [None] * 7
        for i in W2ORD:
            p, q, sign = LHS_TERMS[i]
            lhs = blk(p) if q is None else (blk(p) + blk(q) if sign > 0 else blk(p) - blk(q))
            if keep is None or i in (1, 4):
                rhs = sq_rhs(w_v, i)
            else:
                if build:
                    keep[i * (KH // 2):(i + 1) * (KH // 2), :] = _pk(sq_rhs(w_v, i))
                rhs = _up(keep[i * (KH // 2):(i + 1) * (KH // 2), :])
            ms[i] = _dot(lhs.astype(bf16), rhs)
        return _quadrants(*ms)

    def mix_in(r0, n, first=False):
        m = n // 2
        blk = lambda t: xn_ref[(t // 2) * m:(t // 2 + 1) * m, (t % 2) * KH:(t % 2 + 1) * KH]
        cq = sq_strassen(blk, w1_v, t1_ref if PRE1 else None, first)
        for t in (2, 1, 3, 0):
            h = _gelu(cq[t])
            for q in range(2):
                h_ref[2 * (t % 2) + q, pl.ds(PAD + r0 + (t // 2) * m, m), :] = h[:, q * 128:(q + 1) * 128]

    def mix_out(r0, n):
        m = n // 2

        def blk(t):
            return jnp.concatenate(
                [h_ref[q, pl.ds(PAD + r0 + (t // 2) * m + SHIFTS[q], m), :]
                 for q in (2 * (t % 2), 2 * (t % 2) + 1)], axis=1)

        cs = sq_strassen(blk, w2_v)
        for t in (2, 1, 3, 0):
            rows, cols = pl.ds(r0 + (t // 2) * m, m), slice((t % 2) * KH, (t % 2 + 1) * KH)
            x1_ref[rows, cols] = x_v[rows, cols].astype(f32) + cs[t]

    sa_dyn = sa_ref.at[pl.ds(pl.multiple_of(zero * 8, 8), 9 * HH)] if LDYN else sa_ref

    def ln2(r0, a, b):
        views = [x1_ref.at[pl.ds(pl.multiple_of(r0 + zero * (8 * p), 8), T2)] for p in range(3)]

        def norm(r):
            m = jnp.mean(views[0][r:r + L2R, :], axis=-1, keepdims=True)
            xc = views[1][r:r + L2R, :] - m
            v4 = jnp.sum(xc * xc, axis=-1, keepdims=True) * (4.0 / D)
            rs = jnp.exp2((-0.5 * LOG2E) * jnp.log(v4 + 4e-5))
            return (views[2][r:r + L2R, :] - m) * rs

        if FUSE:
            for r in range(0, HC, L2R):
                ya, yb = norm(r), norm(HC + r)
                quads = (ya[:, :KH], ya[:, KH:], yb[:, :KH], yb[:, KH:])
                for i, s in enumerate(quads + _lhs_sums(*quads)):
                    sa_dyn[i * HH + r // 2:i * HH + (r + L2R) // 2, :] = _pk(s)
        else:
            for r in range(a, b, L2R):
                x1n_ref[r:r + L2R, :] = norm(r)

    def sa_build(i):
        if FUSE:
            return
        p, q, sign = (i, None, 1) if i < 4 else SUM_TERMS[i - 4]
        for r in range(0, HC, SBR):
            blk = lambda t: x1n_ref[(t // 2) * HC + r:(t // 2) * HC + r + SBR, (t % 2) * KH:(t % 2 + 1) * KH]
            s = blk(p) if q is None else (blk(p) + blk(q) if sign > 0 else blk(p) - blk(q))
            sa_ref[i * HH + r // 2:i * HH + (r + SBR) // 2, :] = _pk(s)

    def w4_sum(i):
        p, q, sign = RHS_TERMS[i]
        for k0 in range(0, FH, WC):
            blk = lambda t: w4_v[(t // 2) * FH + k0:(t // 2) * FH + k0 + WC,
                                 (t % 2) * KH:(t % 2 + 1) * KH].astype(f32)
            s = blk(p) + blk(q) if sign > 0 else blk(p) - blk(q)
            t4_ref[i * FQ + k0 // 2:i * FQ + (k0 + WC) // 2, :] = _pk(s)

    c_wk.wait()
    c_wv.start()
    c_w1.start()
    fold(wk_v, MQ // 2)
    c_x0.wait()
    for c in c_loop1:
        c.start()
    phi_k(0, T0, first=True)
    c_x1.wait()
    c_wv.wait()
    for c in c_late:
        c.start()
    wt_ref[MQ:MQ + D // 2, :] = _pk(wv_v[...].T)
    for s in 'pk,ln,vf,W,w1,kv'.split(','):
        if s == 'pk': phi_k(T0, P0 - T0, off=T0)
        elif s == 'ln': ln1(0, P0 + AH, int(32))
        elif s == 'vf': v_proj(0, P0, first=True)
        elif s == 'W': c_w1.wait()
        elif s == 'w1': mix_in(0, P0 + AH, first=True)
        elif s == 'kv': kv_acc(P0, first=True)
    for c in c_loop1:
        c.wait()

    def phase1(i, carry):
        r0 = pl.multiple_of(P0 + i * T1, 256)
        mix_out(pl.multiple_of(i * R2, R2), R2)
        phi_k(r0, T1)
        ln1(r0 + AH, T1, int(16))
        v_proj(r0, T1)
        mix_in(r0 + AH, T1)
        kv_acc(T1)
        return carry

    lax.fori_loop(0, N1, phase1, 0)

    for c in c_late:
        c.wait()
    mix_out(N1 * R2, R2 * (2 - MID2))
    fold(wq_v, 0)
    if PIPE:
        ln2(0, 0, T2)
    z_ref[...] = jnp.broadcast_to(jnp.sum(z_ref[...], axis=1, keepdims=True), z_ref.shape)
    for b in range(FH // NB):
        big_ref[7 * HH + b * 8:7 * HH + (b + 1) * 8, 0:KH] = _pk(w3t_v[b * NB + ANR:b * NB + ANR + 16, 0:KH])
    if MID2:
        mix_out((N1 + 1) * R2, R2)

    def phi_q(r0):
        pq = _dot_nt(_up(wt_ref[0:MQ // 2, :]), x_v[pl.ds(r0, T2), :])
        for c in range(T2 // 128):
            cs = slice(c * 128, (c + 1) * 128)
            for j in range(NJ):
                zp = z_ref[j * 128:j * 128 + 64, :].reshape(8, 8, 128)
                zn = z_ref[j * 128 + 64:(j + 1) * 128, :].reshape(8, 8, 128)
                ep, en, rp, rn = _dual_exp(_logits(pq, j, c))
                den = jnp.sum(ep * zp, axis=0) * rp + jnp.sum(en * zn, axis=0) * rn
                rd = _recip(_fold4(den, jnp.add) + 1e-6)
                phi_ref[j * 64:j * 64 + 32, cs] = _pk((ep * (rp * rd)[None]).reshape(64, 128))
                phi_ref[j * 64 + 32:(j + 1) * 64, cs] = _pk((en * (rn * rd)[None]).reshape(64, 128))

    def mlp_in_tail(k):
        rs = slice(k * HC // 2, (k + 1) * HC // 2)
        xh = jnp.concatenate([sa_ref[2 * k * HH:(2 * k + 1) * HH, :], sa_ref[(2 * k + 1) * HH:(2 * k + 2) * HH, :]], axis=1)
        ut = _gelu(_dot_nt(w3t_v[FM:F, :], _up(xh)))
        ut = jnp.concatenate([ut, jnp.zeros((128 - (F - FM), HC), f32)], axis=0)
        ur_ref[rs, :] = _pk(ut.T)[:, 0:F - FM]

    def mlp_dots(n0, nb):
        def lhs(i):
            if n0 == 0:
                sa_build(i)
            return _up(sa_ref[i * HH:(i + 1) * HH, :])

        blk = lambda t: w3t_v[(t % 2) * FH + n0:(t % 2) * FH + n0 + nb, (t // 2) * KH:(t // 2 + 1) * KH]

        def rsum(i):
            p, q, sign = RHS_TERMS[i]
            w = fresh(w3t_v, i)
            blk = lambda t: w[(t % 2) * FH + n0:(t % 2) * FH + n0 + nb, (t // 2) * KH:(t // 2 + 1) * KH]
            bp, bq = blk(p).astype(f32), blk(q).astype(f32)
            return (bp + bq if sign > 0 else bp - bq).astype(bf16)

        an = 7 * HH + (n0 // NB) * 8
        parts = [w3t_v[n0:n0 + ANR, 0:KH]] if ANR else []
        parts.append(_up(big_ref[an:an + 8, 0:KH]))
        if ANR + 16 < nb:
            parts.append(w3t_v[n0 + ANR + 16:n0 + nb, 0:KH])
        m2 = _dot_nt(lhs(5), jnp.concatenate(parts, axis=0))
        m4 = _dot_nt(lhs(3), rsum(2))
        if not W3O:
            m1 = _dot_nt(lhs(4), rsum(0))
        m3 = _dot_nt(lhs(0), rsum(1))
        m5 = _dot_nt(lhs(6), blk(3))
        if W3O:
            m1 = _dot_nt(lhs(4), rsum(0))
        m6 = _dot_nt(lhs(7), rsum(3))
        m7 = _dot_nt(lhs(8), rsum(4))
        return [m1, m2, m3, m4, m5, m6, m7]

    act_ref = big_ref.at[pl.ds(pl.multiple_of(zero * 8, 8), 7 * HH)]

    def mlp_act(ms, n0, nb):
        for r in range(0, HC, AR):
            u11, u12, u21, u22 = (_gelu(c) for c in _quadrants(*[m[r:r + AR] for m in ms]))
            s1, s2, s5, s6, s7 = _lhs_sums(u11, u12, u21, u22)
            for i, s in enumerate((s1, s2, u11, u22, s5, s6, s7)):
                act_ref[i * HH + r // 2:i * HH + (r + AR) // 2, n0:n0 + nb] = _pk(s)

    def attn_out(r0, h):
        cs = slice(h * AC, (h + 1) * AC)
        own = ((lax.broadcasted_iota(jnp.int32, (64, 128), 1) & 3)
               == (lax.broadcasted_iota(jnp.int32, (64, 128), 0) >> 4))
        ot = [_dot(jnp.where(own, kv_ref[j * 64:(j + 1) * 64, :], 0.0).astype(bf16),
                   _up(phi_ref[j * 64:(j + 1) * 64, cs])) for j in range(NJ)]
        o_ref[h * AC:(h + 1) * AC, :] = jnp.concatenate(ot, axis=0).T

    def attn_mix(off, n):
        m = n // 2
        blk = lambda t: o_ref[off + (t // 2) * m:off + (t // 2 + 1) * m, (t % 2) * KH:(t % 2 + 1) * KH]
        for t, c in enumerate(sq_strassen(blk, wo_v)):
            acc_ref[off + (t // 2) * m:off + (t // 2 + 1) * m, (t % 2) * KH:(t % 2 + 1) * KH] = c

    def phase2(t, carry):
        r0 = pl.multiple_of(t * T2, T2)
        r_next = pl.multiple_of(((t + 1) & (NT2 - 1)) * T2, T2)
        phi_q(r0)
        for h in range(T2 // AC):
            attn_out(r0, h)
        if not PIPE:
            ln2(r0, 0, T2)
        for k in range(T2 // WOC):
            attn_mix(k * WOC, WOC)
        prev = None
        for n0 in range(0, FH, NB):
            cur = (mlp_dots(n0, min(NB, FH - n0)), n0, min(NB, FH - n0))
            if prev is not None:
                mlp_act(*prev)
            prev = cur
        sa_build(1)
        sa_build(2)
        mlp_in_tail(0)
        mlp_in_tail(1)
        mlp_act(*prev)
        off = 0
        for k, n in enumerate(OUT_CHUNKS):
            if PIPE and k < 2:
                ln2(r_next, k * HC, (k + 1) * HC)
            rems, gates = [], []
            gw = gw_v[...].astype(f32).reshape(1, D)
            for half in range(2):
                o2 = off + half * HC
                rems.append(_dot(_up(ur_ref[o2 // 2:(o2 + n) // 2, :]), w4_v[FM:F, :]))
                gl = jnp.sum(x_v[pl.ds(r0 + o2, n), :].astype(f32) * gw, axis=-1, keepdims=True)
                gates.append(0.5 * jnp.tanh(0.5 * gl) + 0.5)
            ms = [None] * 7
            for i in W4ORD:
                ti = (0, None, 1, 2, None, 3, 4)[i]
                if ti is None:
                    rhs = w4_v[0:FH, 0:KH] if i == 1 else w4_v[FH:FM, KH:D]
                else:
                    if k == 0:
                        w4_sum(ti)
                    rhs = _up(t4_ref[ti * FQ:(ti + 1) * FQ, :])
                ms[i] = _dot(_up(big_ref[i * HH + off // 2:i * HH + (off + n) // 2, :]), rhs)
            cq = _quadrants(*ms)
            for q in (2, 1, 3, 0):
                c = cq[q]
                half, cs = q // 2, slice((q % 2) * KH, (q % 2 + 1) * KH)
                o2 = off + half * HC
                rows = pl.ds(r0 + o2, n)
                b = x1_ref[rows, cs] + rems[half][:, cs] + c
                out_v[rows, cs] = (b + gates[half] * (acc_ref[o2:o2 + n, cs] - b)).astype(bf16)
            for half in (1, 0):
                rows = pl.ds(r0 + off + half * HC, n)
                copy(out_v.at[rows], out_hbm.at[rows], 0).start()
            off += n
        return carry

    lax.fori_loop(0, NT2, phase2, 0)
    copy(out_v, out_hbm, 0).wait()


def _kernel(*refs):
    trips = refs[-1]
    trips[0] = 1

    def once(i, carry):
        _body(i, *refs[:-1])
        return carry

    lax.fori_loop(0, trips[0], once, 0)


@jax.jit
def pallas_gated_mix__linear_kernel_hedgehog__mixer_s_mlp__prompt_kernel(
        A_x, A_wqkv, A_w_phi, A_wo, B_x, B_w1, B_w2, B_w3, B_w4, gate_w):
    del B_x
    x = A_x.reshape(S, D)
    wphi = jnp.transpose(A_w_phi, (1, 2, 0)).reshape(DH * DH, H)
    w3t = B_w3.T
    hbm = pl.BlockSpec(memory_space=pl.ANY)
    out = pl.pallas_call(
        _kernel,
        out_shape=jax.ShapeDtypeStruct((S, D), bf16),
        in_specs=[hbm] * 9,
        out_specs=hbm,
        scratch_shapes=[
            pltpu.VMEM((S + AH, D), bf16),
            pltpu.VMEM((D, D), bf16),
            pltpu.VMEM((D, D), bf16),
            pltpu.VMEM((D, D), bf16),
            pltpu.VMEM((DH * DH, H), bf16),
            pltpu.VMEM((D, D), bf16),
            pltpu.VMEM((D, D), bf16),
            pltpu.VMEM((D, D), bf16),
            pltpu.VMEM((F, D), bf16),
            pltpu.VMEM((F, D), bf16),
            pltpu.VMEM((D,), bf16),
            pltpu.VMEM((S, D), bf16),
            pltpu.VMEM((MQ + D // 2, D), u32),
            pltpu.VMEM((4, PAD + S + AH, 128), f32),
            pltpu.VMEM((D, 128), f32),
            pltpu.VMEM((NJ * 128, 128), f32),
            pltpu.VMEM((NJ * 64, T2), u32),
            pltpu.VMEM((64, D), u32),
            pltpu.VMEM((T1, D), f32),
            pltpu.VMEM((D // 2, T1), u32),
            pltpu.VMEM((S, D), f32),
            pltpu.VMEM((9 * HH + 8, KH), u32),
            pltpu.VMEM((7 * HH + FQ, FH), u32),
            pltpu.VMEM((T2 // 2, F - FM), u32),
            pltpu.VMEM((5 * FQ, KH), u32),
            pltpu.VMEM((T2, D), f32),
            pltpu.VMEM((T2, D), f32),
            pltpu.VMEM((T2 + 8, D), f32),
            pltpu.VMEM((7 * KH // 2, KH), u32),
            pltpu.VMEM((7 * KH // 2, KH), u32),
            pltpu.SemaphoreType.DMA((4,)),
            pltpu.SMEM((1,), jnp.int32),
        ],
        compiler_params=pltpu.CompilerParams(vmem_limit_bytes=100 * 1024 * 1024, disable_bounds_checks=True),
    )(x, A_wqkv, wphi, A_wo, B_w1, B_w2, w3t, B_w4, gate_w)
    return out.reshape(1, S, D)
```

```python
import jax
import jax.numpy as jnp
from jax import lax
import jax.experimental.pallas as pl
import jax.experimental.pallas.tpu as pltpu

S, D, H, DH, F = 2048, 512, 32, 16, 1376
NJ = 8
MQ = 480
T0 = 384
P0 = 512
T1 = 768
N1 = (S - P0) // T1
R2 = 512
T2 = 1024
NT2 = S // T2
HC = T2 // 2
FM = 1280
AH = 32
PAD = 8
NB = 128
OUT_CHUNKS = (224, 160, 96, 32)
KH, KQ = D // 2, D // 4
FH, FQ = FM // 2, FM // 4
HH = HC // 2
ANCHOR = 7 * HH
LOG2E = 1.4426950408889634
NT_DIMS = (((1,), (1,)), ((), ()))
SHIFTS = (-1, 1, -2, 2)
LHS_TERMS = ((0, 3, 1), (2, 3, 1), (0, None, 1), (3, None, 1), (0, 1, 1), (2, 0, -1), (1, 3, -1))
RHS_TERMS = ((0, 3, 1), (0, None, 1), (1, 3, -1), (2, 0, -1), (3, None, 1), (0, 1, 1), (2, 3, 1))
ORDER = (1, 3, 2, 4, 0, 5, 6)
DONE = (2, 1, 3, 0)
f32 = jnp.float32
bf16 = jnp.bfloat16
u32 = jnp.uint32


def _pk(x):
    return pltpu.bitcast(x.astype(bf16), u32)


def _up(x):
    return pltpu.bitcast(x, bf16)


def _dot(a, b):
    return jnp.dot(a, b, preferred_element_type=f32)


def _dot_nt(a, b):
    return lax.dot_general(a, b, NT_DIMS, preferred_element_type=f32)


def _gelu(hx):
    c = 0.7978845608028654
    t = jnp.tanh(hx * (2.0 * c + (8.0 * c * 0.044715) * (hx * hx)))
    return hx + hx * t


def _half_rstd(xc):
    v4 = jnp.sum(xc * xc, axis=-1, keepdims=True) * (4.0 / D)
    return jnp.exp2((-0.5 * LOG2E) * jnp.log(v4 + 4e-5))


def _recip(x):
    r = pl.reciprocal(x, approx=True)
    return r * (2.0 - x * r)


def _fold4(a, op):
    return op(a, pltpu.roll(a, 4, 0))


def _dual_exp(p):
    mx = _fold4(jnp.max(p, axis=0), jnp.maximum)
    mn = _fold4(jnp.min(p, axis=0), jnp.minimum)
    ep = jnp.exp2(p - mx[None])
    en = jnp.exp2(mn[None] - p)
    rp = _recip(_fold4(jnp.sum(ep, axis=0), jnp.add))
    rn = _recip(_fold4(jnp.sum(en, axis=0), jnp.add))
    return ep, en, rp, rn


def _logits(pm, j, c):
    lo = lax.broadcasted_iota(jnp.int32, (8, 128), 0) < 4
    g, jj = j // 2, j % 2
    cs = slice(c * 128, (c + 1) * 128)
    own = pm[g * 120 + jj * 64:g * 120 + jj * 64 + 56, cs].reshape(7, 8, 128)
    sh = pm[g * 120 + 56:g * 120 + 64, cs]
    last = jnp.where(lo, sh, 0.0) if jj == 0 else jnp.where(lo, 0.0, sh)
    return jnp.concatenate([own, last[None]], axis=0)


def _operand(blk, term):
    p, q, sign = term
    if q is None:
        return blk(p).astype(bf16)
    a, b = blk(p).astype(f32), blk(q).astype(f32)
    return (a + b if sign > 0 else a - b).astype(bf16)


def _products(lhs, rhs, dot, order=ORDER):
    ms = [None] * 7
    for i in order:
        a = lhs(i)
        ms[i] = dot(a, rhs(i))
    return ms


def _quadrants(m1, m2, m3, m4, m5, m6, m7):
    return m4 - m5 + m1 + m7, m3 + m5, m2 + m4, m3 - m2 + m1 + m6


def _half(t, n):
    return slice(t * n, (t + 1) * n)


def _body(zero, x_hbm, wqkv_hbm, wphi_hbm, wo_hbm, w1_hbm, w2_hbm, w3t_hbm, w4_hbm, gw_hbm,
          out_hbm,
          x_v, wq_v, wk_v, wv_v, wphi_v, wo_v, w1_v, w2_v, w3t_v, w4_v, gw_v, out_v,
          wt_ref, h_ref, kv_ref, z_ref, phi_ref, p_ref, xn_ref, vt_ref,
          x1_ref, sa_ref, u_ref, ur_ref, t4_ref, o_ref, a_ref, va_ref, t1_ref, sem):
    def copy(src, dst, k):
        return pltpu.make_async_copy(src, dst, sem.at[k])

    def xcopy(a, b, k):
        return copy(x_hbm.at[a:b], x_v.at[a:b], k)

    def fresh(ref, k):
        return ref.at[pl.ds(pl.multiple_of(zero * (16 * (k + 1)), 16), ref.shape[0])]

    def kept(ref, rows, i, build, make):
        if build:
            ref[_half(i, rows), :] = _pk(make())
        return _up(ref[_half(i, rows), :])

    c_phi = copy(wphi_hbm, wphi_v, 0)
    c_wk = copy(wqkv_hbm.at[:, D:2 * D], wk_v, 1)
    c_x0 = xcopy(0, T0, 2)
    c_x1 = xcopy(T0, P0 + AH, 3)
    c_wv = copy(wqkv_hbm.at[:, 2 * D:3 * D], wv_v, 3)
    c_w1 = copy(w1_hbm, w1_v, 1)
    c_loop1 = [copy(w2_hbm, w2_v, 2), xcopy(P0 + AH, S, 2)]
    c_late = [copy(wqkv_hbm.at[:, 0:D], wq_v, 3), copy(w3t_hbm, w3t_v, 3), copy(w4_hbm, w4_v, 3),
              copy(wo_hbm, wo_v, 3), copy(gw_hbm, gw_v, 3)]
    c_phi.start()
    c_wk.start()

    x_v[S:S + AH, :] = jnp.zeros((AH, D), bf16)
    for q in range(4):
        h_ref[q, 0:PAD, :] = jnp.zeros((PAD, 128), f32)

    c_phi.wait()
    c_x0.start()
    c_x1.start()
    sel = (lax.broadcasted_iota(jnp.int32, (H, D), 0)
           == lax.broadcasted_iota(jnp.int32, (H, D), 1) // DH)
    bm = _dot(wphi_v[...], jnp.where(sel, 1.0, 0.0).astype(bf16))
    dmask = (lax.broadcasted_iota(jnp.int32, (DH * DH, D), 0) // DH
             == lax.broadcasted_iota(jnp.int32, (DH * DH, D), 1) % DH)
    cm = jnp.sum(jnp.where(dmask, bm, 0.0).reshape(DH, DH, D), axis=0).astype(bf16)
    e3 = ((lax.broadcasted_iota(jnp.int32, (128, DH), 0) % 64) // 4
          == lax.broadcasted_iota(jnp.int32, (128, DH), 1))
    pall = _dot(jnp.where(e3, 1.0, 0.0).astype(bf16), cm)
    rr = lax.broadcasted_iota(jnp.int32, (128, D), 0)
    cc = lax.broadcasted_iota(jnp.int32, (128, D), 1)
    pmask = ((cc // DH) % 8) == ((rr // 64) * 4 + rr % 4)
    p_ref[...] = _pk(jnp.where(pmask, pall, 0.0))

    def fold(w_v, base):
        lo = lax.broadcasted_iota(jnp.int32, (8, D), 0) < 4
        for gp in range(2):
            rows = []
            for g in (2 * gp, 2 * gp + 1):
                wt = _dot_nt(_up(p_ref[:, _half(g, 128)]), w_v[:, _half(g, 128)])
                ds = []
                for jj in range(2):
                    a = wt[_half(jj, 64), :].reshape(8, 8, D)
                    f15 = jnp.where(lo, pltpu.roll(a[7], 4, 0), a[7])
                    ds.append((a - f15[None]) * LOG2E)
                f14 = jnp.where(lo, ds[0][7], pltpu.roll(ds[1][7], 4, 0))
                rows += [ds[0][0:7].reshape(56, D), f14, ds[1][0:7].reshape(56, D)]
            wt_ref[base + gp * 120:base + (gp + 1) * 120, :] = _pk(jnp.concatenate(rows, axis=0))

    def phi_k(r0, n, off=0, first=False):
        pk = _dot_nt(_up(wt_ref[MQ // 2:MQ, :]), x_v[pl.ds(r0, n), :])
        for c in range(n // 128):
            cs = slice(off + c * 128, off + (c + 1) * 128)
            for j in range(NJ):
                ep, en, rp, rn = _dual_exp(_logits(pk, j, c))
                ep = (ep * rp[None]).reshape(64, 128)
                en = (en * rn[None]).reshape(64, 128)
                if first and c == 0:
                    z_ref[_half(2 * j, 64), :] = ep
                    z_ref[_half(2 * j + 1, 64), :] = en
                else:
                    z_ref[_half(2 * j, 64), :] += ep
                    z_ref[_half(2 * j + 1, 64), :] += en
                phi_ref[_half(2 * j, 32), cs] = _pk(ep)
                phi_ref[_half(2 * j + 1, 32), cs] = _pk(en)

    def v_proj(r0, n, first=False):
        m = n // 2
        wblk = lambda t: _up(wt_ref[MQ + (t // 2) * KQ:MQ + (t // 2 + 1) * KQ, _half(t % 2, KH)])

        def lhs(i):
            if LHS_TERMS[i][1] is None:
                return wblk(LHS_TERMS[i][0])
            return kept(va_ref, KQ, i, first, lambda: _operand(wblk, LHS_TERMS[i]))

        def rhs(i):
            ri = r0 + zero * (16 * (i + 1))
            xblk = lambda t: x_v[pl.ds(pl.multiple_of(ri + (t % 2) * m, 16), m), _half(t // 2, KH)]
            return _operand(xblk, RHS_TERMS[i])

        ms = _products(lhs, rhs, _dot_nt, (1, 3, 0, 2, 4, 5, 6) if first else ORDER)
        for t, c in enumerate(_quadrants(*ms)):
            vt_ref[_half(t // 2, KQ), _half(t % 2, m)] = _pk(c)

    def kv_acc(n, first=False):
        for j in range(NJ):
            r = _dot_nt(_up(vt_ref[_half(j, 32), 0:n]), _up(phi_ref[_half(j, 64), 0:n]))
            if first:
                kv_ref[_half(j, 64), :] = r
            else:
                kv_ref[_half(j, 64), :] += r

    def ln1(r0, n, ch):
        for r in range(0, n, ch):
            x = x_v[pl.ds(r0 + r, ch), :].astype(f32)
            xc = x - jnp.mean(x, axis=-1, keepdims=True)
            xn_ref[r:r + ch, :] = xc * _half_rstd(xc)

    def times_square(blk, w_v, keep=None, build=False):
        def rhs(i):
            w = fresh(w_v, i)
            make = lambda: _operand(lambda t: w[_half(t // 2, KH), _half(t % 2, KH)], RHS_TERMS[i])
            if keep is None or RHS_TERMS[i][1] is None:
                return make()
            return kept(keep, KQ, i, build, make)

        return _quadrants(*_products(lambda i: _operand(blk, LHS_TERMS[i]), rhs, _dot))

    def mix_in(r0, n, first=False):
        m = n // 2
        cq = times_square(lambda t: xn_ref[_half(t // 2, m), _half(t % 2, KH)], w1_v, t1_ref, first)
        for t in DONE:
            h = _gelu(cq[t])
            for q in range(2):
                h_ref[2 * (t % 2) + q, pl.ds(PAD + r0 + (t // 2) * m, m), :] = h[:, _half(q, 128)]

    def mix_out(r0, n):
        m = n // 2

        def shifted(t):
            return jnp.concatenate(
                [h_ref[q, pl.ds(PAD + r0 + (t // 2) * m + SHIFTS[q], m), :]
                 for q in (2 * (t % 2), 2 * (t % 2) + 1)], axis=1)

        cq = times_square(shifted, w2_v)
        for t in DONE:
            rows, cols = pl.ds(r0 + (t // 2) * m, m), _half(t % 2, KH)
            x1_ref[rows, cols] = x_v[rows, cols].astype(f32) + cq[t]

    c_wk.wait()
    c_wv.start()
    c_w1.start()
    fold(wk_v, MQ // 2)
    c_x0.wait()
    for c in c_loop1:
        c.start()
    phi_k(0, T0, first=True)
    c_x1.wait()
    c_wv.wait()
    for c in c_late:
        c.start()
    wt_ref[MQ:MQ + D // 2, :] = _pk(wv_v[...].T)
    phi_k(T0, P0 - T0, off=T0)
    ln1(0, P0 + AH, 32)
    v_proj(0, P0, first=True)
    c_w1.wait()
    mix_in(0, P0 + AH, first=True)
    kv_acc(P0, first=True)
    for c in c_loop1:
        c.wait()

    def phase1(i, carry):
        r0 = pl.multiple_of(P0 + i * T1, 256)
        mix_out(pl.multiple_of(i * R2, R2), R2)
        phi_k(r0, T1)
        ln1(r0 + AH, T1, 16)
        v_proj(r0, T1)
        mix_in(r0 + AH, T1)
        kv_acc(T1)
        return carry

    lax.fori_loop(0, N1, phase1, 0)

    for c in c_late:
        c.wait()
    for q in (1, 3):
        h_ref[q, PAD + S:PAD + S + 8, :] = jnp.zeros((8, 128), f32)
    mix_out(N1 * R2, R2)
    fold(wq_v, 0)
    z_ref[...] = jnp.broadcast_to(jnp.sum(z_ref[...], axis=1, keepdims=True), z_ref.shape)
    for b in range(FH // NB):
        u_ref[ANCHOR + b * 8:ANCHOR + (b + 1) * 8, 0:KH] = _pk(w3t_v[b * NB:b * NB + 16, 0:KH])
    mix_out((N1 + 1) * R2, R2)

    def phi_q(r0):
        pq = _dot_nt(_up(wt_ref[0:MQ // 2, :]), x_v[pl.ds(r0, T2), :])
        for c in range(T2 // 128):
            for j in range(NJ):
                zp = z_ref[_half(2 * j, 64), :].reshape(8, 8, 128)
                zn = z_ref[_half(2 * j + 1, 64), :].reshape(8, 8, 128)
                ep, en, rp, rn = _dual_exp(_logits(pq, j, c))
                den = jnp.sum(ep * zp, axis=0) * rp + jnp.sum(en * zn, axis=0) * rn
                rd = _recip(_fold4(den, jnp.add) + 1e-6)
                phi_ref[_half(2 * j, 32), _half(c, 128)] = _pk((ep * (rp * rd)[None]).reshape(64, 128))
                phi_ref[_half(2 * j + 1, 32), _half(c, 128)] = _pk((en * (rn * rd)[None]).reshape(64, 128))

    def attn_out(k):
        own = ((lax.broadcasted_iota(jnp.int32, (64, 128), 1) & 3)
               == (lax.broadcasted_iota(jnp.int32, (64, 128), 0) >> 4))
        ot = [_dot(jnp.where(own, kv_ref[_half(j, 64), :], 0.0).astype(bf16),
                   _up(phi_ref[_half(j, 64), _half(k, HC)])) for j in range(NJ)]
        o_ref[_half(k, HC), :] = jnp.concatenate(ot, axis=0).T

    def attn_proj(k):
        cq = times_square(lambda t: o_ref[_half(2 * k + t // 2, HH), _half(t % 2, KH)], wo_v)
        for t, c in enumerate(cq):
            a_ref[_half(2 * k + t // 2, HH), _half(t % 2, KH)] = c

    def ln2(r0):
        views = [x1_ref.at[pl.ds(pl.multiple_of(r0 + zero * (8 * p), 8), T2)] for p in range(3)]

        def norm(r):
            m = jnp.mean(views[0][r:r + 16, :], axis=-1, keepdims=True)
            rs = _half_rstd(views[1][r:r + 16, :] - m)
            return (views[2][r:r + 16, :] - m) * rs

        for r in range(0, HC, 16):
            y = (norm(r), norm(HC + r))
            blk = lambda t: y[t // 2][:, _half(t % 2, KH)]
            for i, term in enumerate(LHS_TERMS + ((1, None, 1), (2, None, 1))):
                sa_ref[i * HH + r // 2:i * HH + r // 2 + 8, :] = _pk(_operand(blk, term))

    def mlp_products(b):
        n0 = b * NB

        def rhs(i):
            if i == ORDER[0]:
                head = _up(u_ref[ANCHOR + b * 8:ANCHOR + (b + 1) * 8, 0:KH])
                return jnp.concatenate([head, w3t_v[n0 + 16:n0 + NB, 0:KH]], axis=0)
            w = w3t_v if RHS_TERMS[i][1] is None else fresh(w3t_v, i)
            blk = lambda t: w[(t % 2) * FH + n0:(t % 2) * FH + n0 + NB, _half(t // 2, KH)]
            return _operand(blk, RHS_TERMS[i])

        return _products(lambda i: _up(sa_ref[_half(i, HH), :]), rhs, _dot_nt)

    act_ref = u_ref.at[pl.ds(pl.multiple_of(zero * 8, 8), ANCHOR)]

    def mlp_act(b, ms):
        for r in range(0, HC, 16):
            u = [_gelu(c) for c in _quadrants(*[m[r:r + 16] for m in ms])]
            for i, term in enumerate(LHS_TERMS):
                act_ref[i * HH + r // 2:i * HH + r // 2 + 8, _half(b, NB)] = _pk(
                    _operand(lambda t: u[t], term))

    def mlp_tail(k):
        xh = jnp.concatenate([sa_ref[_half(i, HH), :] for i in ((2, 7), (8, 3))[k]], axis=1)
        ut = _gelu(_dot_nt(w3t_v[FM:F, :], _up(xh)))
        ut = jnp.concatenate([ut, jnp.zeros((128 - (F - FM), HC), f32)], axis=0)
        ur_ref[_half(k, HH), :] = _pk(ut.T)[:, 0:F - FM]

    def w4_operand(i, build):
        if RHS_TERMS[i][1] is None:
            t = RHS_TERMS[i][0]
            return w4_v[_half(t // 2, FH), _half(t % 2, KH)]
        if build:
            for k0 in range(0, FH, 16):
                blk = lambda t: w4_v[(t // 2) * FH + k0:(t // 2) * FH + k0 + 16, _half(t % 2, KH)]
                t4_ref[i * FQ + k0 // 2:i * FQ + k0 // 2 + 8, :] = _pk(_operand(blk, RHS_TERMS[i]))
        return _up(t4_ref[_half(i, FQ), :])

    def finish(r0, off, n, first):
        tails, gates = [], []
        gw = gw_v[...].astype(f32).reshape(1, D)
        for half in range(2):
            o2 = off + half * HC
            tails.append(_dot(_up(ur_ref[o2 // 2:(o2 + n) // 2, :]), w4_v[FM:F, :]))
            gl = jnp.sum(x_v[pl.ds(r0 + o2, n), :].astype(f32) * gw, axis=-1, keepdims=True)
            gates.append(0.5 * jnp.tanh(0.5 * gl) + 0.5)
        ms = [None] * 7
        for i in ORDER:
            w = w4_operand(i, first)
            ms[i] = _dot(_up(u_ref[i * HH + off // 2:i * HH + (off + n) // 2, :]), w)
        cq = _quadrants(*ms)
        for t in DONE:
            half, cols = t // 2, _half(t % 2, KH)
            o2 = off + half * HC
            rows = pl.ds(r0 + o2, n)
            b = x1_ref[rows, cols] + tails[half][:, cols] + cq[t]
            out_v[rows, cols] = (b + gates[half] * (a_ref[o2:o2 + n, cols] - b)).astype(bf16)
        for half in (1, 0):
            rows = pl.ds(r0 + off + half * HC, n)
            copy(out_v.at[rows], out_hbm.at[rows], 0).start()

    def phase2(t, carry):
        r0 = pl.multiple_of(t * T2, T2)
        phi_q(r0)
        attn_out(0)
        attn_out(1)
        ln2(r0)
        attn_proj(0)
        attn_proj(1)
        prev = None
        for b in range(FH // NB):
            ms = mlp_products(b)
            if prev is not None:
                mlp_act(b - 1, prev)
            prev = ms
        mlp_tail(0)
        mlp_tail(1)
        mlp_act(FH // NB - 1, prev)
        off = 0
        for n in OUT_CHUNKS:
            finish(r0, off, n, off == 0)
            off += n
        return carry

    lax.fori_loop(0, NT2, phase2, 0)
    copy(out_v, out_hbm, 0).wait()


def _kernel(*refs):
    trips = refs[-1]
    trips[0] = 1

    def once(i, carry):
        _body(i, *refs[:-1])
        return carry

    lax.fori_loop(0, trips[0], once, 0)


@jax.jit
def pallas_gated_mix__linear_kernel_hedgehog__mixer_s_mlp__prompt_kernel(
        A_x, A_wqkv, A_w_phi, A_wo, B_x, B_w1, B_w2, B_w3, B_w4, gate_w):
    del B_x
    x = A_x.reshape(S, D)
    wphi = jnp.transpose(A_w_phi, (1, 2, 0)).reshape(DH * DH, H)
    w3t = B_w3.T
    hbm = pl.BlockSpec(memory_space=pl.ANY)
    out = pl.pallas_call(
        _kernel,
        out_shape=jax.ShapeDtypeStruct((S, D), bf16),
        in_specs=[hbm] * 9,
        out_specs=hbm,
        scratch_shapes=[
            pltpu.VMEM((S + AH, D), bf16),
            pltpu.VMEM((D, D), bf16),
            pltpu.VMEM((D, D), bf16),
            pltpu.VMEM((D, D), bf16),
            pltpu.VMEM((DH * DH, H), bf16),
            pltpu.VMEM((D, D), bf16),
            pltpu.VMEM((D, D), bf16),
            pltpu.VMEM((D, D), bf16),
            pltpu.VMEM((F, D), bf16),
            pltpu.VMEM((F, D), bf16),
            pltpu.VMEM((D,), bf16),
            pltpu.VMEM((S, D), bf16),
            pltpu.VMEM((MQ + D // 2, D), u32),
            pltpu.VMEM((4, PAD + S + AH, 128), f32),
            pltpu.VMEM((D, 128), f32),
            pltpu.VMEM((NJ * 128, 128), f32),
            pltpu.VMEM((NJ * 64, T2), u32),
            pltpu.VMEM((64, D), u32),
            pltpu.VMEM((T1, D), f32),
            pltpu.VMEM((D // 2, T1), u32),
            pltpu.VMEM((S, D), f32),
            pltpu.VMEM((9 * HH, KH), u32),
            pltpu.VMEM((ANCHOR + 8 * FH // NB, FH), u32),
            pltpu.VMEM((T2 // 2, F - FM), u32),
            pltpu.VMEM((7 * FQ, KH), u32),
            pltpu.VMEM((T2, D), f32),
            pltpu.VMEM((T2, D), f32),
            pltpu.VMEM((7 * KQ, KH), u32),
            pltpu.VMEM((7 * KQ, KH), u32),
            pltpu.SemaphoreType.DMA((4,)),
            pltpu.SMEM((1,), jnp.int32),
        ],
        compiler_params=pltpu.CompilerParams(vmem_limit_bytes=100 * 1024 * 1024,
                                             disable_bounds_checks=True),
    )(x, A_wqkv, wphi, A_wo, B_w1, B_w2, w3t, B_w4, gate_w)
    return out.reshape(1, S, D)
```

```python
import jax
import jax.numpy as jnp
from jax import lax
import jax.experimental.pallas as pl
import jax.experimental.pallas.tpu as pltpu

S, D, H, DH, F = 2048, 512, 32, 16, 1376
NJ = 8
MQ = 480
T0 = 384
P0 = 512
T1 = 768
N1 = (S - P0) // T1
R2 = 512
T2 = 1024
NT2 = S // T2
HC = T2 // 2
FM = 1280
AH = 32
PAD = 8
NB = 128
OUT_CHUNKS = (224, 160, 96, 32)
KH, KQ = D // 2, D // 4
FH, FQ = FM // 2, FM // 4
HH = HC // 2
ANCHOR = 7 * HH
LOG2E = 1.4426950408889634
NT_DIMS = (((1,), (1,)), ((), ()))
SHIFTS = (-1, 1, -2, 2)
LHS_TERMS = ((0, 3, 1), (2, 3, 1), (0, None, 1), (3, None, 1), (0, 1, 1), (2, 0, -1), (1, 3, -1))
RHS_TERMS = ((0, 3, 1), (0, None, 1), (1, 3, -1), (2, 0, -1), (3, None, 1), (0, 1, 1), (2, 3, 1))
OUT_TERMS = (((0, 1), (3, 1), (4, -1), (6, 1)), ((2, 1), (4, 1)), ((1, 1), (3, 1)),
             ((0, 1), (1, -1), (2, 1), (5, 1)))
O_V0, O_V = (4, 3, 0, 1, 2, 5, 6), (6, 3, 4, 0, 5, 2, 1)
O_W1 = O_W2 = (1, 3, 2, 4, 0, 6, 5)
O_WO, O_W3, O_W4 = (1, 3, 6, 0, 4, 2, 5), (1, 3, 6, 4, 0, 5, 2), (2, 4, 3, 1, 0, 6, 5)
f32 = jnp.float32
bf16 = jnp.bfloat16
u32 = jnp.uint32


def _pk(x):
    return pltpu.bitcast(x.astype(bf16), u32)


def _up(x):
    return pltpu.bitcast(x, bf16)


def _dot(a, b):
    return jnp.dot(a, b, preferred_element_type=f32)


def _dot_nt(a, b):
    return lax.dot_general(a, b, NT_DIMS, preferred_element_type=f32)


def _gelu(hx):
    c = 0.7978845608028654
    t = jnp.tanh(hx * (2.0 * c + (8.0 * c * 0.044715) * (hx * hx)))
    return hx + hx * t


def _half_rstd(xc):
    v4 = jnp.sum(xc * xc, axis=-1, keepdims=True) * (4.0 / D)
    return jnp.exp2((-0.5 * LOG2E) * jnp.log(v4 + 4e-5))


def _recip(x):
    r = pl.reciprocal(x, approx=True)
    return r * (2.0 - x * r)


def _fold4(a, op):
    return op(a, pltpu.roll(a, 4, 0))


def _dual_exp(p):
    mx = _fold4(jnp.max(p, axis=0), jnp.maximum)
    mn = _fold4(jnp.min(p, axis=0), jnp.minimum)
    ep = jnp.exp2(p - mx[None])
    en = jnp.exp2(mn[None] - p)
    rp = _recip(_fold4(jnp.sum(ep, axis=0), jnp.add))
    rn = _recip(_fold4(jnp.sum(en, axis=0), jnp.add))
    return ep, en, rp, rn


def _logits(pm, j, c):
    lo = lax.broadcasted_iota(jnp.int32, (8, 128), 0) < 4
    g, jj = j // 2, j % 2
    cs = slice(c * 128, (c + 1) * 128)
    own = pm[g * 120 + jj * 64:g * 120 + jj * 64 + 56, cs].reshape(7, 8, 128)
    sh = pm[g * 120 + 56:g * 120 + 64, cs]
    last = jnp.where(lo, sh, 0.0) if jj == 0 else jnp.where(lo, 0.0, sh)
    return jnp.concatenate([own, last[None]], axis=0)


def _operand(blk, term):
    p, q, sign = term
    if q is None:
        return blk(p).astype(bf16)
    a, b = blk(p).astype(f32), blk(q).astype(f32)
    return (a + b if sign > 0 else a - b).astype(bf16)


def _products(lhs, rhs, dot, order):
    ms = [None] * 7
    for i in order:
        a = lhs(i)
        ms[i] = dot(a, rhs(i))
    return ms


def _quadrants(ms, order):
    out = []
    for t, terms in enumerate(OUT_TERMS):
        ts = sorted(terms, key=lambda u: order.index(u[0]))
        if ts[0][1] < 0:
            ts[0], ts[1] = ts[1], ts[0]
        acc = ms[ts[0][0]]
        for i, sign in ts[1:]:
            acc = acc + ms[i] if sign > 0 else acc - ms[i]
        out.append((max(order.index(u[0]) for u in terms), t, acc))
    return [(t, acc) for _, t, acc in sorted(out, key=lambda u: u[:2])]


def _half(t, n):
    return slice(t * n, (t + 1) * n)


def _body(zero, x_hbm, wqkv_hbm, wphi_hbm, wo_hbm, w1_hbm, w2_hbm, w3t_hbm, w4_hbm, gw_hbm,
          out_hbm,
          x_v, wq_v, wk_v, wv_v, wphi_v, wo_v, w1_v, w2_v, w3t_v, w4_v, gw_v, out_v,
          wt_ref, h_ref, kv_ref, z_ref, phi_ref, p_ref, xn_ref, vt_ref,
          x1_ref, sa_ref, u_ref, ur_ref, t4_ref, o_ref, a_ref, va_ref, t1_ref, sem):
    def copy(src, dst, k):
        return pltpu.make_async_copy(src, dst, sem.at[k])

    def xcopy(a, b, k):
        return copy(x_hbm.at[a:b], x_v.at[a:b], k)

    def fresh(ref, k):
        return ref.at[pl.ds(pl.multiple_of(zero * (16 * (k + 1)), 16), ref.shape[0])]

    def kept(ref, rows, i, build, make):
        if build:
            ref[_half(i, rows), :] = _pk(make())
        return _up(ref[_half(i, rows), :])

    c_phi = copy(wphi_hbm, wphi_v, 0)
    c_wk = copy(wqkv_hbm.at[:, D:2 * D], wk_v, 1)
    c_x0 = xcopy(0, T0, 2)
    c_x1 = xcopy(T0, P0 + AH, 3)
    c_wv = copy(wqkv_hbm.at[:, 2 * D:3 * D], wv_v, 3)
    c_w1 = copy(w1_hbm, w1_v, 1)
    c_loop1 = [copy(w2_hbm, w2_v, 2), xcopy(P0 + AH, S, 2)]
    c_late = [copy(wqkv_hbm.at[:, 0:D], wq_v, 3), copy(w3t_hbm, w3t_v, 3), copy(w4_hbm, w4_v, 3),
              copy(wo_hbm, wo_v, 3), copy(gw_hbm, gw_v, 3)]
    c_phi.start()
    c_wk.start()

    x_v[S:S + AH, :] = jnp.zeros((AH, D), bf16)
    for q in range(4):
        h_ref[q, 0:PAD, :] = jnp.zeros((PAD, 128), f32)

    c_phi.wait()
    c_x0.start()
    c_x1.start()
    sel = (lax.broadcasted_iota(jnp.int32, (H, D), 0)
           == lax.broadcasted_iota(jnp.int32, (H, D), 1) // DH)
    bm = _dot(wphi_v[...], jnp.where(sel, 1.0, 0.0).astype(bf16))
    dmask = (lax.broadcasted_iota(jnp.int32, (DH * DH, D), 0) // DH
             == lax.broadcasted_iota(jnp.int32, (DH * DH, D), 1) % DH)
    cm = jnp.sum(jnp.where(dmask, bm, 0.0).reshape(DH, DH, D), axis=0).astype(bf16)
    e3 = ((lax.broadcasted_iota(jnp.int32, (128, DH), 0) % 64) // 4
          == lax.broadcasted_iota(jnp.int32, (128, DH), 1))
    pall = _dot(jnp.where(e3, 1.0, 0.0).astype(bf16), cm)
    rr = lax.broadcasted_iota(jnp.int32, (128, D), 0)
    cc = lax.broadcasted_iota(jnp.int32, (128, D), 1)
    pmask = ((cc // DH) % 8) == ((rr // 64) * 4 + rr % 4)
    p_ref[...] = _pk(jnp.where(pmask, pall, 0.0))

    def fold(w_v, base):
        lo = lax.broadcasted_iota(jnp.int32, (8, D), 0) < 4
        for gp in range(2):
            rows = []
            for g in (2 * gp, 2 * gp + 1):
                wt = _dot_nt(_up(p_ref[:, _half(g, 128)]), w_v[:, _half(g, 128)])
                ds = []
                for jj in range(2):
                    a = wt[_half(jj, 64), :].reshape(8, 8, D)
                    f15 = jnp.where(lo, pltpu.roll(a[7], 4, 0), a[7])
                    ds.append((a - f15[None]) * LOG2E)
                f14 = jnp.where(lo, ds[0][7], pltpu.roll(ds[1][7], 4, 0))
                rows += [ds[0][0:7].reshape(56, D), f14, ds[1][0:7].reshape(56, D)]
            wt_ref[base + gp * 120:base + (gp + 1) * 120, :] = _pk(jnp.concatenate(rows, axis=0))

    def phi_k(r0, n, off=0, first=False):
        pk = _dot_nt(_up(wt_ref[MQ // 2:MQ, :]), x_v[pl.ds(r0, n), :])
        for c in range(n // 128):
            cs = slice(off + c * 128, off + (c + 1) * 128)
            for j in range(NJ):
                ep, en, rp, rn = _dual_exp(_logits(pk, j, c))
                ep = (ep * rp[None]).reshape(64, 128)
                en = (en * rn[None]).reshape(64, 128)
                if first and c == 0:
                    z_ref[_half(2 * j, 64), :] = ep
                    z_ref[_half(2 * j + 1, 64), :] = en
                else:
                    z_ref[_half(2 * j, 64), :] += ep
                    z_ref[_half(2 * j + 1, 64), :] += en
                phi_ref[_half(2 * j, 32), cs] = _pk(ep)
                phi_ref[_half(2 * j + 1, 32), cs] = _pk(en)

    def v_proj(r0, n, first=False):
        m = n // 2
        wblk = lambda t: _up(wt_ref[MQ + (t // 2) * KQ:MQ + (t // 2 + 1) * KQ, _half(t % 2, KH)])

        def lhs(i):
            if LHS_TERMS[i][1] is None:
                return wblk(LHS_TERMS[i][0])
            return kept(va_ref, KQ, i, first, lambda: _operand(wblk, LHS_TERMS[i]))

        def rhs(i):
            ri = r0 + zero * (16 * (i + 1))
            xblk = lambda t: x_v[pl.ds(pl.multiple_of(ri + (t % 2) * m, 16), m), _half(t // 2, KH)]
            return _operand(xblk, RHS_TERMS[i])

        order = O_V0 if first else O_V
        for t, c in _quadrants(_products(lhs, rhs, _dot_nt, order), order):
            vt_ref[_half(t // 2, KQ), _half(t % 2, m)] = _pk(c)

    def kv_acc(n, first=False):
        for j in range(NJ):
            r = _dot_nt(_up(vt_ref[_half(j, 32), 0:n]), _up(phi_ref[_half(j, 64), 0:n]))
            if first:
                kv_ref[_half(j, 64), :] = r
            else:
                kv_ref[_half(j, 64), :] += r

    def ln1(r0, n, ch):
        for r in range(0, n, ch):
            x = x_v[pl.ds(r0 + r, ch), :].astype(f32)
            xc = x - jnp.mean(x, axis=-1, keepdims=True)
            xn_ref[r:r + ch, :] = xc * _half_rstd(xc)

    def times_square(blk, w_v, order, keep=None, build=False):
        def rhs(i):
            w = fresh(w_v, i)
            make = lambda: _operand(lambda t: w[_half(t // 2, KH), _half(t % 2, KH)], RHS_TERMS[i])
            if keep is None or RHS_TERMS[i][1] is None:
                return make()
            return kept(keep, KQ, i, build, make)

        return _quadrants(_products(lambda i: _operand(blk, LHS_TERMS[i]), rhs, _dot, order), order)

    def mix_in(r0, n, first=False):
        m = n // 2
        blk = lambda t: xn_ref[_half(t // 2, m), _half(t % 2, KH)]
        for t, c in times_square(blk, w1_v, O_W1, t1_ref, first):
            h = _gelu(c)
            for q in range(2):
                h_ref[2 * (t % 2) + q, pl.ds(PAD + r0 + (t // 2) * m, m), :] = h[:, _half(q, 128)]

    def mix_out(r0, n):
        m = n // 2

        def shifted(t):
            return jnp.concatenate(
                [h_ref[q, pl.ds(PAD + r0 + (t // 2) * m + SHIFTS[q], m), :]
                 for q in (2 * (t % 2), 2 * (t % 2) + 1)], axis=1)

        for t, c in times_square(shifted, w2_v, O_W2):
            rows, cols = pl.ds(r0 + (t // 2) * m, m), _half(t % 2, KH)
            x1_ref[rows, cols] = x_v[rows, cols].astype(f32) + c

    c_wk.wait()
    c_wv.start()
    c_w1.start()
    fold(wk_v, MQ // 2)
    c_x0.wait()
    for c in c_loop1:
        c.start()
    phi_k(0, T0, first=True)
    c_x1.wait()
    c_wv.wait()
    for c in c_late:
        c.start()
    phi_k(T0, P0 - T0, off=T0)
    wt_ref[MQ:MQ + D // 2, :] = _pk(wv_v[...].T)
    ln1(0, P0 + AH, 32)
    v_proj(0, P0, first=True)
    c_w1.wait()
    mix_in(0, P0 + AH, first=True)
    kv_acc(P0, first=True)
    for c in c_loop1:
        c.wait()

    def phase1(i, carry):
        r0 = pl.multiple_of(P0 + i * T1, 256)
        mix_out(pl.multiple_of(i * R2, R2), R2)
        phi_k(r0, T1)
        ln1(r0 + AH, T1, 16)
        v_proj(r0, T1)
        mix_in(r0 + AH, T1)
        kv_acc(T1)
        return carry

    lax.fori_loop(0, N1, phase1, 0)

    for c in c_late:
        c.wait()
    for q in (1, 3):
        h_ref[q, PAD + S:PAD + S + 8, :] = jnp.zeros((8, 128), f32)
    mix_out(N1 * R2, R2)
    fold(wq_v, 0)
    z_ref[...] = jnp.broadcast_to(jnp.sum(z_ref[...], axis=1, keepdims=True), z_ref.shape)
    for b in range(FH // NB):
        u_ref[ANCHOR + b * 8:ANCHOR + (b + 1) * 8, 0:KH] = _pk(w3t_v[b * NB:b * NB + 16, 0:KH])
    mix_out((N1 + 1) * R2, R2)

    def phi_q(r0):
        pq = _dot_nt(_up(wt_ref[0:MQ // 2, :]), x_v[pl.ds(r0, T2), :])
        for c in range(T2 // 128):
            for j in range(NJ):
                zp = z_ref[_half(2 * j, 64), :].reshape(8, 8, 128)
                zn = z_ref[_half(2 * j + 1, 64), :].reshape(8, 8, 128)
                ep, en, rp, rn = _dual_exp(_logits(pq, j, c))
                den = jnp.sum(ep * zp, axis=0) * rp + jnp.sum(en * zn, axis=0) * rn
                rd = _recip(_fold4(den, jnp.add) + 1e-6)
                phi_ref[_half(2 * j, 32), _half(c, 128)] = _pk((ep * (rp * rd)[None]).reshape(64, 128))
                phi_ref[_half(2 * j + 1, 32), _half(c, 128)] = _pk((en * (rn * rd)[None]).reshape(64, 128))

    def attn_out(k):
        own = ((lax.broadcasted_iota(jnp.int32, (64, 128), 1) & 3)
               == (lax.broadcasted_iota(jnp.int32, (64, 128), 0) >> 4))
        ot = [_dot(jnp.where(own, kv_ref[_half(j, 64), :], 0.0).astype(bf16),
                   _up(phi_ref[_half(j, 64), _half(k, HC)])) for j in range(NJ)]
        o_ref[_half(k, HC), :] = jnp.concatenate(ot, axis=0).T

    def attn_proj(k):
        blk = lambda t: o_ref[_half(2 * k + t // 2, HH), _half(t % 2, KH)]
        for t, c in times_square(blk, wo_v, O_WO):
            a_ref[_half(2 * k + t // 2, HH), _half(t % 2, KH)] = c

    def ln2(r0):
        views = [x1_ref.at[pl.ds(pl.multiple_of(r0 + zero * (8 * p), 8), T2)] for p in range(3)]

        def norm(r):
            m = jnp.mean(views[0][r:r + 16, :], axis=-1, keepdims=True)
            rs = _half_rstd(views[1][r:r + 16, :] - m)
            return (views[2][r:r + 16, :] - m) * rs

        for r in range(0, HC, 16):
            y = (norm(r), norm(HC + r))
            blk = lambda t: y[t // 2][:, _half(t % 2, KH)]
            for i, term in enumerate(LHS_TERMS + ((1, None, 1), (2, None, 1))):
                sa_ref[i * HH + r // 2:i * HH + r // 2 + 8, :] = _pk(_operand(blk, term))

    def mlp_products(b):
        n0 = b * NB

        def rhs(i):
            if i == 1:
                head = _up(u_ref[ANCHOR + b * 8:ANCHOR + (b + 1) * 8, 0:KH])
                return jnp.concatenate([head, w3t_v[n0 + 16:n0 + NB, 0:KH]], axis=0)
            w = w3t_v if RHS_TERMS[i][1] is None else fresh(w3t_v, i)
            blk = lambda t: w[(t % 2) * FH + n0:(t % 2) * FH + n0 + NB, _half(t // 2, KH)]
            return _operand(blk, RHS_TERMS[i])

        return _products(lambda i: _up(sa_ref[_half(i, HH), :]), rhs, _dot_nt, O_W3)

    act_ref = u_ref.at[pl.ds(pl.multiple_of(zero * 8, 8), ANCHOR)]

    def mlp_act(b, ms):
        for r in range(0, HC, 16):
            u = {t: _gelu(c) for t, c in _quadrants([m[r:r + 16] for m in ms], O_W3)}
            for i, term in enumerate(LHS_TERMS):
                act_ref[i * HH + r // 2:i * HH + r // 2 + 8, _half(b, NB)] = _pk(
                    _operand(lambda t: u[t], term))

    def mlp_tail(k):
        xh = jnp.concatenate([sa_ref[_half(i, HH), :] for i in ((2, 7), (8, 3))[k]], axis=1)
        ut = _gelu(_dot_nt(w3t_v[FM:F, :], _up(xh)))
        ut = jnp.concatenate([ut, jnp.zeros((128 - (F - FM), HC), f32)], axis=0)
        ur_ref[_half(k, HH), :] = _pk(ut.T)[:, 0:F - FM]

    def w4_operand(i, build):
        if RHS_TERMS[i][1] is None:
            t = RHS_TERMS[i][0]
            return w4_v[_half(t // 2, FH), _half(t % 2, KH)]
        if build:
            for k0 in range(0, FH, 16):
                blk = lambda t: w4_v[(t // 2) * FH + k0:(t // 2) * FH + k0 + 16, _half(t % 2, KH)]
                t4_ref[i * FQ + k0 // 2:i * FQ + k0 // 2 + 8, :] = _pk(_operand(blk, RHS_TERMS[i]))
        return _up(t4_ref[_half(i, FQ), :])

    def finish(r0, off, n, first):
        tails, gates = [], []
        gw = gw_v[...].astype(f32).reshape(1, D)
        for half in range(2):
            o2 = off + half * HC
            tails.append(_dot(_up(ur_ref[o2 // 2:(o2 + n) // 2, :]), w4_v[FM:F, :]))
            gl = jnp.sum(x_v[pl.ds(r0 + o2, n), :].astype(f32) * gw, axis=-1, keepdims=True)
            gates.append(0.5 * jnp.tanh(0.5 * gl) + 0.5)
        ms = [None] * 7
        for i in O_W4:
            w = w4_operand(i, first)
            ms[i] = _dot(_up(u_ref[i * HH + off // 2:i * HH + (off + n) // 2, :]), w)
        cq = _quadrants(ms, O_W4)
        for t, c in cq:
            half, cols = t // 2, _half(t % 2, KH)
            o2 = off + half * HC
            rows = pl.ds(r0 + o2, n)
            b = x1_ref[rows, cols] + tails[half][:, cols] + c
            out_v[rows, cols] = (b + gates[half] * (a_ref[o2:o2 + n, cols] - b)).astype(bf16)
        last = cq[-1][0] // 2
        for half in (1 - last, last):
            rows = pl.ds(r0 + off + half * HC, n)
            copy(out_v.at[rows], out_hbm.at[rows], 0).start()

    def phase2(t, carry):
        r0 = pl.multiple_of(t * T2, T2)
        phi_q(r0)
        attn_out(0)
        attn_out(1)
        ln2(r0)
        attn_proj(0)
        attn_proj(1)
        prev = None
        for b in range(FH // NB):
            ms = mlp_products(b)
            if prev is not None:
                mlp_act(b - 1, prev)
            prev = ms
        mlp_tail(0)
        mlp_tail(1)
        mlp_act(FH // NB - 1, prev)
        off = 0
        for n in OUT_CHUNKS:
            finish(r0, off, n, off == 0)
            off += n
        return carry

    lax.fori_loop(0, NT2, phase2, 0)
    copy(out_v, out_hbm, 0).wait()


def _kernel(*refs):
    trips = refs[-1]
    trips[0] = 1

    def once(i, carry):
        _body(i, *refs[:-1])
        return carry

    lax.fori_loop(0, trips[0], once, 0)


@jax.jit
def pallas_gated_mix__linear_kernel_hedgehog__mixer_s_mlp__prompt_kernel(
        A_x, A_wqkv, A_w_phi, A_wo, B_x, B_w1, B_w2, B_w3, B_w4, gate_w):
    del B_x
    x = A_x.reshape(S, D)
    wphi = jnp.transpose(A_w_phi, (1, 2, 0)).reshape(DH * DH, H)
    w3t = B_w3.T
    hbm = pl.BlockSpec(memory_space=pl.ANY)
    out = pl.pallas_call(
        _kernel,
        out_shape=jax.ShapeDtypeStruct((S, D), bf16),
        in_specs=[hbm] * 9,
        out_specs=hbm,
        scratch_shapes=[
            pltpu.VMEM((S + AH, D), bf16),
            pltpu.VMEM((D, D), bf16),
            pltpu.VMEM((D, D), bf16),
            pltpu.VMEM((D, D), bf16),
            pltpu.VMEM((DH * DH, H), bf16),
            pltpu.VMEM((D, D), bf16),
            pltpu.VMEM((D, D), bf16),
            pltpu.VMEM((D, D), bf16),
            pltpu.VMEM((F, D), bf16),
            pltpu.VMEM((F, D), bf16),
            pltpu.VMEM((D,), bf16),
            pltpu.VMEM((S, D), bf16),
            pltpu.VMEM((MQ + D // 2, D), u32),
            pltpu.VMEM((4, PAD + S + AH, 128), f32),
            pltpu.VMEM((D, 128), f32),
            pltpu.VMEM((NJ * 128, 128), f32),
            pltpu.VMEM((NJ * 64, T2), u32),
            pltpu.VMEM((64, D), u32),
            pltpu.VMEM((T1, D), f32),
            pltpu.VMEM((D // 2, T1), u32),
            pltpu.VMEM((S, D), f32),
            pltpu.VMEM((9 * HH, KH), u32),
            pltpu.VMEM((ANCHOR + 8 * FH // NB, FH), u32),
            pltpu.VMEM((T2 // 2, F - FM), u32),
            pltpu.VMEM((7 * FQ, KH), u32),
            pltpu.VMEM((T2, D), f32),
            pltpu.VMEM((T2, D), f32),
            pltpu.VMEM((7 * KQ, KH), u32),
            pltpu.VMEM((7 * KQ, KH), u32),
            pltpu.SemaphoreType.DMA((4,)),
            pltpu.SMEM((1,), jnp.int32),
        ],
        compiler_params=pltpu.CompilerParams(vmem_limit_bytes=100 * 1024 * 1024,
                                             disable_bounds_checks=True),
    )(x, A_wqkv, wphi, A_wo, B_w1, B_w2, w3t, B_w4, gate_w)
    return out.reshape(1, S, D)
```
